```python
import jax
import jax.numpy as jnp

def _softmax(x, axis=-1):
    return jax.nn.softmax(x, axis=axis)

def _gelu(x):
    return jax.nn.gelu(x, approximate=True)

def _silu(x):
    return jax.nn.silu(x)

def _sigmoid(x):
    return jax.nn.sigmoid(x)

def _layernorm(x, axis=-1, eps=1e-05):
    m = jnp.mean(x, axis=axis, keepdims=True)
    v = jnp.var(x, axis=axis, keepdims=True)
    return (x - m) / jnp.sqrt(v + eps)

def _scatter_add(tgt, idx, src, axis=0):
    return tgt.at[idx].add(src)

def _segment_sum(src, seg, n):
    return jax.ops.segment_sum(src, seg, n)

class _Rng:

    def __init__(self, key):
        self._k = key

    def _next(self):
        self._k, sub = jax.random.split(self._k)
        return sub

    def normal(self, shape):
        return jax.random.normal(self._next(), shape, dtype=jnp.bfloat16)

    def randint(self, lo, hi, shape):
        return jax.random.randint(self._next(), shape, lo, hi, dtype=jnp.int32)

    def uniform(self, shape, lo=0.0, hi=1.0):
        return jax.random.uniform(self._next(), shape, jnp.bfloat16, lo, hi)

    def permutation(self, n):
        return jax.random.permutation(self._next(), n)
kernel_name = 'adaLN_cond__sliding_local_dilated__swiglu_ffn__prompt'

def setup_inputs():
    _rng = _Rng(jax.random.key(int.from_bytes(__import__("os").urandom(4), "little")))
    _w = lambda a: (lambda t: t.astype(jnp.bfloat16) if jnp.issubdtype(t.dtype, jnp.floating) else t)(jnp.asarray(a))

    def _A_setup():
        B, S, D = (1, 2048, 1024)
        return {'x': _w((lambda *s: _rng.normal(s) * 0.05)(B, S, D)), 'wqkv': _w((lambda *s: _rng.normal(s) * 0.05)(D, 3 * D)), 'wo': _w((lambda *s: _rng.normal(s) * 0.05)(D, D))}
    _A_in = _A_setup()

    def _B_setup():
        B, S, D, F = (1, 2048, 1024, 3584)
        return {'x': _w((lambda *s: _rng.normal(s) * 0.05)(B, S, D)), 'w_gate': _w((lambda *s: _rng.normal(s) * 0.05)(D, F)), 'w_up': _w((lambda *s: _rng.normal(s) * 0.05)(D, F)), 'w_down': _w((lambda *s: _rng.normal(s) * 0.05)(F, D))}
    _B_in = _B_setup()
    return {'A_x': _A_in['x'], 'A_wqkv': _A_in['wqkv'], 'A_wo': _A_in['wo'], 'B_x': _B_in['x'], 'B_w_gate': _B_in['w_gate'], 'B_w_up': _B_in['w_up'], 'B_w_down': _B_in['w_down'], 'c': _w((lambda *s: _rng.normal(s) * 0.05)(1, 1024)), 'w_mod': _w((lambda *s: _rng.normal(s) * 0.05)(1024, 6 * 1024) * 1024 ** (-0.5))}

def reference(A_x, A_wqkv, A_wo, B_x, B_w_gate, B_w_up, B_w_down, c, w_mod):

    def _A_ref(x, wqkv, wo):
        B, S, D = x.shape
        H = 32
        Dh = D // H
        W, dil = (8, 2)
        qkv = (lambda x, *d: x.transpose(*d))((x @ wqkv).reshape(B, S, 3, H, Dh), 2, 0, 3, 1, 4)
        q, k, v = (qkv[0], qkv[1], qkv[2])
        scale = Dh ** (-0.5)
        pos = jnp.arange(S)
        off = jnp.arange(W) * dil
        idx = pos[:, None] - off[None, :]
        mask = idx >= 0
        idx_c = jnp.where(mask, idx, 0).reshape(-1)
        kg = k[:, :, idx_c, :].reshape(B, H, S, W, Dh)
        vg = v[:, :, idx_c, :].reshape(B, H, S, W, Dh)
        logits = jnp.einsum('bhsd,bhswd->bhsw', q, kg) * scale
        logits = jnp.where(mask[None, None, :, :], logits, -1000000000.0)
        attn = _softmax(logits, axis=-1)
        o = jnp.einsum('bhsw,bhswd->bhsd', attn, vg)
        return (lambda x, *d: x.transpose(*d))(o, 0, 2, 1, 3).reshape(B, S, D) @ wo

    def _B_ref(x, w_gate, w_up, w_down):
        g = _silu(x @ w_gate)
        u = x @ w_up
        return g * u @ w_down
    x = A_x
    mod = (_silu(c) @ w_mod).reshape(c.shape[0], 6, 1, -1)
    sa, ca, ga, sb, cb, gb = (mod[:, 0].copy(), mod[:, 1].copy(), mod[:, 2].copy(), mod[:, 3].copy(), mod[:, 4].copy(), mod[:, 5].copy())
    h = _layernorm(x, axis=-1) * (1 + ca) + sa
    x = x + ga * _A_ref(h, A_wqkv, A_wo)
    h = _layernorm(x, axis=-1) * (1 + cb) + sb
    x = x + gb * _B_ref(h, B_w_gate, B_w_up, B_w_down)
    return x
```

```python
import jax
import jax.numpy as jnp
from jax import lax
from jax.experimental import pallas as pl
from jax.experimental.pallas import tpu as pltpu

S, D, F = 2048, 1024, 3584
H, DH, W, DIL = 32, 32, 8, 2
TM = 512
NT = S // TM
HALO = 16
FC = 512
NFC = F // FC
DC = 256
NDC = D // DC
AR = 32
LR = 64
MC = 512
NLT = D // 128
QC = 512
N_GU = 12
EPS = 1e-5
SCALE = DH ** -0.5
F32, BF16 = jnp.float32, jnp.bfloat16


def _swap_tiles_lanes(tiles):
    lane = lax.broadcasted_iota(jnp.int32, tiles[0].shape, 1)
    for b in range(3):
        sh = 4 << b
        low = (lane & sh) == 0
        new = list(tiles)
        for t in range(NLT):
            if not (t >> b) & 1:
                a, c = tiles[t], tiles[t | (1 << b)]
                new[t] = jnp.where(low, a, pltpu.roll(c, sh, 1))
                new[t | (1 << b)] = jnp.where(low, pltpu.roll(a, 128 - sh, 1), c)
        tiles = new
    return tiles


def _permute_bf16(val):
    u = pltpu.bitcast(val, jnp.uint32)
    tiles = _swap_tiles_lanes([u[:, t * 128:(t + 1) * 128] for t in range(NLT)])
    return pltpu.bitcast(jnp.concatenate(tiles, axis=1), BF16)


def _ln_mod(x, scale1, shift):
    m = jnp.mean(x, axis=-1, keepdims=True)
    xc = x - m
    v = jnp.mean(xc * xc, axis=-1, keepdims=True)
    return xc * lax.rsqrt(v + EPS) * scale1 + shift


def _kernel(x_hbm, c_ref, wmod_hbm, wqkv_hbm, wo_hbm, wg_hbm, wu_hbm, wd_hbm, out_hbm,
            x_v, out_v, wmod_v, wqkv_v, wo_v, wg_v, wu_v, wd_v, mod_v, h_s, q_s, k_s, v_s, o_s,
            x1_s, h2_s, act_s, sems, xsems, osems):
    n_mod = 6 * D // MC

    def mod_cp(j):
        return pltpu.make_async_copy(wmod_hbm.at[:, pl.ds(j * MC, MC)],
                                     wmod_v.at[:, pl.ds(j * MC, MC)], sems.at[j])

    def qkv_cp(j):
        return pltpu.make_async_copy(wqkv_hbm.at[:, pl.ds(j * D, D)],
                                     wqkv_v.at[:, pl.ds(j * D, D)], sems.at[n_mod + j])

    def x_cp(i):
        return pltpu.make_async_copy(x_hbm.at[i], x_v.at[i], xsems.at[i])

    def out_cp(i, n):
        cs = pl.ds(n * DC, DC)
        return pltpu.make_async_copy(out_v.at[i, :, cs], out_hbm.at[i, :, cs],
                                     osems.at[i * NDC + n])

    wo_cp = pltpu.make_async_copy(wo_hbm, wo_v, sems.at[n_mod + 3])
    wg_cp = pltpu.make_async_copy(wg_hbm, wg_v, sems.at[n_mod + 4])
    wu_cp = pltpu.make_async_copy(wu_hbm, wu_v, sems.at[n_mod + 5])
    wd_cp = pltpu.make_async_copy(wd_hbm, wd_v, sems.at[n_mod + 6])
    per = D // MC

    def mod_cps(k):
        return [mod_cp(j) for j in range(k * per, (k + 1) * per)]

    def start(cps):
        for cp in cps:
            cp.start()

    def mod_chunk(j):
        mod_cp(j).wait()
        cf = c_ref[...].astype(F32)
        sc = jnp.broadcast_to(cf * jax.nn.sigmoid(cf), (16, D)).astype(BF16)
        r = jnp.dot(sc, wmod_v[:, j * MC:(j + 1) * MC], preferred_element_type=F32)
        if j // per in (1, 4):
            r = r + 1.0
        mod_v[:, j * MC:(j + 1) * MC] = r[0:8]

    def mod_vec(k):
        for j in range(k * per, (k + 1) * per):
            mod_chunk(j)

    def mod(k):
        return mod_v[0:1, k * D:(k + 1) * D]

    def ln1(i, r):
        xv = x_v[i, r:r + LR, :].astype(F32)
        h_s[i % 2, r:r + LR, :] = _ln_mod(xv, mod(1), mod(0)).astype(BF16)

    def prep_qkv(j):
        qkv_cp(j).wait()
        for r in range(0, D, 128):
            wqkv_v[r:r + 128, j * D:(j + 1) * D] = _permute_bf16(
                wqkv_v[r:r + 128, j * D:(j + 1) * D])

    def qkv_part(i, j, half):
        sl = i % 2
        c0 = j * D + half * QC
        res = jnp.dot(h_s[sl], wqkv_v[:, c0:c0 + QC], preferred_element_type=F32)
        for tt in range(QC // 128):
            t = half * (QC // 128) + tt
            blk = res[:, tt * 128:(tt + 1) * 128]
            if j == 0:
                q_s[sl, t] = blk * SCALE
                continue
            dst = k_s if j == 1 else v_s
            dst[sl, t, HALO:HALO + TM, :] = blk
            if i == 0:
                dst[sl, t, 0:HALO, :] = jnp.broadcast_to(blk[0:1], (HALO, 128))
            if i + 1 < NT:
                dst[1 - sl, t, 0:HALO, :] = blk[TM - HALO:TM]

    def attn_piece(i, r):
        sl = i % 2
        lane = lax.broadcasted_iota(jnp.int32, (AR, 128), 1)
        b0 = (lane & 1) == 0
        b1 = (lane & 2) == 0
        q = [q_s[sl, t, r:r + AR, :] for t in range(NLT)]
        lg = []
        for w in range(W):
            o = HALO + r - DIL * w
            a = q[0] * k_s[sl, 0, o:o + AR, :]
            for t in range(1, NLT):
                a = a + q[t] * k_s[sl, t, o:o + AR, :]
            a = a + jnp.where(b0, pltpu.roll(a, 127, 1), pltpu.roll(a, 1, 1))
            a = a + jnp.where(b1, pltpu.roll(a, 126, 1), pltpu.roll(a, 2, 1))
            if i == 0 and r < DIL * w:
                row = lax.broadcasted_iota(jnp.int32, (AR, 128), 0) + r
                a = jnp.where(row >= DIL * w, a, -1000000000.0)
            lg.append(a)
        m = lg[0]
        for w in range(1, W):
            m = jnp.maximum(m, lg[w])
        e = [jnp.exp(a - m) for a in lg]
        s = e[0]
        for w in range(1, W):
            s = s + e[w]
        inv = 1.0 / s
        p = [a * inv for a in e]
        outs = []
        for t in range(NLT):
            a = p[0] * v_s[sl, t, HALO + r:HALO + r + AR, :]
            for w in range(1, W):
                o = HALO + r - DIL * w
                a = a + p[w] * v_s[sl, t, o:o + AR, :]
            outs.append(a)
        o_s[r:r + AR, :] = _permute_bf16(jnp.concatenate(outs, axis=1).astype(BF16))

    def wo_part(i, half):
        cs = slice(half * QC, (half + 1) * QC)
        y = jnp.dot(o_s[...], wo_v[:, cs], preferred_element_type=F32)
        ga = mod_v[0:1, 2 * D + half * QC:2 * D + (half + 1) * QC]
        x1_s[i % 2, :, cs] = x_v[i, :, cs].astype(F32) + ga * y

    def ln2(i, r):
        h2_s[r:r + LR, :] = _ln_mod(x1_s[i % 2, r:r + LR, :], mod(4), mod(3)).astype(BF16)

    def gate_up(cix):
        cs = slice(cix * FC, (cix + 1) * FC)
        h2 = h2_s[...]
        g = jnp.dot(h2, wg_v[:, cs], preferred_element_type=F32)
        u = jnp.dot(h2, wu_v[:, cs], preferred_element_type=F32)
        t = 0.5 * g
        act_s[:, cs] = ((t + t * jnp.tanh(t)) * u).astype(BF16)

    def down(i, n):
        cs = slice(n * DC, (n + 1) * DC)
        y = jnp.dot(act_s[...], wd_v[:, cs], preferred_element_type=F32)
        gb = mod_v[0:1, 5 * D + n * DC:5 * D + (n + 1) * DC]
        out_v[i, :, cs] = (x1_s[i % 2, :, cs] + gb * y).astype(out_v.dtype)
        out_cp(i, n).start()

    def par(mxu, vpu):
        done = 0
        for idx, (fn, *args) in enumerate(mxu):
            fn(*args)
            upto = len(vpu) * (idx + 1) // len(mxu)
            for vfn, *vargs in vpu[done:upto]:
                vfn(*vargs)
            done = upto

    halves = range(D // QC)

    def t_qkv(i, js=(0, 1, 2)):
        return [(qkv_part, i, j, hf) for j in js for hf in halves]

    def t_attn(i):
        return [(attn_piece, i, r) for r in range(0, TM, AR)]

    def t_ln(fn, i):
        return [(fn, i, r) for r in range(0, TM, LR)] if i < NT else []

    def t_wo(i):
        return [(wo_part, i, hf) for hf in halves]

    t_gu = [(gate_up, cix) for cix in range(NFC)]

    def t_down(i, ns):
        return [(down, i, n) for n in ns]

    start(mod_cps(0) + mod_cps(1) + [x_cp(0)])
    mod_vec(0)
    start([qkv_cp(0)])
    mod_vec(1)
    start([qkv_cp(1)])
    x_cp(0).wait()
    par(t_ln(ln1, 0), [])
    prep_qkv(0)
    start([qkv_cp(2), x_cp(1)])
    par(t_qkv(0, (0,)), [(prep_qkv, 1)])
    start(mod_cps(2) + [wo_cp])
    par(t_qkv(0, (1,)), [(prep_qkv, 2)])
    start(mod_cps(3) + mod_cps(4) + [x_cp(2)])
    x_cp(1).wait()
    par(t_qkv(0, (2,)), t_ln(ln1, 1))
    start([wg_cp])
    par(t_qkv(1) + [(mod_vec, 2), (mod_vec, 3), (mod_vec, 4)], t_attn(0))
    start([wu_cp])
    wo_cp.wait()
    x_cp(2).wait()
    par(t_wo(0), t_ln(ln1, 2))
    start(mod_cps(5) + [wd_cp] + [x_cp(i) for i in range(3, NT)])
    par(t_qkv(2), t_ln(ln2, 0))
    wg_cp.wait()
    wu_cp.wait()
    first, second = range(NDC // 2), range(NDC // 2, NDC)
    for i in range(1, NT):
        att = t_attn(i)
        par(t_gu, att[:N_GU])
        if i == 1:
            mod_vec(5)
            wd_cp.wait()
        if i + 2 < NT:
            x_cp(i + 2).wait()
        par(t_down(i - 1, first), att[N_GU:])
        par(t_wo(i), t_ln(ln1, i + 2))
        par(t_down(i - 1, second), t_ln(ln2, i))
        if i + 2 < NT:
            par(t_qkv(i + 2), [])
        pass
    par(t_gu, [])
    par(t_down(NT - 1, range(NDC)), [])
    for i in range(NT):
        for n in range(NDC):
            out_cp(i, n).wait()


@jax.jit
def pallas_adaLN_cond__sliding_local_dilated__swiglu_ffn__prompt_kernel(
    A_x: jax.Array,
    A_wqkv: jax.Array,
    A_wo: jax.Array,
    B_x: jax.Array,
    B_w_gate: jax.Array,
    B_w_up: jax.Array,
    B_w_down: jax.Array,
    c: jax.Array,
    w_mod: jax.Array,
):
    del B_x
    x = A_x.reshape(NT, TM, D)
    hbm = pl.BlockSpec(memory_space=pl.ANY)
    out = pl.pallas_call(
        _kernel,
        in_specs=[hbm, pl.BlockSpec(memory_space=pltpu.VMEM), hbm, hbm, hbm, hbm, hbm, hbm],
        out_specs=hbm,
        out_shape=jax.ShapeDtypeStruct((NT, TM, D), A_x.dtype),
        scratch_shapes=[
            pltpu.VMEM((NT, TM, D), BF16),
            pltpu.VMEM((NT, TM, D), BF16),
            pltpu.VMEM((D, 6 * D), BF16),
            pltpu.VMEM((D, 3 * D), BF16),
            pltpu.VMEM((D, D), BF16),
            pltpu.VMEM((D, F), BF16),
            pltpu.VMEM((D, F), BF16),
            pltpu.VMEM((F, D), BF16),
            pltpu.VMEM((8, 6 * D), F32),
            pltpu.VMEM((2, TM, D), BF16),
            pltpu.VMEM((2, NLT, TM, 128), F32),
            pltpu.VMEM((2, NLT, HALO + TM, 128), F32),
            pltpu.VMEM((2, NLT, HALO + TM, 128), F32),
            pltpu.VMEM((TM, D), BF16),
            pltpu.VMEM((2, TM, D), F32),
            pltpu.VMEM((TM, D), BF16),
            pltpu.VMEM((TM, F), BF16),
            pltpu.SemaphoreType.DMA((6 * D // MC + 7,)),
            pltpu.SemaphoreType.DMA((NT,)),
            pltpu.SemaphoreType.DMA((NT * NDC,)),
        ],
        compiler_params=pltpu.CompilerParams(
            vmem_limit_bytes=110 * 1024 * 1024,
        ),
    )(x, c, w_mod, A_wqkv, A_wo, B_w_gate, B_w_up, B_w_down)
    return out.reshape(A_x.shape)
```

```python
import jax
import jax.numpy as jnp
from jax import lax
from jax.experimental import pallas as pl
from jax.experimental.pallas import tpu as pltpu

S, D, F = 2048, 1024, 3584
H, DH, W, DIL = 32, 32, 8, 2
TM = 512
NT = S // TM
HALO = 16
FC = 512
NFC = F // FC
DC = 256
NDC = D // DC
AR = 16
LR = 64
MC = 512
NLT = D // 128
QC = 512
SKEW = 1
N_GU = 120
EPS = 1e-5
SCALE = DH ** -0.5
F32, BF16 = jnp.float32, jnp.bfloat16


def _swap_tiles_lanes(tiles):
    lane = lax.broadcasted_iota(jnp.int32, tiles[0].shape, 1)
    for b in range(3):
        sh = 4 << b
        low = (lane & sh) == 0
        new = list(tiles)
        for t in range(NLT):
            if not (t >> b) & 1:
                a, c = tiles[t], tiles[t | (1 << b)]
                new[t] = jnp.where(low, a, pltpu.roll(c, sh, 1))
                new[t | (1 << b)] = jnp.where(low, pltpu.roll(a, 128 - sh, 1), c)
        tiles = new
    return tiles


def _permute_bf16(val):
    u = pltpu.bitcast(val, jnp.uint32)
    tiles = _swap_tiles_lanes([u[:, t * 128:(t + 1) * 128] for t in range(NLT)])
    return pltpu.bitcast(jnp.concatenate(tiles, axis=1), BF16)


def _ln_mod(x, scale1, shift):
    m = jnp.mean(x, axis=-1, keepdims=True)
    xc = x - m
    v = jnp.mean(xc * xc, axis=-1, keepdims=True)
    return xc * lax.rsqrt(v + EPS) * scale1 + shift


def _kernel(x_hbm, c_ref, wmod_hbm, wqkv_hbm, wo_hbm, wg_hbm, wu_hbm, wd_hbm, out_hbm,
            x_v, out_v, wmod_v, wraw_v, wqkv_v, wo_v, wg_v, wu_v, wd_v, mod_v, h_s, q_s, k_s, v_s, o_s,
            x1_s, h2_s, act_s, sems, xsems, osems):
    n_mod = 6 * D // MC

    def mod_cp(j):
        return pltpu.make_async_copy(wmod_hbm.at[:, pl.ds(j * MC, MC)],
                                     wmod_v.at[:, pl.ds(j * MC, MC)], sems.at[j])

    def qkv_cp(j):
        return pltpu.make_async_copy(wqkv_hbm.at[:, pl.ds(j * D, D)],
                                     wraw_v.at[j], sems.at[n_mod + j])

    def x_cp(i):
        return pltpu.make_async_copy(x_hbm.at[i], x_v.at[i], xsems.at[i])

    def out_cp(i, n):
        cs = pl.ds(n * DC, DC)
        return pltpu.make_async_copy(out_v.at[i, :, cs], out_hbm.at[i, :, cs],
                                     osems.at[i * NDC + n])

    wo_cp = pltpu.make_async_copy(wo_hbm, wo_v, sems.at[n_mod + 3])
    wg_cp = pltpu.make_async_copy(wg_hbm, wg_v, sems.at[n_mod + 4])
    wu_cp = pltpu.make_async_copy(wu_hbm, wu_v, sems.at[n_mod + 5])
    wd_cp = pltpu.make_async_copy(wd_hbm, wd_v, sems.at[n_mod + 6])
    per = D // MC

    def mod_cps(k):
        return [mod_cp(j) for j in range(k * per, (k + 1) * per)]

    def start(cps):
        for cp in cps:
            cp.start()

    def mod_chunk(j):
        mod_cp(j).wait()
        cf = c_ref[...].astype(F32)
        sc = jnp.broadcast_to(cf * jax.nn.sigmoid(cf), (16, D)).astype(BF16)
        r = jnp.dot(sc, wmod_v[:, j * MC:(j + 1) * MC], preferred_element_type=F32)
        if j // per in (1, 4):
            r = r + 1.0
        mod_v[:, j * MC:(j + 1) * MC] = r[0:8]

    def mod_vec(k):
        for j in range(k * per, (k + 1) * per):
            mod_chunk(j)

    def mod(k):
        return mod_v[0:1, k * D:(k + 1) * D]

    def ln1(i, r):
        xv = x_v[i, r:r + LR, :].astype(F32)
        h_s[i % 2, r:r + LR, :] = _ln_mod(xv, mod(1), mod(0)).astype(BF16)

    def qkv_first(j):
        qkv_cp(j).wait()
        wp = _permute_bf16(wraw_v[j])
        wqkv_v[:, j * D:(j + 1) * D] = wp
        h = h_s[0]
        for half in range(D // QC):
            qkv_store(0, j, half, jnp.dot(h, wp[:, half * QC:(half + 1) * QC],
                                          preferred_element_type=F32))

    def qkv_part(i, j, half):
        c0 = j * D + half * QC
        qkv_store(i, j, half, jnp.dot(h_s[i % 2], wqkv_v[:, c0:c0 + QC],
                                      preferred_element_type=F32))

    def qkv_store(i, j, half, res):
        sl = i % 2
        for tt in range(QC // 128):
            t = half * (QC // 128) + tt
            blk = res[:, tt * 128:(tt + 1) * 128]
            if j == 0:
                q_s[sl, t] = blk * SCALE
                continue
            dst = k_s if j == 1 else v_s
            dst[sl, t, HALO:HALO + TM, :] = blk
            if i == 0:
                dst[sl, t, 0:HALO, :] = jnp.broadcast_to(blk[0:1], (HALO, 128))
            if i + 1 < NT:
                dst[1 - sl, t, 0:HALO, :] = blk[TM - HALO:TM]

    live = {}

    def attn_qk(i, r):
        sl = i % 2
        q = [q_s[sl, t, r:r + AR, :] for t in range(NLT)]
        lg = []
        for w in range(W):
            o = HALO + r - DIL * w
            a = q[0] * k_s[sl, 0, o:o + AR, :]
            for t in range(1, NLT):
                a = a + q[t] * k_s[sl, t, o:o + AR, :]
            lg.append(a)
        live[i, r] = lg

    def attn_lanes(i, r):
        lane = lax.broadcasted_iota(jnp.int32, (AR, 128), 1)
        b0 = (lane & 1) == 0
        b1 = (lane & 2) == 0
        lg = [a + jnp.where(b0, pltpu.roll(a, 127, 1), pltpu.roll(a, 1, 1)) for a in live[i, r]]
        lg = [a + jnp.where(b1, pltpu.roll(a, 126, 1), pltpu.roll(a, 2, 1)) for a in lg]
        live[i, r] = lg

    def attn_softmax(i, r):
        lg = live[i, r]
        if i == 0 and r < DIL * (W - 1):
            row = lax.broadcasted_iota(jnp.int32, (AR, 128), 0) + r
            lg = [jnp.where(row >= DIL * w, a, -1000000000.0) for w, a in enumerate(lg)]
        m = lg[0]
        for w in range(1, W):
            m = jnp.maximum(m, lg[w])
        e = [jnp.exp(a - m) for a in lg]
        s = e[0]
        for w in range(1, W):
            s = s + e[w]
        inv = 1.0 / s
        live[i, r] = [a * inv for a in e]

    def attn_pv(i, r):
        sl = i % 2
        p = live.pop((i, r))
        outs = []
        for t in range(NLT):
            a = p[0] * v_s[sl, t, HALO + r:HALO + r + AR, :]
            for w in range(1, W):
                o = HALO + r - DIL * w
                a = a + p[w] * v_s[sl, t, o:o + AR, :]
            outs.append(a)
        o_s[r:r + AR, :] = jnp.concatenate(outs, axis=1).astype(BF16)

    def attn_unpermute(i, r):
        o_s[r:r + AR, :] = _permute_bf16(o_s[r:r + AR, :])

    def wo_part(i, half):
        cs = slice(half * QC, (half + 1) * QC)
        y = jnp.dot(o_s[...], wo_v[:, cs], preferred_element_type=F32)
        ga = mod_v[0:1, 2 * D + half * QC:2 * D + (half + 1) * QC]
        x1_s[i % 2, :, cs] = x_v[i, :, cs].astype(F32) + ga * y

    def ln2(i, r):
        h2_s[r:r + LR, :] = _ln_mod(x1_s[i % 2, r:r + LR, :], mod(4), mod(3)).astype(BF16)

    def gate_up(cix):
        cs = slice(cix * FC, (cix + 1) * FC)
        h2 = h2_s[...]
        g = jnp.dot(h2, wg_v[:, cs], preferred_element_type=F32)
        u = jnp.dot(h2, wu_v[:, cs], preferred_element_type=F32)
        t = 0.5 * g
        act_s[:, cs] = ((t + t * jnp.tanh(t)) * u).astype(BF16)

    def down(i, n):
        cs = slice(n * DC, (n + 1) * DC)
        y = jnp.dot(act_s[...], wd_v[:, cs], preferred_element_type=F32)
        gb = mod_v[0:1, 5 * D + n * DC:5 * D + (n + 1) * DC]
        out_v[i, :, cs] = (x1_s[i % 2, :, cs] + gb * y).astype(out_v.dtype)
        out_cp(i, n).start()

    def par(mxu, vpu):
        done = 0
        for idx, (fn, *args) in enumerate(mxu):
            fn(*args)
            upto = len(vpu) * (idx + 1) // len(mxu)
            for vfn, *vargs in vpu[done:upto]:
                vfn(*vargs)
            done = upto

    halves = range(D // QC)

    def t_qkv(i, js=(0, 1, 2)):
        return [(qkv_part, i, j, hf) for j in js for hf in halves]

    def t_attn(i):
        stages = (attn_qk, attn_lanes, attn_softmax, attn_pv, attn_unpermute)
        nb = TM // AR
        return [(fn, i, (n - k * SKEW) * AR) for n in range(nb + (len(stages) - 1) * SKEW)
                for k, fn in reversed(list(enumerate(stages))) if 0 <= n - k * SKEW < nb]

    def t_ln(fn, i):
        return [(fn, i, r) for r in range(0, TM, LR)] if i < NT else []

    def t_wo(i):
        return [(wo_part, i, hf) for hf in halves]

    t_gu = [(gate_up, cix) for cix in range(NFC)]

    def t_down(i, ns):
        return [(down, i, n) for n in ns]

    start([x_cp(0)] + mod_cps(0) + mod_cps(1))
    mod_vec(0)
    start([qkv_cp(0)])
    x_cp(0).wait()
    mod_vec(1)
    start([qkv_cp(1)])
    par(t_ln(ln1, 0), [])
    start([qkv_cp(2), x_cp(1)])
    qkv_first(0)
    start(mod_cps(2) + [wo_cp])
    qkv_first(1)
    start(mod_cps(3) + mod_cps(4) + [x_cp(2)])
    x_cp(1).wait()
    par([(qkv_first, 2)], t_ln(ln1, 1))
    start([wg_cp])
    par(t_qkv(1) + [(mod_vec, 2), (mod_vec, 3), (mod_vec, 4)], t_attn(0))
    start([wu_cp])
    wo_cp.wait()
    x_cp(2).wait()
    par(t_wo(0), t_ln(ln1, 2))
    start(mod_cps(5) + [wd_cp] + [x_cp(i) for i in range(3, NT)])
    par(t_qkv(2), t_ln(ln2, 0))
    wg_cp.wait()
    wu_cp.wait()
    first, second = range(NDC // 2), range(NDC // 2, NDC)
    for i in range(1, NT):
        att = t_attn(i)
        par(t_gu, att[:N_GU])
        if i == 1:
            mod_vec(5)
            wd_cp.wait()
        if i + 2 < NT:
            x_cp(i + 2).wait()
        par(t_down(i - 1, first), att[N_GU:])
        par(t_wo(i), t_ln(ln1, i + 2))
        par(t_down(i - 1, second), t_ln(ln2, i))
        if i + 2 < NT:
            par(t_qkv(i + 2), [])
        pass
    par(t_gu, [])
    par(t_down(NT - 1, range(NDC)), [])
    for i in range(NT):
        for n in range(NDC):
            out_cp(i, n).wait()


@jax.jit
def pallas_adaLN_cond__sliding_local_dilated__swiglu_ffn__prompt_kernel(
    A_x: jax.Array,
    A_wqkv: jax.Array,
    A_wo: jax.Array,
    B_x: jax.Array,
    B_w_gate: jax.Array,
    B_w_up: jax.Array,
    B_w_down: jax.Array,
    c: jax.Array,
    w_mod: jax.Array,
):
    del B_x
    x = A_x.reshape(NT, TM, D)
    hbm = pl.BlockSpec(memory_space=pl.ANY)
    out = pl.pallas_call(
        _kernel,
        in_specs=[hbm, pl.BlockSpec(memory_space=pltpu.VMEM), hbm, hbm, hbm, hbm, hbm, hbm],
        out_specs=hbm,
        out_shape=jax.ShapeDtypeStruct((NT, TM, D), A_x.dtype),
        scratch_shapes=[
            pltpu.VMEM((NT, TM, D), BF16),
            pltpu.VMEM((NT, TM, D), BF16),
            pltpu.VMEM((D, 6 * D), BF16),
            pltpu.VMEM((3, D, D), BF16),
            pltpu.VMEM((D, 3 * D), BF16),
            pltpu.VMEM((D, D), BF16),
            pltpu.VMEM((D, F), BF16),
            pltpu.VMEM((D, F), BF16),
            pltpu.VMEM((F, D), BF16),
            pltpu.VMEM((8, 6 * D), F32),
            pltpu.VMEM((2, TM, D), BF16),
            pltpu.VMEM((2, NLT, TM, 128), F32),
            pltpu.VMEM((2, NLT, HALO + TM, 128), F32),
            pltpu.VMEM((2, NLT, HALO + TM, 128), F32),
            pltpu.VMEM((TM, D), BF16),
            pltpu.VMEM((2, TM, D), F32),
            pltpu.VMEM((TM, D), BF16),
            pltpu.VMEM((TM, F), BF16),
            pltpu.SemaphoreType.DMA((6 * D // MC + 7,)),
            pltpu.SemaphoreType.DMA((NT,)),
            pltpu.SemaphoreType.DMA((NT * NDC,)),
        ],
        compiler_params=pltpu.CompilerParams(
            vmem_limit_bytes=110 * 1024 * 1024,
        ),
    )(x, c, w_mod, A_wqkv, A_wo, B_w_gate, B_w_up, B_w_down)
    return out.reshape(A_x.shape)
```

```python
import jax
import jax.numpy as jnp
import numpy as np
from jax import lax
from jax.experimental import pallas as pl
from jax.experimental.pallas import tpu as pltpu

S, D, F = 2048, 1024, 3584
H, DH, W, DIL = 32, 32, 8, 2
TM = 512
NT = S // TM
HALO = 16
FC = 512
NFC = F // FC
DC = 256
NDC = D // DC
AR = 16
LR = 64
MC = 512
NLT = D // 128
QC = 512
SKEW = 1
N_GU = 160
EPS = 1e-5
SCALE = DH ** -0.5
F32, BF16 = jnp.float32, jnp.bfloat16


def _swap_tiles_lanes(tiles):
    lane = lax.broadcasted_iota(jnp.int32, tiles[0].shape, 1)
    for b in range(3):
        sh = 4 << b
        low = (lane & sh) == 0
        new = list(tiles)
        for t in range(NLT):
            if not (t >> b) & 1:
                a, c = tiles[t], tiles[t | (1 << b)]
                new[t] = jnp.where(low, a, pltpu.roll(c, sh, 1))
                new[t | (1 << b)] = jnp.where(low, pltpu.roll(a, 128 - sh, 1), c)
        tiles = new
    return tiles


def _permute_bf16(val):
    u = pltpu.bitcast(val, jnp.uint32)
    tiles = _swap_tiles_lanes([u[:, t * 128:(t + 1) * 128] for t in range(NLT)])
    return pltpu.bitcast(jnp.concatenate(tiles, axis=1), BF16)


def _ln_mod(x, scale1, shift):
    m = jnp.mean(x, axis=-1, keepdims=True)
    xc = x - m
    v = jnp.mean(xc * xc, axis=-1, keepdims=True)
    return xc * lax.rsqrt(v + EPS) * scale1 + shift


def _kernel(zero_ref, x_hbm, c_ref, wmod_hbm, wqkv_hbm, wo_hbm, wg_hbm, wu_hbm, wd_hbm, out_hbm,
            x_v, out_v, wmod_v, wraw_v, wqkv_v, wo_v, wg_v, wu_v, wd_v, mod_v, scb_s, h_s, q_s, k_s, v_s, o_s,
            x1_s, h2_s, act_s, sems, xsems, osems):
    n_mod = 6 * D // MC

    def mod_cp(j):
        return pltpu.make_async_copy(wmod_hbm.at[:, pl.ds(j * MC, MC)],
                                     wmod_v.at[:, pl.ds(j * MC, MC)], sems.at[j])

    def qkv_cp(j):
        return pltpu.make_async_copy(wqkv_hbm.at[:, pl.ds(j * D, D)],
                                     wraw_v.at[j], sems.at[n_mod + j])

    def x_cp(i):
        return pltpu.make_async_copy(x_hbm.at[i], x_v.at[i], xsems.at[i])

    def out_cp(i, n):
        cs = pl.ds(n * DC, DC)
        return pltpu.make_async_copy(out_v.at[i, :, cs], out_hbm.at[i, :, cs],
                                     osems.at[i * NDC + n])

    wo_cp = pltpu.make_async_copy(wo_hbm, wo_v, sems.at[n_mod + 3])
    wg_cp = pltpu.make_async_copy(wg_hbm, wg_v, sems.at[n_mod + 4])
    wu_cp = pltpu.make_async_copy(wu_hbm, wu_v, sems.at[n_mod + 5])
    wd_cp = pltpu.make_async_copy(wd_hbm, wd_v, sems.at[n_mod + 6])
    per = D // MC

    def mod_cps(k):
        return [mod_cp(j) for j in range(k * per, (k + 1) * per)]

    def start(cps):
        for cp in cps:
            cp.start()

    def mod_chunk(j):
        mod_cp(j).wait()
        cf = c_ref[...].astype(F32)
        sc = jnp.broadcast_to(cf * jax.nn.sigmoid(cf), (16, D)).astype(BF16)
        r = jnp.dot(sc, wmod_v[:, j * MC:(j + 1) * MC], preferred_element_type=F32)
        if j // per in (1, 4):
            r = r + 1.0
        mod_v[:, j * MC:(j + 1) * MC] = r[0:8]

    def mod_vec(k):
        for j in range(k * per, (k + 1) * per):
            mod_chunk(j)

    def silu_c_columns():
        cf = c_ref[...].astype(F32)
        sc = (cf * jax.nn.sigmoid(cf)).astype(BF16).astype(F32)
        for t in range(NLT):
            blk = jnp.broadcast_to(sc[:, t * 128:(t + 1) * 128], (128, 128))
            scb_s[t * 128:(t + 1) * 128, :] = blk.T

    def mod_tile_vpu(n):
        cs = slice(n * 128, (n + 1) * 128)
        acc = paced(jnp.zeros((AR, 128), F32))
        for r in range(0, D, AR):
            acc = acc + wmod_v[r:r + AR, cs].astype(F32) * scb_s[r:r + AR, :]
        res = jnp.sum(acc, axis=0, keepdims=True)
        if n // NLT in (1, 4):
            res = res + 1.0
        mod_v[:, cs] = jnp.broadcast_to(res, (8, 128))

    tokens = []

    def paced(val):
        if not tokens:
            return val
        never = lax.broadcasted_iota(jnp.int32, val.shape, 0) < zero_ref[0]
        return jnp.where(never, tokens.pop(0), val)

    def post(*results):
        tokens[:] = [res[TM - AR:TM, c:c + 128] for res in results
                     for c in range(0, res.shape[1], 256)]

    def mod(k):
        return mod_v[0:1, k * D:(k + 1) * D]

    def ln1(i, r):
        xv = x_v[i, r:r + LR, :].astype(F32)
        h_s[i % 2, r:r + LR, :] = _ln_mod(xv, mod(1), mod(0)).astype(BF16)

    def prep_qkv(j, r):
        wqkv_v[r:r + 128, j * D:(j + 1) * D] = _permute_bf16(wraw_v[j, r:r + 128, :])

    def qkv_part(i, j, half):
        c0 = j * D + half * QC
        res = jnp.dot(h_s[i % 2], wqkv_v[:, c0:c0 + QC], preferred_element_type=F32)
        qkv_store(i, j, half, res)
        post(res)

    def qkv_store(i, j, half, res):
        sl = i % 2
        for tt in range(QC // 128):
            t = half * (QC // 128) + tt
            blk = res[:, tt * 128:(tt + 1) * 128]
            if j == 0:
                q_s[sl, t] = blk * SCALE
                continue
            dst = k_s if j == 1 else v_s
            dst[sl, t, HALO:HALO + TM, :] = blk
            if i == 0:
                dst[sl, t, 0:HALO, :] = jnp.broadcast_to(blk[0:1], (HALO, 128))
            else:
                dst[sl, t, 0:HALO, :] = dst[1 - sl, t, TM:TM + HALO, :]

    live = {}

    def attn_qk(i, r):
        sl = i % 2
        q = [q_s[sl, t, r:r + AR, :] for t in range(NLT)]
        q[0] = paced(q[0])
        lg = []
        for w in range(W):
            o = HALO + r - DIL * w
            a = q[0] * k_s[sl, 0, o:o + AR, :]
            for t in range(1, NLT):
                a = a + q[t] * k_s[sl, t, o:o + AR, :]
            lg.append(a)
        live[i, r] = lg

    def attn_lanes(i, r):
        lane = lax.broadcasted_iota(jnp.int32, (AR, 128), 1)
        b0 = (lane & 1) == 0
        b1 = (lane & 2) == 0
        lg = [a + jnp.where(b0, pltpu.roll(a, 127, 1), pltpu.roll(a, 1, 1)) for a in live[i, r]]
        lg = [a + jnp.where(b1, pltpu.roll(a, 126, 1), pltpu.roll(a, 2, 1)) for a in lg]
        live[i, r] = lg

    def attn_softmax(i, r):
        lg = live[i, r]
        if i == 0 and r < DIL * (W - 1):
            row = lax.broadcasted_iota(jnp.int32, (AR, 128), 0) + r
            lg = [jnp.where(row >= DIL * w, a, -1000000000.0) for w, a in enumerate(lg)]
        m = lg[0]
        for w in range(1, W):
            m = jnp.maximum(m, lg[w])
        e = [jnp.exp(a - m) for a in lg]
        s = e[0]
        for w in range(1, W):
            s = s + e[w]
        inv = 1.0 / s
        live[i, r] = [a * inv for a in e]

    def attn_pv(i, r):
        sl = i % 2
        p = live.pop((i, r))
        outs = []
        for t in range(NLT):
            a = p[0] * v_s[sl, t, HALO + r:HALO + r + AR, :]
            for w in range(1, W):
                o = HALO + r - DIL * w
                a = a + p[w] * v_s[sl, t, o:o + AR, :]
            outs.append(a)
        o_s[r:r + AR, :] = jnp.concatenate(outs, axis=1).astype(BF16)

    def attn_unpermute(i, r):
        o_s[r:r + AR, :] = _permute_bf16(o_s[r:r + AR, :])

    def wo_part(i, half):
        cs = slice(half * QC, (half + 1) * QC)
        y = jnp.dot(o_s[...], wo_v[:, cs], preferred_element_type=F32)
        ga = mod_v[0:1, 2 * D + half * QC:2 * D + (half + 1) * QC]
        x1_s[i % 2, :, cs] = x_v[i, :, cs].astype(F32) + ga * y

    def ln2(i, r):
        h2_s[r:r + LR, :] = _ln_mod(x1_s[i % 2, r:r + LR, :], mod(4), mod(3)).astype(BF16)

    def gate_up(cix):
        cs = slice(cix * FC, (cix + 1) * FC)
        h2 = h2_s[...]
        g = jnp.dot(h2, wg_v[:, cs], preferred_element_type=F32)
        u = jnp.dot(h2, wu_v[:, cs], preferred_element_type=F32)
        post(g, u)
        t = 0.5 * g
        act_s[:, cs] = ((t + t * jnp.tanh(t)) * u).astype(BF16)

    def down(i, n):
        cs = slice(n * DC, (n + 1) * DC)
        y = jnp.dot(act_s[...], wd_v[:, cs], preferred_element_type=F32)
        gb = mod_v[0:1, 5 * D + n * DC:5 * D + (n + 1) * DC]
        out_v[i, :, cs] = (x1_s[i % 2, :, cs] + gb * y).astype(out_v.dtype)
        out_cp(i, n).start()

    def par(mxu, vpu):
        done = 0
        for idx, (fn, *args) in enumerate(mxu):
            upto = len(vpu) * (idx + 1) // len(mxu)
            for vfn, *vargs in vpu[done:upto]:
                vfn(*vargs)
            done = upto
            fn(*args)

    halves = range(D // QC)

    def t_qkv(i, js=(0, 1, 2)):
        return [(qkv_part, i, j, hf) for j in js for hf in halves]

    def t_attn(i):
        stages = (attn_qk, attn_lanes, attn_softmax, attn_pv, attn_unpermute)
        nb = TM // AR
        return [(fn, i, (n - k * SKEW) * AR) for n in range(nb + (len(stages) - 1) * SKEW)
                for k, fn in reversed(list(enumerate(stages))) if 0 <= n - k * SKEW < nb]

    def t_ln(fn, i):
        return [(fn, i, r) for r in range(0, TM, LR)] if i < NT else []

    def t_wo(i):
        return [(wo_part, i, hf) for hf in halves]

    t_gu = [(gate_up, cix) for cix in range(NFC)]

    def t_down(i, ns):
        return [(down, i, n) for n in ns]

    def t_prep(j):
        return [(prep_qkv, j, r) for r in range(0, D, 128)]

    def t_mod(ks):
        return [(mod_tile_vpu, n) for k in ks for n in range(k * NLT, (k + 1) * NLT)]

    def wait(cps):
        for cp in cps:
            cp.wait()

    start([qkv_cp(0), x_cp(0)] + mod_cps(0))
    silu_c_columns()
    qkv_cp(0).wait()
    start(mod_cps(1))
    par(t_prep(0), [])
    mod_vec(0)
    start([qkv_cp(1)])
    x_cp(0).wait()
    mod_vec(1)
    start([qkv_cp(2), x_cp(1)])
    par(t_ln(ln1, 0), [])
    q0 = t_qkv(0)
    nh = len(halves)
    par(q0[:nh // 2], [])
    qkv_cp(1).wait()
    start([x_cp(2)] + mod_cps(2))
    par(q0[nh // 2:nh], t_prep(1))
    qkv_cp(2).wait()
    start([wo_cp] + mod_cps(3))
    par(q0[nh:2 * nh], t_prep(2))
    x_cp(1).wait()
    start(mod_cps(4) + mod_cps(5))
    par(q0[2 * nh:], t_ln(ln1, 1))
    start([wg_cp])
    x_cp(2).wait()
    par(t_qkv(1), t_attn(0) + t_ln(ln1, 2))
    start([wu_cp])
    wait(mod_cps(2) + mod_cps(3) + mod_cps(4) + mod_cps(5))
    par(t_qkv(2, (0, 1)), t_mod((2, 3, 4, 5)))
    start([wd_cp] + [x_cp(i) for i in range(3, NT)])
    wo_cp.wait()
    par(t_wo(0), [])
    par(t_qkv(2, (2,)), t_ln(ln2, 0))
    wait([wg_cp, wu_cp])
    first, second = range(NDC // 2), range(NDC // 2, NDC)
    for i in range(1, NT):
        att = t_attn(i)
        par(t_gu, att[:N_GU])
        if i == 1:
            wd_cp.wait()
        if i + 2 < NT:
            x_cp(i + 2).wait()
        par(t_down(i - 1, first), att[N_GU:])
        par(t_wo(i), t_ln(ln1, i + 2))
        par(t_down(i - 1, second), t_ln(ln2, i))
        if i + 2 < NT:
            par(t_qkv(i + 2), [])
        pass
    par(t_gu, [])
    par(t_down(NT - 1, range(NDC)), [])
    for i in range(NT):
        for n in range(NDC):
            out_cp(i, n).wait()


@jax.jit
def pallas_adaLN_cond__sliding_local_dilated__swiglu_ffn__prompt_kernel(
    A_x: jax.Array,
    A_wqkv: jax.Array,
    A_wo: jax.Array,
    B_x: jax.Array,
    B_w_gate: jax.Array,
    B_w_up: jax.Array,
    B_w_down: jax.Array,
    c: jax.Array,
    w_mod: jax.Array,
):
    del B_x
    x = A_x.reshape(NT, TM, D)
    hbm = pl.BlockSpec(memory_space=pl.ANY)
    out = pl.pallas_call(
        _kernel,
        in_specs=[pl.BlockSpec(memory_space=pltpu.SMEM), hbm, pl.BlockSpec(memory_space=pltpu.VMEM), hbm, hbm, hbm, hbm, hbm, hbm],
        out_specs=hbm,
        out_shape=jax.ShapeDtypeStruct((NT, TM, D), A_x.dtype),
        scratch_shapes=[
            pltpu.VMEM((NT, TM, D), BF16),
            pltpu.VMEM((NT, TM, D), BF16),
            pltpu.VMEM((D, 6 * D), BF16),
            pltpu.VMEM((3, D, D), BF16),
            pltpu.VMEM((D, 3 * D), BF16),
            pltpu.VMEM((D, D), BF16),
            pltpu.VMEM((D, F), BF16),
            pltpu.VMEM((D, F), BF16),
            pltpu.VMEM((F, D), BF16),
            pltpu.VMEM((8, 6 * D), F32),
            pltpu.VMEM((D, 128), F32),
            pltpu.VMEM((2, TM, D), BF16),
            pltpu.VMEM((2, NLT, TM, 128), F32),
            pltpu.VMEM((2, NLT, HALO + TM, 128), F32),
            pltpu.VMEM((2, NLT, HALO + TM, 128), F32),
            pltpu.VMEM((TM, D), BF16),
            pltpu.VMEM((2, TM, D), F32),
            pltpu.VMEM((TM, D), BF16),
            pltpu.VMEM((TM, F), BF16),
            pltpu.SemaphoreType.DMA((6 * D // MC + 7,)),
            pltpu.SemaphoreType.DMA((NT,)),
            pltpu.SemaphoreType.DMA((NT * NDC,)),
        ],
        compiler_params=pltpu.CompilerParams(
            vmem_limit_bytes=110 * 1024 * 1024,
        ),
    )(np.zeros((1,), np.int32), x, c, w_mod, A_wqkv, A_wo, B_w_gate, B_w_up, B_w_down)
    return out.reshape(A_x.shape)
```

```python
import jax
import jax.numpy as jnp
import numpy as np
from jax import lax
from jax.experimental import pallas as pl
from jax.experimental.pallas import tpu as pltpu

S, D, F = 2048, 1024, 3584
H, DH, W, DIL = 32, 32, 8, 2
TM = 512
NT = S // TM
HALO = 16
FC = 512
NFC = F // FC
DC = 256
NDC = D // DC
AR = 16
LR = 64
MC = 512
NLT = D // 128
QC = 512
WQR = 256
SKEW = 1
N_GU = 160
EPS = 1e-5
LOG2E = 1.4426950408889634
SCALE = DH ** -0.5 * LOG2E
F32, BF16, U32 = jnp.float32, jnp.bfloat16, jnp.uint32


def _swap_tiles_lanes(tiles):
    lane = lax.broadcasted_iota(jnp.int32, tiles[0].shape, 1)
    for b in range(3):
        sh = 4 << b
        low = (lane & sh) == 0
        new = list(tiles)
        for t in range(NLT):
            if not (t >> b) & 1:
                a, c = tiles[t], tiles[t | (1 << b)]
                new[t] = jnp.where(low, a, pltpu.roll(c, sh, 1))
                new[t | (1 << b)] = jnp.where(low, pltpu.roll(a, 128 - sh, 1), c)
        tiles = new
    return tiles


def _permute_cols(u):
    tiles = _swap_tiles_lanes([u[:, t * 128:(t + 1) * 128] for t in range(NLT)])
    return jnp.concatenate(tiles, axis=1)


def _pack(val):
    return pltpu.bitcast(val.astype(BF16), U32)


def _unpack(u):
    return pltpu.bitcast(u, BF16)


def _ln_mod(x, scale1, shift):
    m = jnp.mean(x, axis=-1, keepdims=True)
    xc = x - m
    v = jnp.mean(xc * xc, axis=-1, keepdims=True)
    return xc * lax.rsqrt(v + EPS) * scale1 + shift


def _kernel(zero_ref, x_hbm, c_ref, wmod_hbm, wqkv_hbm, wo_hbm, wg_hbm, wu_hbm, wd_hbm, out_hbm,
            x_v, out_v, wmod_v, wraw_v, wqkv_v, wo_v, wg_v, wu_v, wd_v, mod_v, scb_s, h_s, q_s, k_s, v_s, o_s,
            x1_s, h2_s, act_s, sems, qsems, xsems, osems):
    n_mod = 6 * D // MC

    def mod_cp(j):
        return pltpu.make_async_copy(wmod_hbm.at[:, pl.ds(j * MC, MC)],
                                     wmod_v.at[:, pl.ds(j * MC, MC)], sems.at[j])

    def qkv_cp(j):
        return pltpu.make_async_copy(wqkv_hbm.at[:, pl.ds(j * D, D)],
                                     wraw_v.at[j], sems.at[n_mod + j])

    def wq_cp(n):
        rows = pl.ds(n * WQR, WQR)
        return pltpu.make_async_copy(wqkv_hbm.at[rows, pl.ds(0, D)], wraw_v.at[0, rows, :],
                                     qsems.at[n])

    def x_cp(i):
        return pltpu.make_async_copy(x_hbm.at[i], x_v.at[i], xsems.at[i])

    def out_cp(i, n):
        cs = pl.ds(n * DC, DC)
        return pltpu.make_async_copy(out_v.at[i, :, cs], out_hbm.at[i, :, cs],
                                     osems.at[i * NDC + n])

    wo_cp = pltpu.make_async_copy(wo_hbm, wo_v, sems.at[n_mod + 3])
    wg_cp = pltpu.make_async_copy(wg_hbm, wg_v, sems.at[n_mod + 4])
    wu_cp = pltpu.make_async_copy(wu_hbm, wu_v, sems.at[n_mod + 5])
    wd_cp = pltpu.make_async_copy(wd_hbm, wd_v, sems.at[n_mod + 6])
    per = D // MC

    def mod_cps(k):
        return [mod_cp(j) for j in range(k * per, (k + 1) * per)]

    def start(cps):
        for cp in cps:
            cp.start()

    def mod_chunk(j):
        mod_cp(j).wait()
        cf = c_ref[...].astype(F32)
        sc = jnp.broadcast_to(cf * jax.nn.sigmoid(cf), (16, D)).astype(BF16)
        r = jnp.dot(sc, wmod_v[:, j * MC:(j + 1) * MC], preferred_element_type=F32)
        if j // per in (1, 4):
            r = r + 1.0
        mod_v[:, j * MC:(j + 1) * MC] = r[0:8]

    def mod_vec(k):
        for j in range(k * per, (k + 1) * per):
            mod_chunk(j)

    def silu_c_columns():
        cf = c_ref[...].astype(F32)
        sc = (cf * jax.nn.sigmoid(cf)).astype(BF16).astype(F32)
        for t in range(NLT):
            blk = jnp.broadcast_to(sc[:, t * 128:(t + 1) * 128], (128, 128))
            scb_s[t * 128:(t + 1) * 128, :] = blk.T

    def mod_tile_vpu(n):
        cs = slice(n * 128, (n + 1) * 128)
        acc = paced(jnp.zeros((AR, 128), F32))
        for r in range(0, D, AR):
            acc = acc + wmod_v[r:r + AR, cs].astype(F32) * scb_s[r:r + AR, :]
        res = jnp.sum(acc, axis=0, keepdims=True)
        if n // NLT in (1, 4):
            res = res + 1.0
        mod_v[:, cs] = jnp.broadcast_to(res, (8, 128))

    tokens = []

    def paced(val):
        if not tokens:
            return val
        never = lax.broadcasted_iota(jnp.int32, val.shape, 0) < zero_ref[0]
        return jnp.where(never, tokens.pop(0), val)

    def post(*results):
        tokens[:] = [res[TM - AR:TM, c:c + 128] for res in results
                     for c in range(0, res.shape[1], 256)]

    def mod(k):
        return mod_v[0:1, k * D:(k + 1) * D]

    def ln1(i, r):
        xv = x_v[i, r:r + LR, :].astype(F32)
        h_s[i % 2, r // 2:(r + LR) // 2, :] = _pack(_ln_mod(xv, mod(1), mod(0)))

    def prep_qkv(j, r):
        wqkv_v[r // 2:r // 2 + 64, j * D:(j + 1) * D] = _permute_cols(
            _pack(wraw_v[j, r:r + 128, :]))

    def qkv_part(i, j, half):
        c0 = j * D + half * QC
        res = jnp.dot(_unpack(h_s[i % 2]), _unpack(wqkv_v[:, c0:c0 + QC]),
                      preferred_element_type=F32)
        qkv_store(i, j, half, res)
        post(res)

    def qkv_store(i, j, half, res):
        sl = i % 2
        for tt in range(QC // 128):
            t = half * (QC // 128) + tt
            blk = res[:, tt * 128:(tt + 1) * 128]
            if j == 0:
                q_s[sl, t] = blk * SCALE
                continue
            dst = k_s if j == 1 else v_s
            dst[sl, t, HALO:HALO + TM, :] = blk
            if i == 0:
                dst[sl, t, 0:HALO, :] = jnp.broadcast_to(blk[0:1], (HALO, 128))
            else:
                dst[sl, t, 0:HALO, :] = dst[1 - sl, t, TM:TM + HALO, :]

    live = {}

    def attn_qk(i, r):
        sl = i % 2
        q = [q_s[sl, t, r:r + AR, :] for t in range(NLT)]
        q[0] = paced(q[0])
        lg = []
        for w in range(W):
            o = HALO + r - DIL * w
            a = q[0] * k_s[sl, 0, o:o + AR, :]
            for t in range(1, NLT):
                a = a + q[t] * k_s[sl, t, o:o + AR, :]
            lg.append(a)
        live[i, r] = lg

    def attn_lanes(i, r):
        lane = lax.broadcasted_iota(jnp.int32, (AR, 128), 1)
        b0 = (lane & 1) == 0
        b1 = (lane & 2) == 0
        lg = [a + jnp.where(b0, pltpu.roll(a, 127, 1), pltpu.roll(a, 1, 1)) for a in live[i, r]]
        lg = [a + jnp.where(b1, pltpu.roll(a, 126, 1), pltpu.roll(a, 2, 1)) for a in lg]
        live[i, r] = lg

    def attn_softmax(i, r):
        lg = live[i, r]
        if i == 0 and r < DIL * (W - 1):
            row = lax.broadcasted_iota(jnp.int32, (AR, 128), 0) + r
            lg = [jnp.where(row >= DIL * w, a, -1000000000.0 * LOG2E) for w, a in enumerate(lg)]
        m = lg[0]
        for w in range(1, W):
            m = jnp.maximum(m, lg[w])
        e = [jnp.exp2(a - m) for a in lg]
        s = e[0]
        for w in range(1, W):
            s = s + e[w]
        inv = 1.0 / s
        live[i, r] = [a * inv for a in e]

    def attn_pv(i, r):
        sl = i % 2
        p = live.pop((i, r))
        outs = []
        for t in range(NLT):
            a = p[0] * v_s[sl, t, HALO + r:HALO + r + AR, :]
            for w in range(1, W):
                o = HALO + r - DIL * w
                a = a + p[w] * v_s[sl, t, o:o + AR, :]
            outs.append(a)
        o_s[r // 2:(r + AR) // 2, :] = _pack(jnp.concatenate(outs, axis=1))

    def attn_unpermute(i, r):
        rows = slice(r // 2, (r + AR) // 2)
        o_s[rows, :] = _permute_cols(o_s[rows, :])

    def wo_part(i, half):
        cs = slice(half * QC, (half + 1) * QC)
        y = jnp.dot(_unpack(o_s[...]), wo_v[:, cs], preferred_element_type=F32)
        ga = mod_v[0:1, 2 * D + half * QC:2 * D + (half + 1) * QC]
        x1_s[i % 2, :, cs] = x_v[i, :, cs].astype(F32) + ga * y

    def ln2(i, r):
        h2_s[r // 2:(r + LR) // 2, :] = _pack(_ln_mod(x1_s[i % 2, r:r + LR, :], mod(4), mod(3)))

    def gate_up(cix):
        cs = slice(cix * FC, (cix + 1) * FC)
        h2 = _unpack(h2_s[...])
        g = jnp.dot(h2, wg_v[:, cs], preferred_element_type=F32)
        u = jnp.dot(h2, wu_v[:, cs], preferred_element_type=F32)
        post(g, u)
        t = 0.5 * g
        act_s[:, cs] = _pack((t + t * jnp.tanh(t)) * u)

    def down(i, n):
        cs = slice(n * DC, (n + 1) * DC)
        y = jnp.dot(_unpack(act_s[...]), wd_v[:, cs], preferred_element_type=F32)
        gb = mod_v[0:1, 5 * D + n * DC:5 * D + (n + 1) * DC]
        out_v[i, :, cs] = (x1_s[i % 2, :, cs] + gb * y).astype(out_v.dtype)
        out_cp(i, n).start()

    def par(mxu, vpu):
        done = 0
        for idx, (fn, *args) in enumerate(mxu):
            upto = len(vpu) * (idx + 1) // len(mxu)
            for vfn, *vargs in vpu[done:upto]:
                vfn(*vargs)
            done = upto
            fn(*args)

    halves = range(D // QC)

    def t_qkv(i, js=(0, 1, 2)):
        return [(qkv_part, i, j, hf) for j in js for hf in halves]

    def t_attn(i):
        stages = (attn_qk, attn_lanes, attn_softmax, attn_pv, attn_unpermute)
        nb = TM // AR
        return [(fn, i, (n - k * SKEW) * AR) for n in range(nb + (len(stages) - 1) * SKEW)
                for k, fn in reversed(list(enumerate(stages))) if 0 <= n - k * SKEW < nb]

    def t_ln(fn, i):
        return [(fn, i, r) for r in range(0, TM, LR)] if i < NT else []

    def t_wo(i):
        return [(wo_part, i, hf) for hf in halves]

    t_gu = [(gate_up, cix) for cix in range(NFC)]

    def t_down(i, ns):
        return [(down, i, n) for n in ns]

    def t_prep(j):
        return [(prep_qkv, j, r) for r in range(0, D, 128)]

    def t_mod(ks):
        return [(mod_tile_vpu, n) for k in ks for n in range(k * NLT, (k + 1) * NLT)]

    def wait(cps):
        for cp in cps:
            cp.wait()

    start(mod_cps(0) + mod_cps(1) + [x_cp(0)])
    silu_c_columns()
    n_wq = D // WQR
    todo = [wq_cp(n) for n in range(n_wq)] + [qkv_cp(1)]
    for j in range(2 * per):
        mod_chunk(j)
        start(todo[j * 2 // per:(j + 1) * 2 // per])
    x_cp(0).wait()
    par(t_ln(ln1, 0), [])
    start(todo[4:])
    for n in range(n_wq):
        wq_cp(n).wait()
        par([(prep_qkv, 0, r) for r in range(n * WQR, (n + 1) * WQR, 128)], [])
    start([qkv_cp(2), x_cp(1)])
    q0 = t_qkv(0)
    nh = len(halves)
    par(q0[:nh // 2], [])
    qkv_cp(1).wait()
    start([x_cp(2)] + mod_cps(2))
    par(q0[nh // 2:nh], t_prep(1))
    qkv_cp(2).wait()
    start([wo_cp] + mod_cps(3))
    par(q0[nh:2 * nh], t_prep(2))
    x_cp(1).wait()
    start(mod_cps(4) + mod_cps(5))
    par(q0[2 * nh:], t_ln(ln1, 1))
    start([wg_cp])
    x_cp(2).wait()
    par(t_qkv(1), t_attn(0) + t_ln(ln1, 2))
    start([wu_cp])
    wait(mod_cps(2) + mod_cps(3) + mod_cps(4) + mod_cps(5))
    par(t_qkv(2, (0, 1)), t_mod((2, 3, 4, 5)))
    start([wd_cp] + [x_cp(i) for i in range(3, NT)])
    wo_cp.wait()
    par(t_wo(0), [])
    par(t_qkv(2, (2,)), t_ln(ln2, 0))
    wait([wg_cp, wu_cp])
    first, second = range(NDC // 2), range(NDC // 2, NDC)
    for i in range(1, NT):
        att = t_attn(i)
        par(t_gu, att[:N_GU])
        if i == 1:
            wd_cp.wait()
        if i + 2 < NT:
            x_cp(i + 2).wait()
        par(t_down(i - 1, first), att[N_GU:])
        par(t_wo(i), t_ln(ln1, i + 2))
        par(t_down(i - 1, second), t_ln(ln2, i))
        if i + 2 < NT:
            par(t_qkv(i + 2), [])
        pass
    par(t_gu, [])
    par(t_down(NT - 1, range(NDC)), [])
    for i in range(NT):
        for n in range(NDC):
            out_cp(i, n).wait()


@jax.jit
def pallas_adaLN_cond__sliding_local_dilated__swiglu_ffn__prompt_kernel(
    A_x: jax.Array,
    A_wqkv: jax.Array,
    A_wo: jax.Array,
    B_x: jax.Array,
    B_w_gate: jax.Array,
    B_w_up: jax.Array,
    B_w_down: jax.Array,
    c: jax.Array,
    w_mod: jax.Array,
):
    del B_x
    x = A_x.reshape(NT, TM, D)
    hbm = pl.BlockSpec(memory_space=pl.ANY)
    out = pl.pallas_call(
        _kernel,
        in_specs=[pl.BlockSpec(memory_space=pltpu.SMEM), hbm, pl.BlockSpec(memory_space=pltpu.VMEM), hbm, hbm, hbm, hbm, hbm, hbm],
        out_specs=hbm,
        out_shape=jax.ShapeDtypeStruct((NT, TM, D), A_x.dtype),
        scratch_shapes=[
            pltpu.VMEM((NT, TM, D), BF16),
            pltpu.VMEM((NT, TM, D), BF16),
            pltpu.VMEM((D, 6 * D), BF16),
            pltpu.VMEM((3, D, D), BF16),
            pltpu.VMEM((D // 2, 3 * D), U32),
            pltpu.VMEM((D, D), BF16),
            pltpu.VMEM((D, F), BF16),
            pltpu.VMEM((D, F), BF16),
            pltpu.VMEM((F, D), BF16),
            pltpu.VMEM((8, 6 * D), F32),
            pltpu.VMEM((D, 128), F32),
            pltpu.VMEM((2, TM // 2, D), U32),
            pltpu.VMEM((2, NLT, TM, 128), F32),
            pltpu.VMEM((2, NLT, HALO + TM, 128), F32),
            pltpu.VMEM((2, NLT, HALO + TM, 128), F32),
            pltpu.VMEM((TM // 2, D), U32),
            pltpu.VMEM((2, TM, D), F32),
            pltpu.VMEM((TM // 2, D), U32),
            pltpu.VMEM((TM // 2, F), U32),
            pltpu.SemaphoreType.DMA((6 * D // MC + 7,)),
            pltpu.SemaphoreType.DMA((D // WQR,)),
            pltpu.SemaphoreType.DMA((NT,)),
            pltpu.SemaphoreType.DMA((NT * NDC,)),
        ],
        compiler_params=pltpu.CompilerParams(
            vmem_limit_bytes=110 * 1024 * 1024,
        ),
    )(np.zeros((1,), np.int32), x, c, w_mod, A_wqkv, A_wo, B_w_gate, B_w_up, B_w_down)
    return out.reshape(A_x.shape)
```

```python
import jax
import jax.numpy as jnp
import numpy as np
from jax import lax
from jax.experimental import pallas as pl
from jax.experimental.pallas import tpu as pltpu

S, D, F = 2048, 1024, 3584
H, DH, W, DIL = 32, 32, 8, 2
TM = 512
NT = S // TM
HALO = 16
FC = 512
NFC = F // FC
DC = 256
NDC = D // DC
AR = 16
LR = 32
MC = 256
NLT = D // 128
QC = 512
WQR = 512
SKEW = 1
N_GU = 160
EPS = 1e-5
LOG2E = 1.4426950408889634
SCALE = DH ** -0.5 * LOG2E
F32, BF16, U32 = jnp.float32, jnp.bfloat16, jnp.uint32


def _swap_tiles_lanes(tiles):
    lane = lax.broadcasted_iota(jnp.int32, tiles[0].shape, 1)
    for b in range(3):
        sh = 4 << b
        low = (lane & sh) == 0
        new = list(tiles)
        for t in range(NLT):
            if not (t >> b) & 1:
                a, c = tiles[t], tiles[t | (1 << b)]
                new[t] = jnp.where(low, a, pltpu.roll(c, sh, 1))
                new[t | (1 << b)] = jnp.where(low, pltpu.roll(a, 128 - sh, 1), c)
        tiles = new
    return tiles


def _permute_cols(u):
    tiles = _swap_tiles_lanes([u[:, t * 128:(t + 1) * 128] for t in range(NLT)])
    return jnp.concatenate(tiles, axis=1)


def _pack(val):
    return pltpu.bitcast(val.astype(BF16), U32)


def _unpack(u):
    return pltpu.bitcast(u, BF16)


def _ln(x):
    m = jnp.mean(x, axis=-1, keepdims=True)
    xc = x - m
    v = jnp.mean(xc * xc, axis=-1, keepdims=True)
    return xc * lax.rsqrt(v + EPS)


def _ln_mod(x, scale1, shift):
    return _ln(x) * scale1 + shift


def _kernel(zero_ref, x_hbm, c_ref, wmod_hbm, wqkv_hbm, wo_hbm, wg_hbm, wu_hbm, wd_hbm, out_hbm,
            x_v, out_v, wmod_v, wraw_v, wqkv_v, wo_v, wg_v, wu_v, wd_v, mod_v, scb_s, h_s, q_s, k_s, v_s, o_s,
            x1_s, h2_s, act_s, sems, qsems, xsems, osems):
    n_mod = 6 * D // MC

    def mod_cp(j):
        return pltpu.make_async_copy(wmod_hbm.at[:, pl.ds(j * MC, MC)],
                                     wmod_v.at[:, pl.ds(j * MC, MC)], sems.at[j])

    def qkv_cp(j):
        return pltpu.make_async_copy(wqkv_hbm.at[:, pl.ds(j * D, D)],
                                     wraw_v.at[j], sems.at[n_mod + j])

    def wq_cp(n):
        rows = pl.ds(n * WQR, WQR)
        return pltpu.make_async_copy(wqkv_hbm.at[rows, pl.ds(0, D)], wraw_v.at[0, rows, :],
                                     qsems.at[n])

    def x0_cp(n):
        rows = pl.ds(n * WQR, WQR)
        return pltpu.make_async_copy(x_hbm.at[0, rows, :], x_v.at[0, rows, :],
                                     qsems.at[D // WQR + n])

    def x_cp(i):
        return pltpu.make_async_copy(x_hbm.at[i], x_v.at[i], xsems.at[i])

    def out_cp(i, n):
        cs = pl.ds(n * DC, DC)
        return pltpu.make_async_copy(out_v.at[i, :, cs], out_hbm.at[i, :, cs],
                                     osems.at[i * NDC + n])

    wo_cp = pltpu.make_async_copy(wo_hbm, wo_v, sems.at[n_mod + 3])
    wg_cp = pltpu.make_async_copy(wg_hbm, wg_v, sems.at[n_mod + 4])
    wu_cp = pltpu.make_async_copy(wu_hbm, wu_v, sems.at[n_mod + 5])
    wd_cp = pltpu.make_async_copy(wd_hbm, wd_v, sems.at[n_mod + 6])
    per = D // MC

    def mod_cps(k):
        return [mod_cp(j) for j in range(k * per, (k + 1) * per)]

    def start(cps):
        for cp in cps:
            cp.start()

    def mod_chunk(j):
        mod_cp(j).wait()
        cf = c_ref[...].astype(F32)
        sc = jnp.broadcast_to(cf * jax.nn.sigmoid(cf), (16, D)).astype(BF16)
        r = jnp.dot(sc, wmod_v[:, j * MC:(j + 1) * MC], preferred_element_type=F32)
        if j // per in (1, 4):
            r = r + 1.0
        mod_v[:, j * MC:(j + 1) * MC] = r[0:8]

    def silu_c_columns():
        cf = c_ref[...].astype(F32)
        sc = (cf * jax.nn.sigmoid(cf)).astype(BF16).astype(F32)
        for t in range(NLT):
            blk = jnp.broadcast_to(sc[:, t * 128:(t + 1) * 128], (128, 128))
            scb_s[t * 128:(t + 1) * 128, :] = blk.T

    def mod_chunk_vpu(j):
        cs = slice(j * MC, (j + 1) * MC)
        acc = paced(jnp.zeros((AR, 128), F32))
        acc = jnp.concatenate([acc] * (MC // 128), axis=1)
        for r in range(0, D, AR):
            sc = jnp.concatenate([scb_s[r:r + AR, :]] * (MC // 128), axis=1)
            acc = acc + wmod_v[r:r + AR, cs].astype(F32) * sc
        res = jnp.sum(acc, axis=0, keepdims=True)
        if j // per in (1, 4):
            res = res + 1.0
        mod_v[:, cs] = jnp.broadcast_to(res, (8, MC))

    tokens = []

    def paced(val):
        if not tokens:
            return val
        never = lax.broadcasted_iota(jnp.int32, val.shape, 0) < zero_ref[0]
        return jnp.where(never, tokens.pop(0), val)

    def paced_rows(val):
        top = jnp.concatenate([paced(val[:AR, :128]), val[:AR, 128:]], axis=1)
        return jnp.concatenate([top, val[AR:]], axis=0) if val.shape[0] > AR else top

    def post(*results):
        tokens[:] = [res[TM - AR:TM, c:c + 128] for res in results
                     for c in range(0, res.shape[1], 256)]

    def mod(k):
        return mod_v[0:1, k * D:(k + 1) * D]

    def ln1(i, r):
        xv = paced_rows(x_v[i, r:r + LR, :].astype(F32))
        h_s[i % 2, r // 2:(r + LR) // 2, :] = _pack(_ln_mod(xv, mod(1), mod(0)))

    def ln1_norm0(r):
        x1_s[0, r:r + LR, :] = _ln(x_v[0, r:r + LR, :].astype(F32))

    def ln1_apply0(j):
        cs = slice(j * MC, (j + 1) * MC)
        h_s[0, :, cs] = _pack(x1_s[0, :, cs] * mod_v[0:1, D + j * MC:D + (j + 1) * MC]
                              + mod_v[0:1, cs])

    def prep_qkv(j, r):
        wqkv_v[r // 2:r // 2 + 64, j * D:(j + 1) * D] = _permute_cols(
            _pack(wraw_v[j, r:r + 128, :]))

    def qkv_part(i, j, half):
        c0 = j * D + half * QC
        res = jnp.dot(_unpack(h_s[i % 2]), _unpack(wqkv_v[:, c0:c0 + QC]),
                      preferred_element_type=F32)
        qkv_store(i, j, half, res)
        post(res)

    def qkv_store(i, j, half, res):
        sl = i % 2
        for tt in range(QC // 128):
            t = half * (QC // 128) + tt
            blk = res[:, tt * 128:(tt + 1) * 128]
            if j == 0:
                q_s[sl, t] = blk * SCALE
                continue
            dst = k_s if j == 1 else v_s
            dst[sl, t, HALO:HALO + TM, :] = blk
            if i == 0:
                dst[sl, t, 0:HALO, :] = jnp.broadcast_to(blk[0:1], (HALO, 128))
            else:
                dst[sl, t, 0:HALO, :] = dst[1 - sl, t, TM:TM + HALO, :]

    live = {}

    def attn_qk(i, r):
        sl = i % 2
        q = [q_s[sl, t, r:r + AR, :] for t in range(NLT)]
        q[0] = paced(q[0])
        lg = []
        for w in range(W):
            o = HALO + r - DIL * w
            a = q[0] * k_s[sl, 0, o:o + AR, :]
            for t in range(1, NLT):
                a = a + q[t] * k_s[sl, t, o:o + AR, :]
            lg.append(a)
        live[i, r] = lg

    def attn_lanes(i, r):
        lane = lax.broadcasted_iota(jnp.int32, (AR, 128), 1)
        b0 = (lane & 1) == 0
        b1 = (lane & 2) == 0
        lg = [a + jnp.where(b0, pltpu.roll(a, 127, 1), pltpu.roll(a, 1, 1)) for a in live[i, r]]
        lg = [a + jnp.where(b1, pltpu.roll(a, 126, 1), pltpu.roll(a, 2, 1)) for a in lg]
        live[i, r] = lg

    def attn_softmax(i, r):
        lg = live[i, r]
        if i == 0 and r < DIL * (W - 1):
            row = lax.broadcasted_iota(jnp.int32, (AR, 128), 0) + r
            lg = [jnp.where(row >= DIL * w, a, -1000000000.0 * LOG2E) for w, a in enumerate(lg)]
        m = lg[0]
        for w in range(1, W):
            m = jnp.maximum(m, lg[w])
        e = [jnp.exp2(a - m) for a in lg]
        s = e[0]
        for w in range(1, W):
            s = s + e[w]
        inv = 1.0 / s
        live[i, r] = [a * inv for a in e]

    def attn_pv(i, r):
        sl = i % 2
        p = live.pop((i, r))
        outs = []
        for t in range(NLT):
            a = p[0] * v_s[sl, t, HALO + r:HALO + r + AR, :]
            for w in range(1, W):
                o = HALO + r - DIL * w
                a = a + p[w] * v_s[sl, t, o:o + AR, :]
            outs.append(a)
        o_s[r // 2:(r + AR) // 2, :] = _pack(jnp.concatenate(outs, axis=1))

    def attn_unpermute(i, r):
        rows = slice(r // 2, (r + AR) // 2)
        o_s[rows, :] = _permute_cols(o_s[rows, :])

    def wo_part(i, half):
        cs = slice(half * QC, (half + 1) * QC)
        y = jnp.dot(_unpack(o_s[...]), wo_v[:, cs], preferred_element_type=F32)
        ga = mod_v[0:1, 2 * D + half * QC:2 * D + (half + 1) * QC]
        x1_s[i % 2, :, cs] = x_v[i, :, cs].astype(F32) + ga * y

    def ln2(i, r):
        h2_s[r // 2:(r + LR) // 2, :] = _pack(_ln_mod(paced_rows(x1_s[i % 2, r:r + LR, :]), mod(4), mod(3)))

    def gate_up(cix):
        cs = slice(cix * FC, (cix + 1) * FC)
        h2 = _unpack(h2_s[...])
        g = jnp.dot(h2, wg_v[:, cs], preferred_element_type=F32)
        u = jnp.dot(h2, wu_v[:, cs], preferred_element_type=F32)
        post(g, u)
        t = 0.5 * g
        act_s[:, cs] = _pack((t + t * jnp.tanh(t)) * u)

    def down(i, n):
        cs = slice(n * DC, (n + 1) * DC)
        y = jnp.dot(_unpack(act_s[...]), wd_v[:, cs], preferred_element_type=F32)
        gb = mod_v[0:1, 5 * D + n * DC:5 * D + (n + 1) * DC]
        out_v[i, :, cs] = (x1_s[i % 2, :, cs] + gb * y).astype(out_v.dtype)
        out_cp(i, n).start()

    def par(mxu, vpu):
        done = 0
        for idx, (fn, *args) in enumerate(mxu):
            upto = len(vpu) * (idx + 1) // len(mxu)
            for vfn, *vargs in vpu[done:upto]:
                vfn(*vargs)
            done = upto
            fn(*args)

    halves = range(D // QC)

    def t_qkv(i, js=(0, 1, 2)):
        return [(qkv_part, i, j, hf) for j in js for hf in halves]

    def t_attn(i):
        stages = (attn_qk, attn_lanes, attn_softmax, attn_pv, attn_unpermute)
        nb = TM // AR
        return [(fn, i, (n - k * SKEW) * AR) for n in range(nb + (len(stages) - 1) * SKEW)
                for k, fn in reversed(list(enumerate(stages))) if 0 <= n - k * SKEW < nb]

    def t_ln(fn, i):
        return [(fn, i, r) for r in range(0, TM, LR)] if i < NT else []

    def t_wo(i):
        return [(wo_part, i, hf) for hf in halves]

    t_gu = [(gate_up, cix) for cix in range(NFC)]

    def t_down(i, ns):
        return [(down, i, n) for n in ns]

    def t_prep(j):
        return [(prep_qkv, j, r) for r in range(0, D, 128)]

    def t_mod(ks):
        return [(mod_chunk_vpu, j) for k in ks for j in range(k * per, (k + 1) * per)]

    def wait(cps):
        for cp in cps:
            cp.wait()

    n_wq, n_x0 = D // WQR, TM // WQR
    pairs = [[mod_cp(j), mod_cp(per + j)] for j in range(per)]
    start([x0_cp(n) for n in range(n_x0)] + [wq_cp(n) for n in range(n_wq)])
    silu_c_columns()
    wait([x0_cp(n) for n in range(n_x0)])
    start(pairs[0])
    par([(ln1_norm0, r) for r in range(0, TM, LR)], [])
    wait([wq_cp(n) for n in range(n_wq)])
    start(pairs[1] + pairs[2])
    par(t_prep(0), [])
    later = pairs[3:] + [[qkv_cp(1)]] + [[]] * per
    for j in range(per):
        start(later[j])
        par([(mod_chunk, j), (mod_chunk, per + j), (ln1_apply0, j)], [])
    start([qkv_cp(2), x_cp(1)])
    q0 = t_qkv(0)
    nh = len(halves)
    par(q0[:nh // 2], [])
    qkv_cp(1).wait()
    start([x_cp(2)] + mod_cps(2))
    par(q0[nh // 2:nh], t_prep(1))
    qkv_cp(2).wait()
    start([wo_cp] + mod_cps(3))
    par(q0[nh:2 * nh], t_prep(2))
    wait([x_cp(1)] + mod_cps(2))
    start(mod_cps(4) + mod_cps(5))
    par(q0[2 * nh:], t_ln(ln1, 1) + t_mod((2,)))
    start([wg_cp])
    x_cp(2).wait()
    par(t_qkv(1), t_attn(0) + t_ln(ln1, 2))
    start([wu_cp])
    wait(mod_cps(3) + mod_cps(4) + mod_cps(5))
    par(t_qkv(2, (0, 1)), t_mod((3, 4)))
    start([wd_cp] + [x_cp(i) for i in range(3, NT)])
    wo_cp.wait()
    par(t_wo(0), t_mod((5,)))
    par(t_qkv(2, (2,)), t_ln(ln2, 0))
    wait([wg_cp, wu_cp])
    first, second = range(NDC // 2), range(NDC // 2, NDC)
    for i in range(1, NT):
        att = t_attn(i)
        par(t_gu, att[:N_GU])
        if i == 1:
            wd_cp.wait()
        if i + 2 < NT:
            x_cp(i + 2).wait()
        par(t_down(i - 1, first), att[N_GU:])
        par(t_wo(i), t_ln(ln1, i + 2))
        par(t_down(i - 1, second), t_ln(ln2, i))
        if i + 2 < NT:
            par(t_qkv(i + 2), [])
        pass
    par(t_gu, [])
    par(t_down(NT - 1, range(NDC)), [])
    for i in range(NT):
        for n in range(NDC):
            out_cp(i, n).wait()


@jax.jit
def pallas_adaLN_cond__sliding_local_dilated__swiglu_ffn__prompt_kernel(
    A_x: jax.Array,
    A_wqkv: jax.Array,
    A_wo: jax.Array,
    B_x: jax.Array,
    B_w_gate: jax.Array,
    B_w_up: jax.Array,
    B_w_down: jax.Array,
    c: jax.Array,
    w_mod: jax.Array,
):
    del B_x
    x = A_x.reshape(NT, TM, D)
    hbm = pl.BlockSpec(memory_space=pl.ANY)
    out = pl.pallas_call(
        _kernel,
        in_specs=[pl.BlockSpec(memory_space=pltpu.SMEM), hbm, pl.BlockSpec(memory_space=pltpu.VMEM), hbm, hbm, hbm, hbm, hbm, hbm],
        out_specs=hbm,
        out_shape=jax.ShapeDtypeStruct((NT, TM, D), A_x.dtype),
        scratch_shapes=[
            pltpu.VMEM((NT, TM, D), BF16),
            pltpu.VMEM((NT, TM, D), BF16),
            pltpu.VMEM((D, 6 * D), BF16),
            pltpu.VMEM((3, D, D), BF16),
            pltpu.VMEM((D // 2, 3 * D), U32),
            pltpu.VMEM((D, D), BF16),
            pltpu.VMEM((D, F), BF16),
            pltpu.VMEM((D, F), BF16),
            pltpu.VMEM((F, D), BF16),
            pltpu.VMEM((8, 6 * D), F32),
            pltpu.VMEM((D, 128), F32),
            pltpu.VMEM((2, TM // 2, D), U32),
            pltpu.VMEM((2, NLT, TM, 128), F32),
            pltpu.VMEM((2, NLT, HALO + TM, 128), F32),
            pltpu.VMEM((2, NLT, HALO + TM, 128), F32),
            pltpu.VMEM((TM // 2, D), U32),
            pltpu.VMEM((2, TM, D), F32),
            pltpu.VMEM((TM // 2, D), U32),
            pltpu.VMEM((TM // 2, F), U32),
            pltpu.SemaphoreType.DMA((6 * D // MC + 7,)),
            pltpu.SemaphoreType.DMA(((D + TM) // WQR,)),
            pltpu.SemaphoreType.DMA((NT,)),
            pltpu.SemaphoreType.DMA((NT * NDC,)),
        ],
        compiler_params=pltpu.CompilerParams(
            vmem_limit_bytes=110 * 1024 * 1024,
        ),
    )(np.zeros((1,), np.int32), x, c, w_mod, A_wqkv, A_wo, B_w_gate, B_w_up, B_w_down)
    return out.reshape(A_x.shape)
```

```python
import jax
import jax.numpy as jnp
import numpy as np
from jax import lax
from jax.experimental import pallas as pl
from jax.experimental.pallas import tpu as pltpu

S, D, F = 2048, 1024, 3584
H, DH, W, DIL = 32, 32, 8, 2
TM = 512
NT = S // TM
HALO = 16
FC = 512
NFC = F // FC
DC = 256
NDC = D // DC
AR = 16
LR = 32
MC = 256
NLT = D // 128
QC = 512
NSTAGE = 5
SKEW = 1
N_GU = 160
EPS = 1e-5
LOG2E = 1.4426950408889634
SCALE = DH ** -0.5 * LOG2E
F32, BF16, U32 = jnp.float32, jnp.bfloat16, jnp.uint32


def _swap_tiles_lanes(tiles):
    lane = lax.broadcasted_iota(jnp.int32, tiles[0].shape, 1)
    for b in range(3):
        sh = 4 << b
        low = (lane & sh) == 0
        new = list(tiles)
        for t in range(NLT):
            if not (t >> b) & 1:
                a, c = tiles[t], tiles[t | (1 << b)]
                new[t] = jnp.where(low, a, pltpu.roll(c, sh, 1))
                new[t | (1 << b)] = jnp.where(low, pltpu.roll(a, 128 - sh, 1), c)
        tiles = new
    return tiles


def _permute_cols(u):
    tiles = _swap_tiles_lanes([u[:, t * 128:(t + 1) * 128] for t in range(NLT)])
    return jnp.concatenate(tiles, axis=1)


def _pack(val):
    return pltpu.bitcast(val.astype(BF16), U32)


def _unpack(u):
    return pltpu.bitcast(u, BF16)


def _ln(x):
    m = jnp.mean(x, axis=-1, keepdims=True)
    xc = x - m
    v = jnp.mean(xc * xc, axis=-1, keepdims=True)
    return xc * lax.rsqrt(v + EPS)


def _ln_mod(x, scale1, shift):
    return _ln(x) * scale1 + shift


def _kernel(zero_ref, x_hbm, c_ref, wmod_hbm, wqkv_hbm, wo_hbm, wg_hbm, wu_hbm, wd_hbm, out_hbm,
            x_v, out_v, wmod_v, wraw_v, wqkv_v, wo_v, wg_v, wu_v, wd_v, mod_v, scb_s, h_s, q_s, k_s, v_s, o_s,
            x1_s, h2_s, act_s, sems, qsems, xsems, osems):
    n_mod = 6 * D // MC

    def mod_cp(j):
        return pltpu.make_async_copy(wmod_hbm.at[:, pl.ds(j * MC, MC)],
                                     wmod_v.at[:, pl.ds(j * MC, MC)], sems.at[j])

    def qkv_cp(k):
        rows = pl.ds(k * MC, MC)
        return pltpu.make_async_copy(wqkv_hbm.at[rows, :], wraw_v.at[rows, :], qsems.at[k])

    def x_cp(i):
        return pltpu.make_async_copy(x_hbm.at[i], x_v.at[i], xsems.at[i])

    def out_cp(i, n):
        cs = pl.ds(n * DC, DC)
        return pltpu.make_async_copy(out_v.at[i, :, cs], out_hbm.at[i, :, cs],
                                     osems.at[i * NDC + n])

    wo_cp = pltpu.make_async_copy(wo_hbm, wo_v, sems.at[n_mod + 3])
    wg_cp = pltpu.make_async_copy(wg_hbm, wg_v, sems.at[n_mod + 4])
    wu_cp = pltpu.make_async_copy(wu_hbm, wu_v, sems.at[n_mod + 5])
    wd_cp = pltpu.make_async_copy(wd_hbm, wd_v, sems.at[n_mod + 6])
    per = D // MC

    def mod_cps(k):
        return [mod_cp(j) for j in range(k * per, (k + 1) * per)]

    def start(cps):
        for cp in cps:
            cp.start()

    def mod_chunk(j):
        mod_cp(j).wait()
        cf = c_ref[...].astype(F32)
        sc = jnp.broadcast_to(cf * jax.nn.sigmoid(cf), (16, D)).astype(BF16)
        r = jnp.dot(sc, wmod_v[:, j * MC:(j + 1) * MC], preferred_element_type=F32)
        if j // per in (1, 4):
            r = r + 1.0
        mod_v[:, j * MC:(j + 1) * MC] = r[0:8]

    def silu_c_columns():
        cf = c_ref[...].astype(F32)
        sc = (cf * jax.nn.sigmoid(cf)).astype(BF16).astype(F32)
        for t in range(NLT):
            blk = jnp.broadcast_to(sc[:, t * 128:(t + 1) * 128], (128, 128))
            scb_s[t * 128:(t + 1) * 128, :] = blk.T

    def mod_chunk_vpu(j):
        cs = slice(j * MC, (j + 1) * MC)
        acc = paced(jnp.zeros((AR, 128), F32))
        acc = jnp.concatenate([acc] * (MC // 128), axis=1)
        for r in range(0, D, AR):
            sc = jnp.concatenate([scb_s[r:r + AR, :]] * (MC // 128), axis=1)
            acc = acc + wmod_v[r:r + AR, cs].astype(F32) * sc
        res = jnp.sum(acc, axis=0, keepdims=True)
        if j // per in (1, 4):
            res = res + 1.0
        mod_v[:, cs] = jnp.broadcast_to(res, (8, MC))

    tokens = []

    def paced(val):
        if not tokens:
            return val
        never = lax.broadcasted_iota(jnp.int32, val.shape, 0) < zero_ref[0]
        return jnp.where(never, tokens.pop(0), val)

    def paced_rows(val):
        top = jnp.concatenate([paced(val[:AR, :128]), val[:AR, 128:]], axis=1)
        return jnp.concatenate([top, val[AR:]], axis=0) if val.shape[0] > AR else top

    def post(*results):
        tokens[:] = [res[TM - AR:TM, c:c + 128] for res in results
                     for c in range(0, res.shape[1], 256)]

    def mod(k):
        return mod_v[0:1, k * D:(k + 1) * D]

    def ln1(i, r):
        xv = paced_rows(x_v[i, r:r + LR, :].astype(F32))
        h_s[i % 2, r // 2:(r + LR) // 2, :] = _pack(_ln_mod(xv, mod(1), mod(0)))

    def ln1_norm0(r):
        x1_s[0, r:r + LR, :] = _ln(x_v[0, r:r + LR, :].astype(F32))

    def ln1_apply0(j):
        cs = slice(j * MC, (j + 1) * MC)
        h_s[0, :, cs] = _pack(x1_s[0, :, cs] * mod_v[0:1, D + j * MC:D + (j + 1) * MC]
                              + mod_v[0:1, cs])

    def prep_qkv(j, k):
        for r in range(k * MC, (k + 1) * MC, 128):
            wqkv_v[r // 2:r // 2 + 64, j * D:(j + 1) * D] = _permute_cols(
                _pack(wraw_v[r:r + 128, j * D:(j + 1) * D]))

    def qkv_first(j, k):
        res = jnp.dot(_unpack(h_s[0, :, k * MC:(k + 1) * MC]),
                      _unpack(wqkv_v[k * MC // 2:(k + 1) * MC // 2, j * D:(j + 1) * D]),
                      preferred_element_type=F32)
        post(res)
        if k > 0:
            dst, r0 = ((q_s, 0), (k_s, HALO), (v_s, HALO))[j]
            res = res + jnp.concatenate([dst[0, t, r0:r0 + TM, :] for t in range(NLT)], axis=1)
        qkv_store(0, j, 0, res, final=k == D // MC - 1)

    def qkv_part(i, j, half):
        c0 = j * D + half * QC
        res = jnp.dot(_unpack(h_s[i % 2]), _unpack(wqkv_v[:, c0:c0 + QC]),
                      preferred_element_type=F32)
        qkv_store(i, j, half, res)
        post(res)

    def qkv_store(i, j, half, res, final=True):
        sl = i % 2
        for tt in range(res.shape[1] // 128):
            t = half * (QC // 128) + tt
            blk = res[:, tt * 128:(tt + 1) * 128]
            if j == 0:
                q_s[sl, t] = blk * SCALE if final else blk
                continue
            dst = k_s if j == 1 else v_s
            dst[sl, t, HALO:HALO + TM, :] = blk
            if not final:
                continue
            if i == 0:
                dst[sl, t, 0:HALO, :] = jnp.broadcast_to(blk[0:1], (HALO, 128))
            else:
                dst[sl, t, 0:HALO, :] = dst[1 - sl, t, TM:TM + HALO, :]

    live = {}

    def attn_qk(i, r):
        sl = i % 2
        q = [q_s[sl, t, r:r + AR, :] for t in range(NLT)]
        q[0] = paced(q[0])
        lg = []
        for w in range(W):
            o = HALO + r - DIL * w
            a = q[0] * k_s[sl, 0, o:o + AR, :]
            for t in range(1, NLT):
                a = a + q[t] * k_s[sl, t, o:o + AR, :]
            lg.append(a)
        live[i, r] = lg

    def attn_lanes(i, r):
        lane = lax.broadcasted_iota(jnp.int32, (AR, 128), 1)
        b0 = (lane & 1) == 0
        b1 = (lane & 2) == 0
        lg = [a + jnp.where(b0, pltpu.roll(a, 127, 1), pltpu.roll(a, 1, 1)) for a in live[i, r]]
        lg = [a + jnp.where(b1, pltpu.roll(a, 126, 1), pltpu.roll(a, 2, 1)) for a in lg]
        live[i, r] = lg

    def attn_softmax(i, r):
        lg = live[i, r]
        if i == 0 and r < DIL * (W - 1):
            row = lax.broadcasted_iota(jnp.int32, (AR, 128), 0) + r
            lg = [jnp.where(row >= DIL * w, a, -1000000000.0 * LOG2E) for w, a in enumerate(lg)]
        m = lg[0]
        for w in range(1, W):
            m = jnp.maximum(m, lg[w])
        e = [jnp.exp2(a - m) for a in lg]
        s = e[0]
        for w in range(1, W):
            s = s + e[w]
        inv = 1.0 / s
        live[i, r] = [a * inv for a in e]

    def attn_pv(i, r):
        sl = i % 2
        p = live.pop((i, r))
        outs = []
        for t in range(NLT):
            a = p[0] * v_s[sl, t, HALO + r:HALO + r + AR, :]
            for w in range(1, W):
                o = HALO + r - DIL * w
                a = a + p[w] * v_s[sl, t, o:o + AR, :]
            outs.append(a)
        o_s[r // 2:(r + AR) // 2, :] = _pack(jnp.concatenate(outs, axis=1))

    def attn_unpermute(i, r):
        rows = slice(r // 2, (r + AR) // 2)
        o_s[rows, :] = _permute_cols(o_s[rows, :])

    def wo_part(i, half):
        cs = slice(half * QC, (half + 1) * QC)
        y = jnp.dot(_unpack(o_s[...]), wo_v[:, cs], preferred_element_type=F32)
        ga = mod_v[0:1, 2 * D + half * QC:2 * D + (half + 1) * QC]
        x1_s[i % 2, :, cs] = x_v[i, :, cs].astype(F32) + ga * y

    def ln2(i, r):
        h2_s[r // 2:(r + LR) // 2, :] = _pack(_ln_mod(paced_rows(x1_s[i % 2, r:r + LR, :]), mod(4), mod(3)))

    def gate_up(cix):
        cs = slice(cix * FC, (cix + 1) * FC)
        h2 = _unpack(h2_s[...])
        g = jnp.dot(h2, wg_v[:, cs], preferred_element_type=F32)
        u = jnp.dot(h2, wu_v[:, cs], preferred_element_type=F32)
        post(g, u)
        t = 0.5 * g
        act_s[:, cs] = _pack((t + t * jnp.tanh(t)) * u)

    def down(i, n):
        cs = slice(n * DC, (n + 1) * DC)
        y = jnp.dot(_unpack(act_s[...]), wd_v[:, cs], preferred_element_type=F32)
        gb = mod_v[0:1, 5 * D + n * DC:5 * D + (n + 1) * DC]
        out_v[i, :, cs] = (x1_s[i % 2, :, cs] + gb * y).astype(out_v.dtype)
        out_cp(i, n).start()

    def par(mxu, vpu):
        done = 0
        for idx, (fn, *args) in enumerate(mxu):
            upto = len(vpu) * (idx + 1) // len(mxu)
            for vfn, *vargs in vpu[done:upto]:
                vfn(*vargs)
            done = upto
            fn(*args)

    halves = range(D // QC)

    def t_qkv(i, js=(0, 1, 2)):
        return [(qkv_part, i, j, hf) for j in js for hf in halves]

    def t_attn(i):
        stages = (attn_qk, attn_lanes, attn_softmax, attn_pv, attn_unpermute)[:NSTAGE]
        nb = TM // AR
        return [(fn, i, (n - k * SKEW) * AR) for n in range(nb + (len(stages) - 1) * SKEW)
                for k, fn in reversed(list(enumerate(stages))) if 0 <= n - k * SKEW < nb]

    def t_ln(fn, i):
        return [(fn, i, r) for r in range(0, TM, LR)] if i < NT else []

    def t_wo(i):
        return [(wo_part, i, hf) for hf in halves]

    t_gu = [(gate_up, cix) for cix in range(NFC)]

    def t_down(i, ns):
        return [(down, i, n) for n in ns]

    def t_mod(ks):
        return [(mod_chunk_vpu, j) for k in ks for j in range(k * per, (k + 1) * per)]

    def wait(cps):
        for cp in cps:
            cp.wait()

    def chunk_cps(k):
        return [mod_cp(k), mod_cp(per + k), qkv_cp(k)]

    def chunk_ready(k):
        mod_chunk(k)
        mod_chunk(per + k)
        ln1_apply0(k)
        qkv_cp(k).wait()

    start([x_cp(0)] + chunk_cps(0))
    silu_c_columns()
    x_cp(0).wait()
    start(chunk_cps(1))
    par([(ln1_norm0, r) for r in range(0, TM, LR)], [])
    chunk_ready(0)
    prep_qkv(0, 0)
    later = [chunk_cps(k) for k in range(2, per)] + [[x_cp(1), x_cp(2)], mod_cps(2) + [wo_cp]]
    steps = [(j, k) for k in range(per) for j in range(3)]
    ln_next = t_ln(ln1, 1)
    for n, (j, k) in enumerate(steps):
        if j == 0:
            start(later[k])
        if n + 1 < len(steps):
            if steps[n + 1][0] == 0:
                chunk_ready(k + 1)
            prep_qkv(*steps[n + 1])
        if n == len(steps) - 3:
            x_cp(1).wait()
        if n >= len(steps) - 2:
            half = len(ln_next) // 2
            par(ln_next[:half] if n == len(steps) - 2 else ln_next[half:], [])
        qkv_first(j, k)
    start(mod_cps(3) + mod_cps(4) + mod_cps(5) + [wg_cp])
    x_cp(2).wait()
    par(t_qkv(1), t_attn(0) + t_ln(ln1, 2))
    start([wu_cp])
    wait(mod_cps(2) + mod_cps(3) + mod_cps(4) + mod_cps(5))
    q2 = t_qkv(2)
    par(q2[:-1], t_mod((2, 3, 4)))
    start([wd_cp] + [x_cp(i) for i in range(3, NT)])
    wo_cp.wait()
    par(t_wo(0), [])
    par(q2[-1:], t_ln(ln2, 0))
    wait([wg_cp, wu_cp])
    first, second = range(NDC // 2), range(NDC // 2, NDC)
    for i in range(1, NT):
        att = t_attn(i)
        par(t_gu, att[:N_GU] + (t_mod((5,)) if i == 1 else []))
        if i == 1:
            wd_cp.wait()
        if i + 2 < NT:
            x_cp(i + 2).wait()
        par(t_down(i - 1, first), att[N_GU:])
        par(t_wo(i), t_ln(ln1, i + 2))
        par(t_down(i - 1, second), t_ln(ln2, i))
        if i + 2 < NT:
            par(t_qkv(i + 2), [])
        pass
    par(t_gu, [])
    par(t_down(NT - 1, range(NDC)), [])
    for i in range(NT):
        for n in range(NDC):
            out_cp(i, n).wait()


@jax.jit
def pallas_adaLN_cond__sliding_local_dilated__swiglu_ffn__prompt_kernel(
    A_x: jax.Array,
    A_wqkv: jax.Array,
    A_wo: jax.Array,
    B_x: jax.Array,
    B_w_gate: jax.Array,
    B_w_up: jax.Array,
    B_w_down: jax.Array,
    c: jax.Array,
    w_mod: jax.Array,
):
    del B_x
    x = A_x.reshape(NT, TM, D)
    hbm = pl.BlockSpec(memory_space=pl.ANY)
    out = pl.pallas_call(
        _kernel,
        in_specs=[pl.BlockSpec(memory_space=pltpu.SMEM), hbm, pl.BlockSpec(memory_space=pltpu.VMEM), hbm, hbm, hbm, hbm, hbm, hbm],
        out_specs=hbm,
        out_shape=jax.ShapeDtypeStruct((NT, TM, D), A_x.dtype),
        scratch_shapes=[
            pltpu.VMEM((NT, TM, D), BF16),
            pltpu.VMEM((NT, TM, D), BF16),
            pltpu.VMEM((D, 6 * D), BF16),
            pltpu.VMEM((D, 3 * D), BF16),
            pltpu.VMEM((D // 2, 3 * D), U32),
            pltpu.VMEM((D, D), BF16),
            pltpu.VMEM((D, F), BF16),
            pltpu.VMEM((D, F), BF16),
            pltpu.VMEM((F, D), BF16),
            pltpu.VMEM((8, 6 * D), F32),
            pltpu.VMEM((D, 128), F32),
            pltpu.VMEM((2, TM // 2, D), U32),
            pltpu.VMEM((2, NLT, TM, 128), F32),
            pltpu.VMEM((2, NLT, HALO + TM, 128), F32),
            pltpu.VMEM((2, NLT, HALO + TM, 128), F32),
            pltpu.VMEM((TM // 2, D), U32),
            pltpu.VMEM((2, TM, D), F32),
            pltpu.VMEM((TM // 2, D), U32),
            pltpu.VMEM((TM // 2, F), U32),
            pltpu.SemaphoreType.DMA((6 * D // MC + 7,)),
            pltpu.SemaphoreType.DMA((D // MC,)),
            pltpu.SemaphoreType.DMA((NT,)),
            pltpu.SemaphoreType.DMA((NT * NDC,)),
        ],
        compiler_params=pltpu.CompilerParams(
            vmem_limit_bytes=110 * 1024 * 1024,
        ),
    )(np.zeros((1,), np.int32), x, c, w_mod, A_wqkv, A_wo, B_w_gate, B_w_up, B_w_down)
    return out.reshape(A_x.shape)


def _rederive():
    global NT, NFC, NDC
    NT, NFC, NDC = S // TM, F // FC, D // DC
```

```python
import jax
import jax.numpy as jnp
import numpy as np
from jax import lax
from jax.experimental import pallas as pl
from jax.experimental.pallas import tpu as pltpu

S, D, F = 2048, 1024, 3584
H, DH, W, DIL = 32, 32, 8, 2
TM = 512
NT = S // TM
HALO = 16
FC = 512
NFC = F // FC
DC = 256
NDC = D // DC
AR = 16
LR = 16
MC = 256
NLT = D // 128
QC = 512
WR = 256
N_D1 = 3
NSTAGE = 5
SKEW = 1
N_GU = 160
EPS = 1e-5
LOG2E = 1.4426950408889634
SCALE = DH ** -0.5 * LOG2E
F32, BF16, U32 = jnp.float32, jnp.bfloat16, jnp.uint32


def _swap_tiles_lanes(tiles):
    lane = lax.broadcasted_iota(jnp.int32, tiles[0].shape, 1)
    for b in range(3):
        sh = 4 << b
        low = (lane & sh) == 0
        new = list(tiles)
        for t in range(NLT):
            if not (t >> b) & 1:
                a, c = tiles[t], tiles[t | (1 << b)]
                new[t] = jnp.where(low, a, pltpu.roll(c, sh, 1))
                new[t | (1 << b)] = jnp.where(low, pltpu.roll(a, 128 - sh, 1), c)
        tiles = new
    return tiles


def _permute_cols(u):
    tiles = _swap_tiles_lanes([u[:, t * 128:(t + 1) * 128] for t in range(NLT)])
    return jnp.concatenate(tiles, axis=1)


def _pack(val):
    return pltpu.bitcast(val.astype(BF16), U32)


def _unpack(u):
    return pltpu.bitcast(u, BF16)


def _ln(x):
    m = jnp.mean(x, axis=-1, keepdims=True)
    xc = x - m
    v = jnp.mean(xc * xc, axis=-1, keepdims=True)
    return xc * lax.rsqrt(v + EPS)


def _ln_mod(x, scale1, shift):
    return _ln(x) * scale1 + shift


def _kernel(zero_ref, x_hbm, c_ref, wmod_hbm, wqkv_hbm, wo_hbm, wg_hbm, wu_hbm, wd_hbm, out_hbm,
            x_v, out_v, wmod_v, wraw_v, wqkv_v, wo_v, wg_v, wu_v, wd_v, mod_v, scb_s, h_s, q_s, k_s, v_s, o_s,
            x1_s, h2_s, act_s, sems, qsems, xsems, osems):
    n_mod = 6 * D // MC

    def mod_cp(j):
        return pltpu.make_async_copy(wmod_hbm.at[:, pl.ds(j * MC, MC)],
                                     wmod_v.at[:, pl.ds(j * MC, MC)], sems.at[j])

    def qkv_cp(k):
        rows = pl.ds(k * MC, MC)
        return pltpu.make_async_copy(wqkv_hbm.at[rows, :], wraw_v.at[rows, :], qsems.at[k])

    def x_cp(i):
        return pltpu.make_async_copy(x_hbm.at[i], x_v.at[i], xsems.at[i])

    def out_cp(i, n):
        cs = pl.ds(n * DC, DC)
        return pltpu.make_async_copy(out_v.at[i, :, cs], out_hbm.at[i, :, cs],
                                     osems.at[i * NDC + n])

    wo_cp = pltpu.make_async_copy(wo_hbm, wo_v, sems.at[n_mod + 3])
    wg_cp = pltpu.make_async_copy(wg_hbm, wg_v, sems.at[n_mod + 4])
    wu_cp = pltpu.make_async_copy(wu_hbm, wu_v, sems.at[n_mod + 5])
    wd_cp = pltpu.make_async_copy(wd_hbm, wd_v, sems.at[n_mod + 6])
    per = D // MC

    def mod_cps(k):
        return [mod_cp(j) for j in range(k * per, (k + 1) * per)]

    def start(cps):
        for cp in cps:
            cp.start()

    def mod_chunk(j):
        mod_cp(j).wait()
        cf = c_ref[...].astype(F32)
        sc = jnp.broadcast_to(cf * jax.nn.sigmoid(cf), (16, D)).astype(BF16)
        r = jnp.dot(sc, wmod_v[:, j * MC:(j + 1) * MC], preferred_element_type=F32)
        if j // per in (1, 4):
            r = r + 1.0
        mod_v[:, j * MC:(j + 1) * MC] = r[0:8]

    def silu_c_columns():
        cf = c_ref[...].astype(F32)
        sc = (cf * jax.nn.sigmoid(cf)).astype(BF16).astype(F32)
        for t in range(NLT):
            blk = jnp.broadcast_to(sc[:, t * 128:(t + 1) * 128], (128, 128))
            scb_s[t * 128:(t + 1) * 128, :] = blk.T

    def mod_chunk_vpu(j):
        cs = slice(j * MC, (j + 1) * MC)
        acc = paced(jnp.zeros((AR, 128), F32))
        acc = jnp.concatenate([acc] * (MC // 128), axis=1)
        for r in range(0, D, AR):
            sc = jnp.concatenate([scb_s[r:r + AR, :]] * (MC // 128), axis=1)
            acc = acc + wmod_v[r:r + AR, cs].astype(F32) * sc
        res = jnp.sum(acc, axis=0, keepdims=True)
        if j // per in (1, 4):
            res = res + 1.0
        mod_v[:, cs] = jnp.broadcast_to(res, (8, MC))

    tokens = []

    def paced(val):
        if not tokens:
            return val
        never = lax.broadcasted_iota(jnp.int32, val.shape, 0) < zero_ref[0]
        return jnp.where(never, tokens.pop(0), val)

    def paced_rows(val):
        top = jnp.concatenate([paced(val[:AR, :128]), val[:AR, 128:]], axis=1)
        return jnp.concatenate([top, val[AR:]], axis=0) if val.shape[0] > AR else top

    def post(*results):
        tokens[:] = [res[TM - AR:TM, c:c + 128] for res in results
                     for c in range(0, res.shape[1], 256)]

    def mod(k):
        return mod_v[0:1, k * D:(k + 1) * D]

    def ln1(i, r):
        xv = paced_rows(x_v[i, r:r + LR, :].astype(F32))
        h_s[i % 2, r // 2:(r + LR) // 2, :] = _pack(_ln_mod(xv, mod(1), mod(0)))

    def ln1_norm0(r):
        x1_s[0, r:r + LR, :] = _ln(x_v[0, r:r + LR, :].astype(F32))

    def ln1_apply0(j):
        cs = slice(j * MC, (j + 1) * MC)
        h_s[0, :, cs] = _pack(x1_s[0, :, cs] * mod_v[0:1, D + j * MC:D + (j + 1) * MC]
                              + mod_v[0:1, cs])

    def prep_qkv(j, k):
        for r in range(k * MC, (k + 1) * MC, 128):
            wqkv_v[r // 2:r // 2 + 64, j * D:(j + 1) * D] = _permute_cols(
                _pack(wraw_v[r:r + 128, j * D:(j + 1) * D]))

    def qkv_first(j, k):
        res = jnp.dot(_unpack(h_s[0, :, k * MC:(k + 1) * MC]),
                      _unpack(wqkv_v[k * MC // 2:(k + 1) * MC // 2, j * D:(j + 1) * D]),
                      preferred_element_type=F32)
        post(res)
        if k > 0:
            dst, r0 = ((q_s, 0), (k_s, HALO), (v_s, HALO))[j]
            res = res + jnp.concatenate([dst[0, t, r0:r0 + TM, :] for t in range(NLT)], axis=1)
        qkv_store(0, j, 0, res, final=k == D // MC - 1)

    def qkv_part(i, j, half):
        c0 = j * D + half * QC
        res = jnp.dot(_unpack(h_s[i % 2]), _unpack(wqkv_v[:, c0:c0 + QC]),
                      preferred_element_type=F32)
        qkv_store(i, j, half, res)
        post(res)

    def qkv_store(i, j, half, res, final=True):
        sl = i % 2
        for tt in range(res.shape[1] // 128):
            t = half * (QC // 128) + tt
            blk = res[:, tt * 128:(tt + 1) * 128]
            if j == 0:
                q_s[sl, t] = blk * SCALE if final else blk
                continue
            dst = k_s if j == 1 else v_s
            dst[sl, t, HALO:HALO + TM, :] = blk
            if not final:
                continue
            if i == 0:
                dst[sl, t, 0:HALO, :] = jnp.broadcast_to(blk[0:1], (HALO, 128))
            else:
                dst[sl, t, 0:HALO, :] = dst[1 - sl, t, TM:TM + HALO, :]

    live = {}

    def attn_qk(i, r):
        sl = i % 2
        q = [q_s[sl, t, r:r + AR, :] for t in range(NLT)]
        q[0] = paced(q[0])
        lg = []
        for w in range(W):
            o = HALO + r - DIL * w
            a = q[0] * k_s[sl, 0, o:o + AR, :]
            for t in range(1, NLT):
                a = a + q[t] * k_s[sl, t, o:o + AR, :]
            lg.append(a)
        live[i, r] = lg

    def attn_lanes(i, r):
        lane = lax.broadcasted_iota(jnp.int32, (AR, 128), 1)
        b0 = (lane & 1) == 0
        b1 = (lane & 2) == 0
        lg = [a + jnp.where(b0, pltpu.roll(a, 127, 1), pltpu.roll(a, 1, 1)) for a in live[i, r]]
        lg = [a + jnp.where(b1, pltpu.roll(a, 126, 1), pltpu.roll(a, 2, 1)) for a in lg]
        live[i, r] = lg

    def attn_softmax(i, r):
        lg = live[i, r]
        if i == 0 and r < DIL * (W - 1):
            row = lax.broadcasted_iota(jnp.int32, (AR, 128), 0) + r
            lg = [jnp.where(row >= DIL * w, a, -1000000000.0 * LOG2E) for w, a in enumerate(lg)]
        m = lg[0]
        for w in range(1, W):
            m = jnp.maximum(m, lg[w])
        e = [jnp.exp2(a - m) for a in lg]
        s = e[0]
        for w in range(1, W):
            s = s + e[w]
        inv = 1.0 / s
        live[i, r] = [a * inv for a in e]

    def attn_pv(i, r):
        sl = i % 2
        p = live.pop((i, r))
        outs = []
        for t in range(NLT):
            a = p[0] * v_s[sl, t, HALO + r:HALO + r + AR, :]
            for w in range(1, W):
                o = HALO + r - DIL * w
                a = a + p[w] * v_s[sl, t, o:o + AR, :]
            outs.append(a)
        o_s[r // 2:(r + AR) // 2, :] = _pack(jnp.concatenate(outs, axis=1))

    def attn_unpermute(i, r):
        rows = slice(r // 2, (r + AR) // 2)
        o_s[rows, :] = _permute_cols(o_s[rows, :])

    def wo_part(i, r0):
        y = jnp.dot(_unpack(o_s[r0 // 2:(r0 + WR) // 2, :]), wo_v[...],
                    preferred_element_type=F32)
        for r in range(r0, r0 + WR, LR):
            x1 = x_v[i, r:r + LR, :].astype(F32) + mod(2) * y[r - r0:r - r0 + LR]
            x1_s[i % 2, r:r + LR, :] = x1
            h2_s[r // 2:(r + LR) // 2, :] = _pack(_ln_mod(x1, mod(4), mod(3)))

    def gate_up(cix):
        cs = slice(cix * FC, (cix + 1) * FC)
        h2 = _unpack(h2_s[...])
        g = jnp.dot(h2, wg_v[:, cs], preferred_element_type=F32)
        u = jnp.dot(h2, wu_v[:, cs], preferred_element_type=F32)
        post(g, u)
        t = 0.5 * g
        act_s[:, cs] = _pack((t + t * jnp.tanh(t)) * u)

    def down(i, n):
        cs = slice(n * DC, (n + 1) * DC)
        y = jnp.dot(_unpack(act_s[...]), wd_v[:, cs], preferred_element_type=F32)
        post(y)
        gb = mod_v[0:1, 5 * D + n * DC:5 * D + (n + 1) * DC]
        out_v[i, :, cs] = (x1_s[i % 2, :, cs] + gb * y).astype(out_v.dtype)
        out_cp(i, n).start()

    def par(mxu, vpu):
        done = 0
        for idx, (fn, *args) in enumerate(mxu):
            upto = len(vpu) * (idx + 1) // len(mxu)
            for vfn, *vargs in vpu[done:upto]:
                vfn(*vargs)
            done = upto
            fn(*args)

    halves = range(D // QC)

    def t_qkv(i, js=(0, 1, 2)):
        return [(qkv_part, i, j, hf) for j in js for hf in halves]

    def t_attn(i):
        stages = (attn_qk, attn_lanes, attn_softmax, attn_pv, attn_unpermute)[:NSTAGE]
        nb = TM // AR
        return [(fn, i, (n - k * SKEW) * AR) for n in range(nb + (len(stages) - 1) * SKEW)
                for k, fn in reversed(list(enumerate(stages))) if 0 <= n - k * SKEW < nb]

    def t_ln(fn, i):
        return [(fn, i, r) for r in range(0, TM, LR)] if i < NT else []

    def t_wo(i):
        return [(wo_part, i, r) for r in range(0, TM, WR)]

    t_gu = [(gate_up, cix) for cix in range(NFC)]

    def t_down(i, ns):
        return [(down, i, n) for n in ns]

    def t_mod(ks):
        return [(mod_chunk_vpu, j) for k in ks for j in range(k * per, (k + 1) * per)]

    def wait(cps):
        for cp in cps:
            cp.wait()

    def chunk_cps(k):
        return [mod_cp(k), mod_cp(per + k), qkv_cp(k)]

    def chunk_ready(k):
        mod_chunk(k)
        mod_chunk(per + k)
        ln1_apply0(k)
        qkv_cp(k).wait()

    start([x_cp(0)] + chunk_cps(0))
    silu_c_columns()
    x_cp(0).wait()
    start(chunk_cps(1))
    par([(ln1_norm0, r) for r in range(0, TM, LR)], [])
    chunk_ready(0)
    prep_qkv(0, 0)
    later = [chunk_cps(k) for k in range(2, per)] + [[x_cp(1), x_cp(2)], mod_cps(2) + [wo_cp]]
    steps = [(j, k) for k in range(per) for j in range(3)]
    ln_next = t_ln(ln1, 1)
    for n, (j, k) in enumerate(steps):
        if j == 0:
            start(later[k])
        if n + 1 < len(steps):
            if steps[n + 1][0] == 0:
                chunk_ready(k + 1)
            prep_qkv(*steps[n + 1])
        if n == len(steps) - 3:
            x_cp(1).wait()
        if n >= len(steps) - 2:
            half = len(ln_next) // 2
            par(ln_next[:half] if n == len(steps) - 2 else ln_next[half:], [])
        qkv_first(j, k)
    start(mod_cps(3) + mod_cps(4) + mod_cps(5) + [wg_cp])
    x_cp(2).wait()
    par(t_qkv(1), t_attn(0) + t_ln(ln1, 2))
    start([wu_cp])
    wait(mod_cps(2) + mod_cps(3) + mod_cps(4) + mod_cps(5))
    q2 = t_qkv(2)
    par(q2[:-1], t_mod((2, 3, 4)))
    start([wd_cp] + [x_cp(i) for i in range(3, NT)])
    wo_cp.wait()
    par(t_wo(0), [])
    par(q2[-1:], [])
    wait([wg_cp, wu_cp])
    first, second = range(N_D1), range(N_D1, NDC)
    for i in range(1, NT):
        att = t_attn(i)
        par(t_gu, att[:N_GU] + (t_mod((5,)) if i == 1 else []))
        if i == 1:
            wd_cp.wait()
        if i + 2 < NT:
            x_cp(i + 2).wait()
        par(t_down(i - 1, first), att[N_GU:] + t_ln(ln1, i + 2))
        par(t_wo(i), [])
        par(t_down(i - 1, second), [])
        if i + 2 < NT:
            par(t_qkv(i + 2), [])
        pass
    par(t_gu, [])
    par(t_down(NT - 1, range(NDC)), [])
    for i in range(NT):
        for n in range(NDC):
            out_cp(i, n).wait()


@jax.jit
def pallas_adaLN_cond__sliding_local_dilated__swiglu_ffn__prompt_kernel(
    A_x: jax.Array,
    A_wqkv: jax.Array,
    A_wo: jax.Array,
    B_x: jax.Array,
    B_w_gate: jax.Array,
    B_w_up: jax.Array,
    B_w_down: jax.Array,
    c: jax.Array,
    w_mod: jax.Array,
):
    del B_x
    x = A_x.reshape(NT, TM, D)
    hbm = pl.BlockSpec(memory_space=pl.ANY)
    out = pl.pallas_call(
        _kernel,
        in_specs=[pl.BlockSpec(memory_space=pltpu.SMEM), hbm, pl.BlockSpec(memory_space=pltpu.VMEM), hbm, hbm, hbm, hbm, hbm, hbm],
        out_specs=hbm,
        out_shape=jax.ShapeDtypeStruct((NT, TM, D), A_x.dtype),
        scratch_shapes=[
            pltpu.VMEM((NT, TM, D), BF16),
            pltpu.VMEM((NT, TM, D), BF16),
            pltpu.VMEM((D, 6 * D), BF16),
            pltpu.VMEM((D, 3 * D), BF16),
            pltpu.VMEM((D // 2, 3 * D), U32),
            pltpu.VMEM((D, D), BF16),
            pltpu.VMEM((D, F), BF16),
            pltpu.VMEM((D, F), BF16),
            pltpu.VMEM((F, D), BF16),
            pltpu.VMEM((8, 6 * D), F32),
            pltpu.VMEM((D, 128), F32),
            pltpu.VMEM((2, TM // 2, D), U32),
            pltpu.VMEM((2, NLT, TM, 128), F32),
            pltpu.VMEM((2, NLT, HALO + TM, 128), F32),
            pltpu.VMEM((2, NLT, HALO + TM, 128), F32),
            pltpu.VMEM((TM // 2, D), U32),
            pltpu.VMEM((2, TM, D), F32),
            pltpu.VMEM((TM // 2, D), U32),
            pltpu.VMEM((TM // 2, F), U32),
            pltpu.SemaphoreType.DMA((6 * D // MC + 7,)),
            pltpu.SemaphoreType.DMA((D // MC,)),
            pltpu.SemaphoreType.DMA((NT,)),
            pltpu.SemaphoreType.DMA((NT * NDC,)),
        ],
        compiler_params=pltpu.CompilerParams(
            vmem_limit_bytes=110 * 1024 * 1024,
        ),
    )(np.zeros((1,), np.int32), x, c, w_mod, A_wqkv, A_wo, B_w_gate, B_w_up, B_w_down)
    return out.reshape(A_x.shape)


def _rederive():
    global NT, NFC, NDC
    NT, NFC, NDC = S // TM, F // FC, D // DC
```

```python
import jax
import jax.numpy as jnp
import numpy as np
from jax import lax
from jax.experimental import pallas as pl
from jax.experimental.pallas import tpu as pltpu

S, D, F = 2048, 1024, 3584
H, DH, W, DIL = 32, 32, 8, 2
TM = 512
NT = S // TM
HALO = 16
FC = 512
NFC = F // FC
DC = 256
NDC = D // DC
AR = 16
LR = 16
MC = 256
NLT = D // 128
QC = 512
WR = 256
N_D1 = 3
NSTAGE = 5
SKEW = 1
N_GU = 160
EPS = 1e-5
LOG2E = 1.4426950408889634
SCALE = DH ** -0.5 * LOG2E
F32, BF16, U32 = jnp.float32, jnp.bfloat16, jnp.uint32


def _swap_tiles_lanes(tiles):
    lane = lax.broadcasted_iota(jnp.int32, tiles[0].shape, 1)
    for b in range(3):
        sh = 4 << b
        low = (lane & sh) == 0
        new = list(tiles)
        for t in range(NLT):
            if not (t >> b) & 1:
                a, c = tiles[t], tiles[t | (1 << b)]
                new[t] = jnp.where(low, a, pltpu.roll(c, sh, 1))
                new[t | (1 << b)] = jnp.where(low, pltpu.roll(a, 128 - sh, 1), c)
        tiles = new
    return tiles


def _permute_cols(u):
    tiles = _swap_tiles_lanes([u[:, t * 128:(t + 1) * 128] for t in range(NLT)])
    return jnp.concatenate(tiles, axis=1)


def _pack(val):
    return pltpu.bitcast(val.astype(BF16), U32)


def _unpack(u):
    return pltpu.bitcast(u, BF16)


def _ln(x):
    m = jnp.mean(x, axis=-1, keepdims=True)
    xc = x - m
    v = jnp.mean(xc * xc, axis=-1, keepdims=True)
    return xc * lax.rsqrt(v + EPS)


def _ln_mod(x, scale1, shift):
    return _ln(x) * scale1 + shift


def _kernel(zero_ref, x_hbm, c_ref, wmod_hbm, wqkv_hbm, wo_hbm, wg_hbm, wu_hbm, wd_hbm, out_hbm,
            x_v, out_v, wmod_v, wraw_v, wqkv_v, wo_v, wg_v, wu_v, wd_v, mod_v, scb_s, h_s, q_s, k_s, v_s, o_s,
            x1_s, h2_s, act_s, sems, qsems, xsems, osems):
    n_mod = 6 * D // MC

    def mod_cp(j):
        return pltpu.make_async_copy(wmod_hbm.at[:, pl.ds(j * MC, MC)],
                                     wmod_v.at[:, pl.ds(j * MC, MC)], sems.at[j])

    def qkv_cp(k):
        rows = pl.ds(k * MC, MC)
        return pltpu.make_async_copy(wqkv_hbm.at[rows, :], wraw_v.at[rows, :], qsems.at[k])

    def x_cp(i):
        return pltpu.make_async_copy(x_hbm.at[i], x_v.at[i], xsems.at[i])

    last_cs = (pl.ds(0, D - DC), pl.ds(D - DC, DC))
    out_cps = [pltpu.make_async_copy(out_v.at[pl.ds(0, NT - 1)], out_hbm.at[pl.ds(0, NT - 1)],
                                     osems.at[0])]
    out_cps += [pltpu.make_async_copy(out_v.at[NT - 1, :, cs], out_hbm.at[NT - 1, :, cs],
                                      osems.at[1 + n]) for n, cs in enumerate(last_cs)]

    wo_cp = pltpu.make_async_copy(wo_hbm, wo_v, sems.at[n_mod + 3])
    wg_cp = pltpu.make_async_copy(wg_hbm, wg_v, sems.at[n_mod + 4])
    wu_cp = pltpu.make_async_copy(wu_hbm, wu_v, sems.at[n_mod + 5])
    wd_cp = pltpu.make_async_copy(wd_hbm, wd_v, sems.at[n_mod + 6])
    per = D // MC

    def mod_cps(k):
        return [mod_cp(j) for j in range(k * per, (k + 1) * per)]

    def start(cps):
        for cp in cps:
            cp.start()

    def mod_chunk(j):
        cf = c_ref[...].astype(F32)
        sc = jnp.broadcast_to(cf * jax.nn.sigmoid(cf), (16, D)).astype(BF16)
        r = jnp.dot(sc, wmod_v[:, j * MC:(j + 1) * MC], preferred_element_type=F32)
        if j // per in (1, 4):
            r = r + 1.0
        mod_v[:, j * MC:(j + 1) * MC] = r[0:8]

    def silu_c_columns():
        cf = c_ref[...].astype(F32)
        sc = (cf * jax.nn.sigmoid(cf)).astype(BF16).astype(F32)
        for t in range(NLT):
            blk = jnp.broadcast_to(sc[:, t * 128:(t + 1) * 128], (128, 128))
            scb_s[t * 128:(t + 1) * 128, :] = blk.T

    def mod_chunk_vpu(j):
        cs = slice(j * MC, (j + 1) * MC)
        acc = paced(jnp.zeros((AR, 128), F32))
        acc = jnp.concatenate([acc] * (MC // 128), axis=1)
        for r in range(0, D, AR):
            sc = jnp.concatenate([scb_s[r:r + AR, :]] * (MC // 128), axis=1)
            acc = acc + wmod_v[r:r + AR, cs].astype(F32) * sc
        res = jnp.sum(acc, axis=0, keepdims=True)
        if j // per in (1, 4):
            res = res + 1.0
        mod_v[:, cs] = jnp.broadcast_to(res, (8, MC))

    tokens = []

    def paced(val):
        if not tokens:
            return val
        never = lax.broadcasted_iota(jnp.int32, val.shape, 0) < zero_ref[0]
        return jnp.where(never, tokens.pop(0), val)

    def paced_rows(val):
        top = jnp.concatenate([paced(val[:AR, :128]), val[:AR, 128:]], axis=1)
        return jnp.concatenate([top, val[AR:]], axis=0) if val.shape[0] > AR else top

    def post(*results):
        tokens[:] = [res[TM - AR:TM, c:c + 128] for res in results
                     for c in range(0, res.shape[1], 256)]

    def mod(k):
        return mod_v[0:1, k * D:(k + 1) * D]

    def ln1(i, r):
        xv = paced_rows(x_v[i, r:r + LR, :].astype(F32))
        h_s[i % 2, r // 2:(r + LR) // 2, :] = _pack(_ln_mod(xv, mod(1), mod(0)))

    def ln1_norm0(r):
        x1_s[0, r:r + LR, :] = _ln(x_v[0, r:r + LR, :].astype(F32))

    def ln1_apply0(j):
        cs = slice(j * MC, (j + 1) * MC)
        h_s[0, :, cs] = _pack(x1_s[0, :, cs] * mod_v[0:1, D + j * MC:D + (j + 1) * MC]
                              + mod_v[0:1, cs])

    def prep_qkv(j, k):
        for r in range(k * MC, (k + 1) * MC, 128):
            wqkv_v[r // 2:r // 2 + 64, j * D:(j + 1) * D] = _permute_cols(
                _pack(wraw_v[r:r + 128, j * D:(j + 1) * D]))

    def qkv_first(j, k):
        res = jnp.dot(_unpack(h_s[0, :, k * MC:(k + 1) * MC]),
                      _unpack(wqkv_v[k * MC // 2:(k + 1) * MC // 2, j * D:(j + 1) * D]),
                      preferred_element_type=F32)
        post(res)
        if k > 0:
            dst, r0 = ((q_s, 0), (k_s, HALO), (v_s, HALO))[j]
            res = res + jnp.concatenate([dst[0, t, r0:r0 + TM, :] for t in range(NLT)], axis=1)
        qkv_store(0, j, 0, res, final=k == D // MC - 1)

    def qkv_part(i, j, half):
        c0 = j * D + half * QC
        res = jnp.dot(_unpack(h_s[i % 2]), _unpack(wqkv_v[:, c0:c0 + QC]),
                      preferred_element_type=F32)
        qkv_store(i, j, half, res)
        post(res)

    def qkv_store(i, j, half, res, final=True):
        sl = i % 2
        for tt in range(res.shape[1] // 128):
            t = half * (QC // 128) + tt
            blk = res[:, tt * 128:(tt + 1) * 128]
            if j == 0:
                q_s[sl, t] = blk * SCALE if final else blk
                continue
            dst = k_s if j == 1 else v_s
            dst[sl, t, HALO:HALO + TM, :] = blk
            if not final:
                continue
            if i == 0:
                dst[sl, t, 0:HALO, :] = jnp.broadcast_to(blk[0:1], (HALO, 128))
            else:
                dst[sl, t, 0:HALO, :] = dst[1 - sl, t, TM:TM + HALO, :]

    live = {}

    def window(ref, sl, t, r):
        hw = W // 2
        back = DIL * hw
        slabs = [ref[sl, t, HALO + r - DIL * w - back:HALO + r - DIL * w + AR, :]
                 for w in range(hw)]
        return [sb[back:] for sb in slabs] + [sb[:AR] for sb in slabs]

    def attn_qk(i, r):
        sl = i % 2
        lg = None
        for t in range(NLT):
            q = q_s[sl, t, r:r + AR, :]
            if t == 0:
                q = paced(q)
            prod = [q * kw for kw in window(k_s, sl, t, r)]
            lg = prod if lg is None else [a + b for a, b in zip(lg, prod)]
        live[i, r] = lg

    def attn_lanes(i, r):
        lane = lax.broadcasted_iota(jnp.int32, (AR, 128), 1)
        b0 = (lane & 1) == 0
        b1 = (lane & 2) == 0
        lg = [a + jnp.where(b0, pltpu.roll(a, 127, 1), pltpu.roll(a, 1, 1)) for a in live[i, r]]
        lg = [a + jnp.where(b1, pltpu.roll(a, 126, 1), pltpu.roll(a, 2, 1)) for a in lg]
        live[i, r] = lg

    def attn_softmax(i, r):
        lg = live[i, r]
        if i == 0 and r < DIL * (W - 1):
            row = lax.broadcasted_iota(jnp.int32, (AR, 128), 0) + r
            lg = [jnp.where(row >= DIL * w, a, -1000000000.0 * LOG2E) for w, a in enumerate(lg)]
        m = lg[0]
        for w in range(1, W):
            m = jnp.maximum(m, lg[w])
        e = [jnp.exp2(a - m) for a in lg]
        s = e[0]
        for w in range(1, W):
            s = s + e[w]
        inv = 1.0 / s
        live[i, r] = [a * inv for a in e]

    def attn_pv(i, r):
        sl = i % 2
        p = live.pop((i, r))
        outs = []
        for t in range(NLT):
            vw = window(v_s, sl, t, r)
            a = p[0] * vw[0]
            for w in range(1, W):
                a = a + p[w] * vw[w]
            outs.append(a)
        o_s[r // 2:(r + AR) // 2, :] = _pack(jnp.concatenate(outs, axis=1))

    def attn_unpermute(i, r):
        rows = slice(r // 2, (r + AR) // 2)
        o_s[rows, :] = _permute_cols(o_s[rows, :])

    def wo_part(i, r0):
        y = jnp.dot(_unpack(o_s[r0 // 2:(r0 + WR) // 2, :]), wo_v[...],
                    preferred_element_type=F32)
        for r in range(r0, r0 + WR, LR):
            x1 = x_v[i, r:r + LR, :].astype(F32) + mod(2) * y[r - r0:r - r0 + LR]
            x1_s[i % 2, r:r + LR, :] = x1
            h2_s[r // 2:(r + LR) // 2, :] = _pack(_ln_mod(x1, mod(4), mod(3)))

    def gate_up(cix):
        cs = slice(cix * FC, (cix + 1) * FC)
        h2 = _unpack(h2_s[...])
        g = jnp.dot(h2, wg_v[:, cs], preferred_element_type=F32)
        u = jnp.dot(h2, wu_v[:, cs], preferred_element_type=F32)
        post(g, u)
        t = 0.5 * g
        act_s[:, cs] = _pack((t + t * jnp.tanh(t)) * u)

    def down(i, n):
        cs = slice(n * DC, (n + 1) * DC)
        y = jnp.dot(_unpack(act_s[...]), wd_v[:, cs], preferred_element_type=F32)
        post(y)
        gb = mod_v[0:1, 5 * D + n * DC:5 * D + (n + 1) * DC]
        out_v[i, :, cs] = (x1_s[i % 2, :, cs] + gb * y).astype(out_v.dtype)

    def par(mxu, vpu):
        done = 0
        for idx, (fn, *args) in enumerate(mxu):
            upto = len(vpu) * (idx + 1) // len(mxu)
            for vfn, *vargs in vpu[done:upto]:
                vfn(*vargs)
            done = upto
            fn(*args)

    halves = range(D // QC)

    def t_qkv(i, js=(0, 1, 2)):
        return [(qkv_part, i, j, hf) for j in js for hf in halves]

    def t_attn(i):
        stages = (attn_qk, attn_lanes, attn_softmax, attn_pv, attn_unpermute)[:NSTAGE]
        nb = TM // AR
        return [(fn, i, (n - k * SKEW) * AR) for n in range(nb + (len(stages) - 1) * SKEW)
                for k, fn in reversed(list(enumerate(stages))) if 0 <= n - k * SKEW < nb]

    def t_ln(fn, i):
        return [(fn, i, r) for r in range(0, TM, LR)] if i < NT else []

    def t_wo(i):
        return [(wo_part, i, r) for r in range(0, TM, WR)]

    t_gu = [(gate_up, cix) for cix in range(NFC)]

    def t_down(i, ns):
        return [(down, i, n) for n in ns]

    def t_mod(ks):
        return [(mod_chunk_vpu, j) for k in ks for j in range(k * per, (k + 1) * per)]

    def wait(cps):
        for cp in cps:
            cp.wait()

    def chunk_cps(k):
        return [mod_cp(k), mod_cp(per + k), qkv_cp(k)]

    def modulate0(k):
        mod_chunk(k)
        mod_chunk(per + k)
        ln1_apply0(k)

    start([x_cp(0)] + chunk_cps(0))
    silu_c_columns()
    x_cp(0).wait()
    par([(ln1_norm0, r) for r in range(0, TM, LR)], [])
    wait(chunk_cps(0)[:2])
    start(chunk_cps(1))
    modulate0(0)
    qkv_cp(0).wait()
    start(chunk_cps(2))
    prep_qkv(0, 0)
    x_next = [x_cp(1), x_cp(2)]
    arrive = [chunk_cps(k) for k in range(per)]
    arrive[-1] += x_next
    later = arrive[3:] + [mod_cps(2) + [wo_cp], mod_cps(3) + mod_cps(4) + mod_cps(5)]
    steps = [(j, k) for k in range(per) for j in range(3)]
    ln_next = t_ln(ln1, 1)
    for n, (j, k) in enumerate(steps):
        if j == 2 and k + 1 < per:
            wait(arrive[k + 1])
            start(later[k])
            modulate0(k + 1)
        if n + 1 < len(steps):
            prep_qkv(*steps[n + 1])
        if n + 2 >= len(steps):
            half = len(ln_next) // 2
            par(ln_next[:half] if n + 2 == len(steps) else ln_next[half:], [])
        qkv_first(j, k)
    start([wg_cp])
    par(t_qkv(1), t_attn(0) + t_ln(ln1, 2))
    wait(mod_cps(2) + mod_cps(3) + mod_cps(4) + mod_cps(5) + [wo_cp])
    x_rest = [x_cp(i) for i in range(3, NT)]
    start([wu_cp])
    q2 = t_qkv(2)
    par(q2[:-1], t_mod((2, 3, 4)))
    start([wd_cp] + x_rest)
    par(t_wo(0), [])
    par(q2[-1:], [])
    wait([wg_cp, wu_cp])
    first, second = range(N_D1), range(N_D1, NDC)
    for i in range(1, NT):
        att = t_attn(i)
        par(t_gu, att[:N_GU] + (t_mod((5,)) if i == 1 else []))
        if i == 1:
            wait([wd_cp] + x_rest)
        par(t_down(i - 1, first), att[N_GU:] + t_ln(ln1, i + 2))
        par(t_wo(i), [])
        par(t_down(i - 1, second), [])
        if i + 2 < NT:
            par(t_qkv(i + 2), [])
        pass
    out_cps[0].start()
    par(t_gu, [])
    par(t_down(NT - 1, range(NDC - 1)), [])
    out_cps[1].start()
    down(NT - 1, NDC - 1)
    out_cps[2].start()
    wait(out_cps)


@jax.jit
def pallas_adaLN_cond__sliding_local_dilated__swiglu_ffn__prompt_kernel(
    A_x: jax.Array,
    A_wqkv: jax.Array,
    A_wo: jax.Array,
    B_x: jax.Array,
    B_w_gate: jax.Array,
    B_w_up: jax.Array,
    B_w_down: jax.Array,
    c: jax.Array,
    w_mod: jax.Array,
):
    del B_x
    x = A_x.reshape(NT, TM, D)
    hbm = pl.BlockSpec(memory_space=pl.ANY)
    out = pl.pallas_call(
        _kernel,
        in_specs=[pl.BlockSpec(memory_space=pltpu.SMEM), hbm, pl.BlockSpec(memory_space=pltpu.VMEM), hbm, hbm, hbm, hbm, hbm, hbm],
        out_specs=hbm,
        out_shape=jax.ShapeDtypeStruct((NT, TM, D), A_x.dtype),
        scratch_shapes=[
            pltpu.VMEM((NT, TM, D), BF16),
            pltpu.VMEM((NT, TM, D), BF16),
            pltpu.VMEM((D, 6 * D), BF16),
            pltpu.VMEM((D, 3 * D), BF16),
            pltpu.VMEM((D // 2, 3 * D), U32),
            pltpu.VMEM((D, D), BF16),
            pltpu.VMEM((D, F), BF16),
            pltpu.VMEM((D, F), BF16),
            pltpu.VMEM((F, D), BF16),
            pltpu.VMEM((8, 6 * D), F32),
            pltpu.VMEM((D, 128), F32),
            pltpu.VMEM((2, TM // 2, D), U32),
            pltpu.VMEM((2, NLT, TM, 128), F32),
            pltpu.VMEM((2, NLT, HALO + TM, 128), F32),
            pltpu.VMEM((2, NLT, HALO + TM, 128), F32),
            pltpu.VMEM((TM // 2, D), U32),
            pltpu.VMEM((2, TM, D), F32),
            pltpu.VMEM((TM // 2, D), U32),
            pltpu.VMEM((TM // 2, F), U32),
            pltpu.SemaphoreType.DMA((6 * D // MC + 7,)),
            pltpu.SemaphoreType.DMA((D // MC,)),
            pltpu.SemaphoreType.DMA((NT,)),
            pltpu.SemaphoreType.DMA((3,)),
        ],
        compiler_params=pltpu.CompilerParams(
            vmem_limit_bytes=110 * 1024 * 1024,
        ),
    )(np.zeros((1,), np.int32), x, c, w_mod, A_wqkv, A_wo, B_w_gate, B_w_up, B_w_down)
    return out.reshape(A_x.shape)


def _rederive():
    global NT, NFC, NDC
    NT, NFC, NDC = S // TM, F // FC, D // DC
```

```python
import jax
import jax.numpy as jnp
import numpy as np
from jax import lax
from jax.experimental import pallas as pl
from jax.experimental.pallas import tpu as pltpu

S, D, F = 2048, 1024, 3584
H, DH, W, DIL = 32, 32, 8, 2
TM = 512
NT = S // TM
HALO = 16
FC = 512
NFC = F // FC
DC = 256
NDC = D // DC
AR = 16
LR = 16
MC = 256
NLT = D // 128
QC = 512
WR = 256
N_D1 = 3
NSTAGE = 5
SKEW = 1
N_GU = 160
EPS = 1e-5
LOG2E = 1.4426950408889634
SCALE = DH ** -0.5 * LOG2E
F32, BF16, U32 = jnp.float32, jnp.bfloat16, jnp.uint32


def _swap_tiles_lanes(tiles):
    lane = lax.broadcasted_iota(jnp.int32, tiles[0].shape, 1)
    for b in range(3):
        sh = 4 << b
        low = (lane & sh) == 0
        new = list(tiles)
        for t in range(NLT):
            if not (t >> b) & 1:
                a, c = tiles[t], tiles[t | (1 << b)]
                new[t] = jnp.where(low, a, pltpu.roll(c, sh, 1))
                new[t | (1 << b)] = jnp.where(low, pltpu.roll(a, 128 - sh, 1), c)
        tiles = new
    return tiles


def _permute_cols(u):
    tiles = _swap_tiles_lanes([u[:, t * 128:(t + 1) * 128] for t in range(NLT)])
    return jnp.concatenate(tiles, axis=1)


def _pack(val):
    return pltpu.bitcast(val.astype(BF16), U32)


def _unpack(u):
    return pltpu.bitcast(u, BF16)


def _ln(x):
    m = jnp.mean(x, axis=-1, keepdims=True)
    xc = x - m
    v = jnp.mean(xc * xc, axis=-1, keepdims=True)
    return xc * lax.rsqrt(v + EPS)


def _ln_mod(x, scale1, shift):
    return _ln(x) * scale1 + shift


def _kernel(zero_hbm, x_hbm, c_hbm, wmod_hbm, wqkv_hbm, wo_hbm, wg_hbm, wu_hbm, wd_hbm, out_hbm,
            zero_v, c_v, x_v, out_v, wmod_v, wraw_v, wqkv_v, wo_v, wg_v, wu_v, wd_v, mod_v, scb_s, h_s, q_s, k_s, v_s, o_s,
            x1_s, h2_s, act_s, sems, qsems, xsems, osems):
    n_mod = 6 * D // MC

    def mod_cp(j):
        return pltpu.make_async_copy(wmod_hbm.at[:, pl.ds(j * MC, MC)],
                                     wmod_v.at[:, pl.ds(j * MC, MC)], sems.at[j])

    def qkv_cp(k):
        rows = pl.ds(k * MC, MC)
        return pltpu.make_async_copy(wqkv_hbm.at[rows, :], wraw_v.at[rows, :], qsems.at[k])

    def x_cp(i):
        return pltpu.make_async_copy(x_hbm.at[i], x_v.at[i], xsems.at[i])

    last_cs = (pl.ds(0, D - DC), pl.ds(D - DC, DC))
    out_cps = [pltpu.make_async_copy(out_v.at[pl.ds(0, NT - 1)], out_hbm.at[pl.ds(0, NT - 1)],
                                     osems.at[0])]
    out_cps += [pltpu.make_async_copy(out_v.at[NT - 1, :, cs], out_hbm.at[NT - 1, :, cs],
                                      osems.at[1 + n]) for n, cs in enumerate(last_cs)]

    wo_cp = pltpu.make_async_copy(wo_hbm, wo_v, sems.at[n_mod + 3])
    wg_cp = pltpu.make_async_copy(wg_hbm, wg_v, sems.at[n_mod + 4])
    wu_cp = pltpu.make_async_copy(wu_hbm, wu_v, sems.at[n_mod + 5])
    wd_cp = pltpu.make_async_copy(wd_hbm, wd_v, sems.at[n_mod + 6])
    small_cps = [pltpu.make_async_copy(c_hbm, c_v, sems.at[n_mod + 7]),
                 pltpu.make_async_copy(zero_hbm, zero_v, sems.at[n_mod + 8])]
    per = D // MC

    def mod_cps(k):
        return [mod_cp(j) for j in range(k * per, (k + 1) * per)]

    def start(cps):
        for cp in cps:
            cp.start()

    def mod_chunk(j):
        cf = c_v[...].astype(F32)
        sc = jnp.broadcast_to(cf * jax.nn.sigmoid(cf), (16, D)).astype(BF16)
        r = jnp.dot(sc, wmod_v[:, j * MC:(j + 1) * MC], preferred_element_type=F32)
        if j // per in (1, 4):
            r = r + 1.0
        mod_v[:, j * MC:(j + 1) * MC] = r[0:8]

    def silu_c_columns():
        cf = c_v[...].astype(F32)
        sc = (cf * jax.nn.sigmoid(cf)).astype(BF16).astype(F32)
        for t in range(NLT):
            blk = jnp.broadcast_to(sc[:, t * 128:(t + 1) * 128], (128, 128))
            scb_s[t * 128:(t + 1) * 128, :] = blk.T

    def mod_chunk_vpu(j):
        cs = slice(j * MC, (j + 1) * MC)
        acc = paced(jnp.zeros((AR, 128), F32))
        acc = jnp.concatenate([acc] * (MC // 128), axis=1)
        for r in range(0, D, AR):
            sc = jnp.concatenate([scb_s[r:r + AR, :]] * (MC // 128), axis=1)
            acc = acc + wmod_v[r:r + AR, cs].astype(F32) * sc
        res = jnp.sum(acc, axis=0, keepdims=True)
        if j // per in (1, 4):
            res = res + 1.0
        mod_v[:, cs] = jnp.broadcast_to(res, (8, MC))

    tokens = []

    def paced(val):
        if not tokens:
            return val
        never = zero_v[...] != 0
        return jnp.where(never, tokens.pop(0), val)

    def paced_rows(val):
        top = jnp.concatenate([paced(val[:AR, :128]), val[:AR, 128:]], axis=1)
        return jnp.concatenate([top, val[AR:]], axis=0) if val.shape[0] > AR else top

    def post(*results):
        tokens[:] = [res[TM - AR:TM, c:c + 128] for res in results
                     for c in range(0, res.shape[1], 256)]

    def mod(k):
        return mod_v[0:1, k * D:(k + 1) * D]

    def ln1(i, r):
        xv = paced_rows(x_v[i, r:r + LR, :].astype(F32))
        h_s[i % 2, r // 2:(r + LR) // 2, :] = _pack(_ln_mod(xv, mod(1), mod(0)))

    def ln1_norm0(r):
        x1_s[0, r:r + LR, :] = _ln(x_v[0, r:r + LR, :].astype(F32))

    def ln1_apply0(j):
        cs = slice(j * MC, (j + 1) * MC)
        h_s[0, :, cs] = _pack(x1_s[0, :, cs] * mod_v[0:1, D + j * MC:D + (j + 1) * MC]
                              + mod_v[0:1, cs])

    def prep_qkv(j, k):
        for r in range(k * MC, (k + 1) * MC, 128):
            wqkv_v[r // 2:r // 2 + 64, j * D:(j + 1) * D] = _permute_cols(
                _pack(wraw_v[r:r + 128, j * D:(j + 1) * D]))

    def qkv_first(j, k):
        res = jnp.dot(_unpack(h_s[0, :, k * MC:(k + 1) * MC]),
                      _unpack(wqkv_v[k * MC // 2:(k + 1) * MC // 2, j * D:(j + 1) * D]),
                      preferred_element_type=F32)
        post(res)
        if k > 0:
            dst, r0 = ((q_s, 0), (k_s, HALO), (v_s, HALO))[j]
            res = res + jnp.concatenate([dst[0, t, r0:r0 + TM, :] for t in range(NLT)], axis=1)
        qkv_store(0, j, 0, res, final=k == D // MC - 1)

    def qkv_part(i, j, half):
        c0 = j * D + half * QC
        res = jnp.dot(_unpack(h_s[i % 2]), _unpack(wqkv_v[:, c0:c0 + QC]),
                      preferred_element_type=F32)
        qkv_store(i, j, half, res)
        post(res)

    def qkv_store(i, j, half, res, final=True):
        sl = i % 2
        for tt in range(res.shape[1] // 128):
            t = half * (QC // 128) + tt
            blk = res[:, tt * 128:(tt + 1) * 128]
            if j == 0:
                q_s[sl, t] = blk * SCALE if final else blk
                continue
            dst = k_s if j == 1 else v_s
            dst[sl, t, HALO:HALO + TM, :] = blk
            if not final:
                continue
            if i == 0:
                dst[sl, t, 0:HALO, :] = jnp.broadcast_to(blk[0:1], (HALO, 128))
            else:
                dst[sl, t, 0:HALO, :] = dst[1 - sl, t, TM:TM + HALO, :]

    live = {}

    def window(ref, sl, t, r):
        hw = W // 2
        back = DIL * hw
        slabs = [ref[sl, t, HALO + r - DIL * w - back:HALO + r - DIL * w + AR, :]
                 for w in range(hw)]
        return [sb[back:] for sb in slabs] + [sb[:AR] for sb in slabs]

    def attn_qk(i, r):
        sl = i % 2
        lg = None
        for t in range(NLT):
            q = q_s[sl, t, r:r + AR, :]
            if t == 0:
                q = paced(q)
            prod = [q * kw for kw in window(k_s, sl, t, r)]
            lg = prod if lg is None else [a + b for a, b in zip(lg, prod)]
        live[i, r] = lg

    def attn_lanes(i, r):
        lane = lax.broadcasted_iota(jnp.int32, (AR, 128), 1)
        b0 = (lane & 1) == 0
        b1 = (lane & 2) == 0
        lg = [a + jnp.where(b0, pltpu.roll(a, 127, 1), pltpu.roll(a, 1, 1)) for a in live[i, r]]
        lg = [a + jnp.where(b1, pltpu.roll(a, 126, 1), pltpu.roll(a, 2, 1)) for a in lg]
        live[i, r] = lg

    def attn_softmax(i, r):
        lg = live[i, r]
        if i == 0 and r < DIL * (W - 1):
            row = lax.broadcasted_iota(jnp.int32, (AR, 128), 0) + r
            lg = [jnp.where(row >= DIL * w, a, -1000000000.0 * LOG2E) for w, a in enumerate(lg)]
        m = lg[0]
        for w in range(1, W):
            m = jnp.maximum(m, lg[w])
        e = [jnp.exp2(a - m) for a in lg]
        s = e[0]
        for w in range(1, W):
            s = s + e[w]
        inv = 1.0 / s
        live[i, r] = [a * inv for a in e]

    def attn_pv(i, r):
        sl = i % 2
        p = live.pop((i, r))
        outs = []
        for t in range(NLT):
            vw = window(v_s, sl, t, r)
            a = p[0] * vw[0]
            for w in range(1, W):
                a = a + p[w] * vw[w]
            outs.append(a)
        o_s[r // 2:(r + AR) // 2, :] = _pack(jnp.concatenate(outs, axis=1))

    def attn_unpermute(i, r):
        rows = slice(r // 2, (r + AR) // 2)
        o_s[rows, :] = _permute_cols(o_s[rows, :])

    def wo_part(i, r0):
        y = jnp.dot(_unpack(o_s[r0 // 2:(r0 + WR) // 2, :]), wo_v[...],
                    preferred_element_type=F32)
        for r in range(r0, r0 + WR, LR):
            x1 = x_v[i, r:r + LR, :].astype(F32) + mod(2) * y[r - r0:r - r0 + LR]
            x1_s[i % 2, r:r + LR, :] = x1
            h2_s[r // 2:(r + LR) // 2, :] = _pack(_ln_mod(x1, mod(4), mod(3)))

    def gate_up(cix):
        cs = slice(cix * FC, (cix + 1) * FC)
        h2 = _unpack(h2_s[...])
        g = jnp.dot(h2, wg_v[:, cs], preferred_element_type=F32)
        u = jnp.dot(h2, wu_v[:, cs], preferred_element_type=F32)
        post(g, u)
        t = 0.5 * g
        act_s[:, cs] = _pack((t + t * jnp.tanh(t)) * u)

    def down(i, n):
        cs = slice(n * DC, (n + 1) * DC)
        y = jnp.dot(_unpack(act_s[...]), wd_v[:, cs], preferred_element_type=F32)
        post(y)
        gb = mod_v[0:1, 5 * D + n * DC:5 * D + (n + 1) * DC]
        out_v[i, :, cs] = (x1_s[i % 2, :, cs] + gb * y).astype(out_v.dtype)

    def par(mxu, vpu):
        done = 0
        for idx, (fn, *args) in enumerate(mxu):
            upto = len(vpu) * (idx + 1) // len(mxu)
            for vfn, *vargs in vpu[done:upto]:
                vfn(*vargs)
            done = upto
            fn(*args)

    halves = range(D // QC)

    def t_qkv(i, js=(0, 1, 2)):
        return [(qkv_part, i, j, hf) for j in js for hf in halves]

    def t_attn(i):
        stages = (attn_qk, attn_lanes, attn_softmax, attn_pv, attn_unpermute)[:NSTAGE]
        nb = TM // AR
        return [(fn, i, (n - k * SKEW) * AR) for n in range(nb + (len(stages) - 1) * SKEW)
                for k, fn in reversed(list(enumerate(stages))) if 0 <= n - k * SKEW < nb]

    def t_ln(fn, i):
        return [(fn, i, r) for r in range(0, TM, LR)] if i < NT else []

    def t_wo(i):
        return [(wo_part, i, r) for r in range(0, TM, WR)]

    t_gu = [(gate_up, cix) for cix in range(NFC)]

    def t_down(i, ns):
        return [(down, i, n) for n in ns]

    def t_mod(ks):
        return [(mod_chunk_vpu, j) for k in ks for j in range(k * per, (k + 1) * per)]

    def wait(cps):
        for cp in cps:
            cp.wait()

    def chunk_cps(k):
        return [mod_cp(k), mod_cp(per + k), qkv_cp(k)]

    def modulate0(k):
        mod_chunk(k)
        mod_chunk(per + k)
        ln1_apply0(k)

    start(small_cps + [x_cp(0)] + chunk_cps(0))
    wait(small_cps)
    silu_c_columns()
    x_cp(0).wait()
    par([(ln1_norm0, r) for r in range(0, TM, LR)], [])
    wait(chunk_cps(0)[:2])
    start(chunk_cps(1))
    modulate0(0)
    qkv_cp(0).wait()
    start(chunk_cps(2))
    prep_qkv(0, 0)
    x_next = [x_cp(1), x_cp(2)]
    arrive = [chunk_cps(k) for k in range(per)]
    arrive[-1] += x_next
    later = arrive[3:] + [mod_cps(2) + [wo_cp], mod_cps(3) + mod_cps(4) + mod_cps(5)]
    steps = [(j, k) for k in range(per) for j in range(3)]
    ln_next = t_ln(ln1, 1)
    for n, (j, k) in enumerate(steps):
        if j == 2 and k + 1 < per:
            wait(arrive[k + 1])
            start(later[k])
            modulate0(k + 1)
        if n + 1 < len(steps):
            prep_qkv(*steps[n + 1])
        if n + 2 >= len(steps):
            half = len(ln_next) // 2
            par(ln_next[:half] if n + 2 == len(steps) else ln_next[half:], [])
        qkv_first(j, k)
    start([wg_cp])
    par(t_qkv(1), t_attn(0) + t_ln(ln1, 2))
    wait(mod_cps(2) + mod_cps(3) + mod_cps(4) + mod_cps(5) + [wo_cp])
    x_rest = [x_cp(i) for i in range(3, NT)]
    start([wu_cp])
    q2 = t_qkv(2)
    par(q2[:-1], t_mod((2, 3, 4)))
    start([wd_cp] + x_rest)
    par(t_wo(0), [])
    par(q2[-1:], [])
    wait([wg_cp, wu_cp])
    first, second = range(N_D1), range(N_D1, NDC)
    for i in range(1, NT):
        att = t_attn(i)
        par(t_gu, att[:N_GU] + (t_mod((5,)) if i == 1 else []))
        if i == 1:
            wait([wd_cp] + x_rest)
        par(t_down(i - 1, first), att[N_GU:] + t_ln(ln1, i + 2))
        par(t_wo(i), [])
        par(t_down(i - 1, second), [])
        if i + 2 < NT:
            par(t_qkv(i + 2), [])
        pass
    out_cps[0].start()
    par(t_gu, [])
    par(t_down(NT - 1, range(NDC - 1)), [])
    out_cps[1].start()
    down(NT - 1, NDC - 1)
    out_cps[2].start()
    wait(out_cps)


@jax.jit
def pallas_adaLN_cond__sliding_local_dilated__swiglu_ffn__prompt_kernel(
    A_x: jax.Array,
    A_wqkv: jax.Array,
    A_wo: jax.Array,
    B_x: jax.Array,
    B_w_gate: jax.Array,
    B_w_up: jax.Array,
    B_w_down: jax.Array,
    c: jax.Array,
    w_mod: jax.Array,
):
    del B_x
    x = A_x.reshape(NT, TM, D)
    hbm = pl.BlockSpec(memory_space=pl.ANY)
    out = pl.pallas_call(
        _kernel,
        in_specs=[hbm] * 9,
        out_specs=hbm,
        out_shape=jax.ShapeDtypeStruct((NT, TM, D), A_x.dtype),
        scratch_shapes=[
            pltpu.VMEM((AR, 128), jnp.int32),
            pltpu.VMEM((1, D), BF16),
            pltpu.VMEM((NT, TM, D), BF16),
            pltpu.VMEM((NT, TM, D), BF16),
            pltpu.VMEM((D, 6 * D), BF16),
            pltpu.VMEM((D, 3 * D), BF16),
            pltpu.VMEM((D // 2, 3 * D), U32),
            pltpu.VMEM((D, D), BF16),
            pltpu.VMEM((D, F), BF16),
            pltpu.VMEM((D, F), BF16),
            pltpu.VMEM((F, D), BF16),
            pltpu.VMEM((8, 6 * D), F32),
            pltpu.VMEM((D, 128), F32),
            pltpu.VMEM((2, TM // 2, D), U32),
            pltpu.VMEM((2, NLT, TM, 128), F32),
            pltpu.VMEM((2, NLT, HALO + TM, 128), F32),
            pltpu.VMEM((2, NLT, HALO + TM, 128), F32),
            pltpu.VMEM((TM // 2, D), U32),
            pltpu.VMEM((2, TM, D), F32),
            pltpu.VMEM((TM // 2, D), U32),
            pltpu.VMEM((TM // 2, F), U32),
            pltpu.SemaphoreType.DMA((6 * D // MC + 9,)),
            pltpu.SemaphoreType.DMA((D // MC,)),
            pltpu.SemaphoreType.DMA((NT,)),
            pltpu.SemaphoreType.DMA((3,)),
        ],
        compiler_params=pltpu.CompilerParams(
            vmem_limit_bytes=110 * 1024 * 1024,
        ),
    )(np.zeros((AR, 128), np.int32), x, c, w_mod, A_wqkv, A_wo, B_w_gate, B_w_up, B_w_down)
    return out.reshape(A_x.shape)


def _rederive():
    global NT, NFC, NDC
    NT, NFC, NDC = S // TM, F // FC, D // DC
```

```python
import jax
import jax.numpy as jnp
import numpy as np
from jax import lax
from jax.experimental import pallas as pl
from jax.experimental.pallas import tpu as pltpu

S, D, F = 2048, 1024, 3584
H, DH, W, DIL = 32, 32, 8, 2
TM = 512
NT = S // TM
HALO = 16
FC = 512
NFC = F // FC
DC = 256
NDC = D // DC
AR = 16
LR = 16
MC = 256
NLT = D // 128
QC = 512
WR = 256
N_D1 = 3
V = 0
SKEW = 1
N_GU = 160
EPS = 1e-5
LOG2E = 1.4426950408889634
SCALE = DH ** -0.5 * LOG2E
F32, BF16, U32 = jnp.float32, jnp.bfloat16, jnp.uint32


def _swap_tiles_lanes(tiles):
    lane = lax.broadcasted_iota(jnp.int32, tiles[0].shape, 1)
    for b in range(3):
        sh = 4 << b
        low = (lane & sh) == 0
        new = list(tiles)
        for t in range(NLT):
            if not (t >> b) & 1:
                a, c = tiles[t], tiles[t | (1 << b)]
                new[t] = jnp.where(low, a, pltpu.roll(c, sh, 1))
                new[t | (1 << b)] = jnp.where(low, pltpu.roll(a, 128 - sh, 1), c)
        tiles = new
    return tiles


def _permute_cols(u):
    tiles = _swap_tiles_lanes([u[:, t * 128:(t + 1) * 128] for t in range(NLT)])
    return jnp.concatenate(tiles, axis=1)


def _pack(val):
    return pltpu.bitcast(val.astype(BF16), U32)


def _unpack(u):
    return pltpu.bitcast(u, BF16)


def _ln(x):
    m = jnp.mean(x, axis=-1, keepdims=True)
    xc = x - m
    v = jnp.mean(xc * xc, axis=-1, keepdims=True)
    return xc * lax.rsqrt(v + EPS)


def _ln_mod(x, scale1, shift):
    return _ln(x) * scale1 + shift


def _kernel(zero_hbm, x_hbm, c_hbm, wmod_hbm, wqkv_hbm, wo_hbm, wg_hbm, wu_hbm, wd_hbm, out_hbm,
            zero_v, c_v, x_v, out_v, wmod_v, wraw_v, wqkv_v, wo_v, wg_v, wu_v, wd_v, mod_v, scb_s, h_s, q_s, k_s, v_s, o_s,
            x1_s, h2_s, act_s, sems, qsems, xsems, osems):
    n_mod = 6 * D // MC

    def mod_cp(j):
        return pltpu.make_async_copy(wmod_hbm.at[:, pl.ds(j * MC, MC)],
                                     wmod_v.at[:, pl.ds(j * MC, MC)], sems.at[j])

    def qkv_cp(k):
        blk = (pl.ds(k * MC, MC), pl.ds(0, 3 * D if k else D))
        return pltpu.make_async_copy(wqkv_hbm.at[blk], wraw_v.at[blk], qsems.at[k])

    kv0 = (pl.ds(0, MC), pl.ds(D, 2 * D))
    kv0_cp = pltpu.make_async_copy(wqkv_hbm.at[kv0], wraw_v.at[kv0], qsems.at[D // MC])

    def x_cp(i):
        return pltpu.make_async_copy(x_hbm.at[i], x_v.at[i], xsems.at[i])

    last_cs = (pl.ds(0, D - DC), pl.ds(D - DC, DC))
    out_cps = [pltpu.make_async_copy(out_v.at[pl.ds(0, NT - 1)], out_hbm.at[pl.ds(0, NT - 1)],
                                     osems.at[0])]
    out_cps += [pltpu.make_async_copy(out_v.at[NT - 1, :, cs], out_hbm.at[NT - 1, :, cs],
                                      osems.at[1 + n]) for n, cs in enumerate(last_cs)]

    wo_cp = pltpu.make_async_copy(wo_hbm, wo_v, sems.at[n_mod + 3])
    wg_cp = pltpu.make_async_copy(wg_hbm, wg_v, sems.at[n_mod + 4])
    wu_cp = pltpu.make_async_copy(wu_hbm, wu_v, sems.at[n_mod + 5])
    wd_cp = pltpu.make_async_copy(wd_hbm, wd_v, sems.at[n_mod + 6])
    small_cps = [pltpu.make_async_copy(c_hbm, c_v, sems.at[n_mod + 7]),
                 pltpu.make_async_copy(zero_hbm, zero_v, sems.at[n_mod + 8])]
    per = D // MC

    def mod_cps(k):
        return [mod_cp(j) for j in range(k * per, (k + 1) * per)]

    def start(cps):
        for cp in cps:
            cp.start()

    def mod_chunk(j):
        cf = c_v[...].astype(F32)
        sc = jnp.broadcast_to(cf * jax.nn.sigmoid(cf), (16, D)).astype(BF16)
        r = jnp.dot(sc, wmod_v[:, j * MC:(j + 1) * MC], preferred_element_type=F32)
        if j // per in (1, 4):
            r = r + 1.0
        mod_v[:, j * MC:(j + 1) * MC] = r[0:8]

    def silu_c_columns():
        cf = c_v[...].astype(F32)
        sc = (cf * jax.nn.sigmoid(cf)).astype(BF16).astype(F32)
        for t in range(NLT):
            blk = jnp.broadcast_to(sc[:, t * 128:(t + 1) * 128], (128, 128))
            scb_s[t * 128:(t + 1) * 128, :] = blk.T

    def mod_chunk_vpu(j):
        cs = slice(j * MC, (j + 1) * MC)
        acc = paced(jnp.zeros((AR, 128), F32))
        acc = jnp.concatenate([acc] * (MC // 128), axis=1)
        for r in range(0, D, AR):
            sc = jnp.concatenate([scb_s[r:r + AR, :]] * (MC // 128), axis=1)
            acc = acc + wmod_v[r:r + AR, cs].astype(F32) * sc
        res = jnp.sum(acc, axis=0, keepdims=True)
        if j // per in (1, 4):
            res = res + 1.0
        mod_v[:, cs] = jnp.broadcast_to(res, (8, MC))

    tokens = []

    def paced(val):
        if not tokens:
            return val
        never = zero_v[...] != 0
        return jnp.where(never, tokens.pop(0), val)

    def paced_rows(val):
        top = jnp.concatenate([paced(val[:AR, :128]), val[:AR, 128:]], axis=1)
        return jnp.concatenate([top, val[AR:]], axis=0) if val.shape[0] > AR else top

    def post(*results):
        tokens[:] = [res[TM - AR:TM, c:c + 128] for res in results
                     for c in range(0, res.shape[1], 256)]

    def mod(k):
        return mod_v[0:1, k * D:(k + 1) * D]

    def ln1(i, r):
        xv = paced_rows(x_v[i, r:r + LR, :].astype(F32))
        h_s[i % 2, r // 2:(r + LR) // 2, :] = _pack(_ln_mod(xv, mod(1), mod(0)))

    def ln1_norm0(r):
        x1_s[0, r:r + LR, :] = _ln(x_v[0, r:r + LR, :].astype(F32))

    def ln1_apply0(j):
        cs = slice(j * MC, (j + 1) * MC)
        h_s[0, :, cs] = _pack(x1_s[0, :, cs] * mod_v[0:1, D + j * MC:D + (j + 1) * MC]
                              + mod_v[0:1, cs])

    def prep_qkv(j, k):
        for r in range(k * MC, (k + 1) * MC, 128):
            wqkv_v[r // 2:r // 2 + 64, j * D:(j + 1) * D] = _permute_cols(
                _pack(wraw_v[r:r + 128, j * D:(j + 1) * D]))

    def qkv_first(j, k):
        res = jnp.dot(_unpack(h_s[0, :, k * MC:(k + 1) * MC]),
                      _unpack(wqkv_v[k * MC // 2:(k + 1) * MC // 2, j * D:(j + 1) * D]),
                      preferred_element_type=F32)
        post(res)
        if k > 0:
            dst, r0 = ((q_s, 0), (k_s, HALO), (v_s, HALO))[j]
            res = res + jnp.concatenate([dst[0, t, r0:r0 + TM, :] for t in range(NLT)], axis=1)
        qkv_store(0, j, 0, res, final=k == D // MC - 1)

    def qkv_part(i, j, half):
        c0 = j * D + half * QC
        res = jnp.dot(_unpack(h_s[i % 2]), _unpack(wqkv_v[:, c0:c0 + QC]),
                      preferred_element_type=F32)
        qkv_store(i, j, half, res)
        post(res)

    def qkv_store(i, j, half, res, final=True):
        sl = i % 2
        for tt in range(res.shape[1] // 128):
            t = half * (QC // 128) + tt
            blk = res[:, tt * 128:(tt + 1) * 128]
            if j == 0:
                q_s[sl, t] = blk * SCALE if final else blk
                continue
            dst = k_s if j == 1 else v_s
            dst[sl, t, HALO:HALO + TM, :] = blk
            if not final:
                continue
            if i == 0:
                dst[sl, t, 0:HALO, :] = jnp.broadcast_to(blk[0:1], (HALO, 128))
            else:
                dst[sl, t, 0:HALO, :] = dst[1 - sl, t, TM:TM + HALO, :]

    live = {}

    def window(ref, sl, t, r):
        hw = W // 2
        back = DIL * hw
        slabs = [ref[sl, t, HALO + r - DIL * w - back:HALO + r - DIL * w + AR, :]
                 for w in range(hw)]
        return [sb[back:] for sb in slabs] + [sb[:AR] for sb in slabs]

    def attn_qk(i, r):
        sl = i % 2
        lg = None
        for t in range(NLT):
            q = q_s[sl, t, r:r + AR, :]
            if t == 0:
                q = paced(q)
            prod = [q * kw for kw in window(k_s, sl, t, r)]
            lg = prod if lg is None else [a + b for a, b in zip(lg, prod)]
        live[i, r] = lg

    def attn_lanes(i, r):
        lane = lax.broadcasted_iota(jnp.int32, (AR, 128), 1)
        b0 = (lane & 1) == 0
        b1 = (lane & 2) == 0
        lg = [a + jnp.where(b0, pltpu.roll(a, 127, 1), pltpu.roll(a, 1, 1)) for a in live[i, r]]
        lg = [a + jnp.where(b1, pltpu.roll(a, 126, 1), pltpu.roll(a, 2, 1)) for a in lg]
        live[i, r] = lg

    def attn_softmax(i, r):
        lg = live[i, r]
        if i == 0 and r < DIL * (W - 1):
            row = lax.broadcasted_iota(jnp.int32, (AR, 128), 0) + r
            lg = [jnp.where(row >= DIL * w, a, -1000000000.0 * LOG2E) for w, a in enumerate(lg)]
        m = lg[0]
        for w in range(1, W):
            m = jnp.maximum(m, lg[w])
        e = [jnp.exp2(a - m) for a in lg]
        s = e[0]
        for w in range(1, W):
            s = s + e[w]
        inv = 1.0 / s
        live[i, r] = [a * inv for a in e]

    def attn_pv(i, r):
        sl = i % 2
        p = live.pop((i, r))
        outs = []
        for t in range(NLT):
            vw = window(v_s, sl, t, r)
            a = p[0] * vw[0]
            for w in range(1, W):
                a = a + p[w] * vw[w]
            outs.append(a)
        o_s[r // 2:(r + AR) // 2, :] = _pack(jnp.concatenate(outs, axis=1))

    def attn_unpermute(i, r):
        rows = slice(r // 2, (r + AR) // 2)
        o_s[rows, :] = _permute_cols(o_s[rows, :])

    def wo_part(i, r0):
        y = jnp.dot(_unpack(o_s[r0 // 2:(r0 + WR) // 2, :]), wo_v[...],
                    preferred_element_type=F32)
        for r in range(r0, r0 + WR, LR):
            x1 = x_v[i, r:r + LR, :].astype(F32) + mod(2) * y[r - r0:r - r0 + LR]
            x1_s[i % 2, r:r + LR, :] = x1
            h2_s[r // 2:(r + LR) // 2, :] = _pack(_ln_mod(x1, mod(4), mod(3)))

    def gate_up(cix):
        cs = slice(cix * FC, (cix + 1) * FC)
        h2 = _unpack(h2_s[...])
        g = jnp.dot(h2, wg_v[:, cs], preferred_element_type=F32)
        u = jnp.dot(h2, wu_v[:, cs], preferred_element_type=F32)
        post(g, u)
        t = 0.5 * g
        act_s[:, cs] = _pack((t + t * jnp.tanh(t)) * u)

    def down(i, n):
        cs = slice(n * DC, (n + 1) * DC)
        y = jnp.dot(_unpack(act_s[...]), wd_v[:, cs], preferred_element_type=F32)
        post(y)
        gb = mod_v[0:1, 5 * D + n * DC:5 * D + (n + 1) * DC]
        out_v[i, :, cs] = (x1_s[i % 2, :, cs] + gb * y).astype(out_v.dtype)

    def par(mxu, vpu):
        done = 0
        for idx, (fn, *args) in enumerate(mxu):
            upto = len(vpu) * (idx + 1) // len(mxu)
            for vfn, *vargs in vpu[done:upto]:
                vfn(*vargs)
            done = upto
            fn(*args)

    halves = range(D // QC)

    def t_qkv(i, js=(0, 1, 2)):
        return [(qkv_part, i, j, hf) for j in js for hf in halves]

    def t_attn(i):
        stages = (attn_qk, attn_lanes, attn_softmax, attn_pv, attn_unpermute)
        nb = TM // AR
        return [(fn, i, (n - k * SKEW) * AR) for n in range(nb + (len(stages) - 1) * SKEW)
                for k, fn in reversed(list(enumerate(stages))) if 0 <= n - k * SKEW < nb]

    def t_ln(fn, i):
        return [(fn, i, r) for r in range(0, TM, LR)] if i < NT else []

    def t_wo(i):
        return [(wo_part, i, r) for r in range(0, TM, WR)]

    t_gu = [(gate_up, cix) for cix in range(NFC)]

    def t_down(i, ns):
        return [(down, i, n) for n in ns]

    def t_mod(ks):
        return [(mod_chunk_vpu, j) for k in ks for j in range(k * per, (k + 1) * per)]

    def wait(cps):
        for cp in cps:
            cp.wait()

    def chunk_cps(k):
        return [mod_cp(k), mod_cp(per + k), qkv_cp(k)]

    def modulate0(k):
        mod_chunk(k)
        mod_chunk(per + k)
        ln1_apply0(k)

    start(small_cps + [x_cp(0)] + chunk_cps(0))
    wait(small_cps)
    silu_c_columns()
    x_cp(0).wait()
    start([kv0_cp])
    par([(ln1_norm0, r) for r in range(0, TM, LR)], [])
    qkv_cp(0).wait()
    prep_qkv(0, 0)
    wait(chunk_cps(0)[:2])
    start(chunk_cps(1))
    modulate0(0)
    kv0_cp.wait()
    arrive = [chunk_cps(k) for k in range(per)]
    arrive[-1] += [x_cp(1)]
    later = [chunk_cps(k) for k in range(2, per)]
    later += [[x_cp(2)] + mod_cps(2) + [wo_cp], mod_cps(3) + mod_cps(4) + mod_cps(5)]
    steps = [(j, k) for k in range(per) for j in range(3)]
    ln_next = t_ln(ln1, 1)
    for n, (j, k) in enumerate(steps):
        if j == 2:
            if k + 1 < per:
                wait(arrive[k + 1])
            start(later[k])
            if k == 0:
                x_cp(1).start()
            if k + 1 < per:
                modulate0(k + 1)
        if n + 1 < len(steps):
            prep_qkv(*steps[n + 1])
        if n + 2 >= len(steps):
            half = len(ln_next) // 2
            par(ln_next[:half] if n + 2 == len(steps) else ln_next[half:], [])
        qkv_first(j, k)
    x_cp(2).wait()
    start([wg_cp])
    par(t_qkv(1), t_attn(0) + t_ln(ln1, 2))
    wait(mod_cps(2) + mod_cps(3) + mod_cps(4) + mod_cps(5) + [wo_cp])
    x_rest = [x_cp(i) for i in range(3, NT)]
    start([wu_cp])
    q2 = t_qkv(2)
    par(q2[:-1], t_mod((2, 3, 4)))
    start([wd_cp] + x_rest)
    par(t_wo(0), [])
    par(q2[-1:], [])
    wait([wg_cp, wu_cp])
    first, second = range(N_D1), range(N_D1, NDC)
    for i in range(1, NT):
        att = t_attn(i)
        par(t_gu, att[:N_GU] + (t_mod((5,)) if i == 1 else []))
        if i == 1:
            wait([wd_cp] + x_rest)
        par(t_down(i - 1, first), att[N_GU:] + t_ln(ln1, i + 2))
        par(t_wo(i), [])
        par(t_down(i - 1, second), [])
        if i + 2 < NT:
            par(t_qkv(i + 2), [])
        pass
    out_cps[0].start()
    par(t_gu, [])
    par(t_down(NT - 1, range(NDC - 1)), [])
    out_cps[1].start()
    down(NT - 1, NDC - 1)
    out_cps[2].start()
    wait(out_cps)


@jax.jit
def pallas_adaLN_cond__sliding_local_dilated__swiglu_ffn__prompt_kernel(
    A_x: jax.Array,
    A_wqkv: jax.Array,
    A_wo: jax.Array,
    B_x: jax.Array,
    B_w_gate: jax.Array,
    B_w_up: jax.Array,
    B_w_down: jax.Array,
    c: jax.Array,
    w_mod: jax.Array,
):
    del B_x
    x = A_x.reshape(NT, TM, D)
    hbm = pl.BlockSpec(memory_space=pl.ANY)
    out = pl.pallas_call(
        _kernel,
        in_specs=[hbm] * 9,
        out_specs=hbm,
        out_shape=jax.ShapeDtypeStruct((NT, TM, D), A_x.dtype),
        scratch_shapes=[
            pltpu.VMEM((AR, 128), jnp.int32),
            pltpu.VMEM((1, D), BF16),
            pltpu.VMEM((NT, TM, D), BF16),
            pltpu.VMEM((NT, TM, D), BF16),
            pltpu.VMEM((D, 6 * D), BF16),
            pltpu.VMEM((D, 3 * D), BF16),
            pltpu.VMEM((D // 2, 3 * D), U32),
            pltpu.VMEM((D, D), BF16),
            pltpu.VMEM((D, F), BF16),
            pltpu.VMEM((D, F), BF16),
            pltpu.VMEM((F, D), BF16),
            pltpu.VMEM((8, 6 * D), F32),
            pltpu.VMEM((D, 128), F32),
            pltpu.VMEM((2, TM // 2, D), U32),
            pltpu.VMEM((2, NLT, TM, 128), F32),
            pltpu.VMEM((2, NLT, HALO + TM, 128), F32),
            pltpu.VMEM((2, NLT, HALO + TM, 128), F32),
            pltpu.VMEM((TM // 2, D), U32),
            pltpu.VMEM((2, TM, D), F32),
            pltpu.VMEM((TM // 2, D), U32),
            pltpu.VMEM((TM // 2, F), U32),
            pltpu.SemaphoreType.DMA((6 * D // MC + 9,)),
            pltpu.SemaphoreType.DMA((D // MC + 1,)),
            pltpu.SemaphoreType.DMA((NT,)),
            pltpu.SemaphoreType.DMA((3,)),
        ],
        compiler_params=pltpu.CompilerParams(
            vmem_limit_bytes=110 * 1024 * 1024,
        ),
    )(np.zeros((AR, 128), np.int32), x, c, w_mod, A_wqkv, A_wo, B_w_gate, B_w_up, B_w_down)
    return out.reshape(A_x.shape)


def _rederive():
    global NT, NFC, NDC
    NT, NFC, NDC = S // TM, F // FC, D // DC
```

```python
import jax
import jax.numpy as jnp
import numpy as np
from jax import lax
from jax.experimental import pallas as pl
from jax.experimental.pallas import tpu as pltpu

S, D, F = 2048, 1024, 3584
H, DH, W, DIL = 32, 32, 8, 2
TM = 512
NT = S // TM
HALO = 16
FC = 256
NFC = F // FC
DC = 256
NDC = D // DC
AR = 16
LR = 16
MC = 256
NLT = D // 128
QC = 512
WR = 256
N_D1 = 3
G = 4
GP = 4
SKEW = 1
N_GU = 160
EPS = 1e-5
LOG2E = 1.4426950408889634
SCALE = DH ** -0.5 * LOG2E
F32, BF16, U32 = jnp.float32, jnp.bfloat16, jnp.uint32


def _swap_tiles_lanes(tiles):
    lane = lax.broadcasted_iota(jnp.int32, tiles[0].shape, 1)
    for b in range(3):
        sh = 4 << b
        low = (lane & sh) == 0
        new = list(tiles)
        for t in range(NLT):
            if not (t >> b) & 1:
                a, c = tiles[t], tiles[t | (1 << b)]
                new[t] = jnp.where(low, a, pltpu.roll(c, sh, 1))
                new[t | (1 << b)] = jnp.where(low, pltpu.roll(a, 128 - sh, 1), c)
        tiles = new
    return tiles


def _permute_cols(u):
    tiles = _swap_tiles_lanes([u[:, t * 128:(t + 1) * 128] for t in range(NLT)])
    return jnp.concatenate(tiles, axis=1)


def _pack(val):
    return pltpu.bitcast(val.astype(BF16), U32)


def _unpack(u):
    return pltpu.bitcast(u, BF16)


def _ln(x):
    m = jnp.mean(x, axis=-1, keepdims=True)
    xc = x - m
    v = jnp.mean(xc * xc, axis=-1, keepdims=True)
    return xc * lax.rsqrt(v + EPS)


def _ln_mod(x, scale1, shift):
    return _ln(x) * scale1 + shift


def _kernel(zero_hbm, x_hbm, c_hbm, wmod_hbm, wqkv_hbm, wo_hbm, wg_hbm, wu_hbm, wd_hbm, out_hbm,
            zero_v, c_v, x_v, out_v, wmod_v, wraw_v, wqkv_v, wo_v, wg_v, wu_v, wd_v, mod_v, scb_s, h_s, q_s, k_s, v_s, o_s,
            x1_s, h2_s, act_s, sems, qsems, xsems, osems):
    n_mod = 6 * D // MC

    def mod_cp(j):
        return pltpu.make_async_copy(wmod_hbm.at[:, pl.ds(j * MC, MC)],
                                     wmod_v.at[:, pl.ds(j * MC, MC)], sems.at[j])

    def qkv_cp(k):
        blk = (pl.ds(k * MC, MC), pl.ds(0, 3 * D if k else D))
        return pltpu.make_async_copy(wqkv_hbm.at[blk], wraw_v.at[blk], qsems.at[k])

    kv0 = (pl.ds(0, MC), pl.ds(D, 2 * D))
    kv0_cp = pltpu.make_async_copy(wqkv_hbm.at[kv0], wraw_v.at[kv0], qsems.at[D // MC])

    def x_cp(i):
        return pltpu.make_async_copy(x_hbm.at[i], x_v.at[i], xsems.at[i])

    last_cs = (pl.ds(0, D - DC), pl.ds(D - DC, DC))
    out_cps = [pltpu.make_async_copy(out_v.at[pl.ds(0, NT - 1)], out_hbm.at[pl.ds(0, NT - 1)],
                                     osems.at[0])]
    out_cps += [pltpu.make_async_copy(out_v.at[NT - 1, :, cs], out_hbm.at[NT - 1, :, cs],
                                      osems.at[1 + n]) for n, cs in enumerate(last_cs)]

    wo_cp = pltpu.make_async_copy(wo_hbm, wo_v, sems.at[n_mod + 3])
    wg_cp = pltpu.make_async_copy(wg_hbm, wg_v, sems.at[n_mod + 4])
    wu_cp = pltpu.make_async_copy(wu_hbm, wu_v, sems.at[n_mod + 5])
    wd_cp = pltpu.make_async_copy(wd_hbm, wd_v, sems.at[n_mod + 6])
    small_cps = [pltpu.make_async_copy(c_hbm, c_v, sems.at[n_mod + 7]),
                 pltpu.make_async_copy(zero_hbm, zero_v, sems.at[n_mod + 8])]
    per = D // MC

    def mod_cps(k):
        return [mod_cp(j) for j in range(k * per, (k + 1) * per)]

    def start(cps):
        for cp in cps:
            cp.start()

    def mod_chunk(j):
        cf = c_v[...].astype(F32)
        sc = jnp.broadcast_to(cf * jax.nn.sigmoid(cf), (16, D)).astype(BF16)
        r = jnp.dot(sc, wmod_v[:, j * MC:(j + 1) * MC], preferred_element_type=F32)
        if j // per in (1, 4):
            r = r + 1.0
        mod_v[:, j * MC:(j + 1) * MC] = r[0:8]

    def silu_c_columns():
        cf = c_v[...].astype(F32)
        sc = (cf * jax.nn.sigmoid(cf)).astype(BF16).astype(F32)
        for t in range(NLT):
            blk = jnp.broadcast_to(sc[:, t * 128:(t + 1) * 128], (128, 128))
            scb_s[t * 128:(t + 1) * 128, :] = blk.T

    def mod_chunk_vpu(j):
        cs = slice(j * MC, (j + 1) * MC)
        acc = paced(jnp.zeros((AR, 128), F32))
        acc = jnp.concatenate([acc] * (MC // 128), axis=1)
        for r in range(0, D, AR):
            sc = scb_s[r:r + AR, :]
            sc = jnp.concatenate([sc] * (MC // 128), axis=1)
            acc = acc + wmod_v[r:r + AR, cs].astype(F32) * sc
        res = jnp.sum(acc, axis=0, keepdims=True)
        if j // per in (1, 4):
            res = res + 1.0
        mod_v[:, cs] = jnp.broadcast_to(res, (8, MC))

    tokens = []

    def after(dep, val):
        return jnp.where(zero_v[...] != 0, dep, val)

    def paced(val):
        if not tokens:
            return val
        return after(tokens.pop(0), val)

    def paced_rows(val):
        top = jnp.concatenate([paced(val[:AR, :128]), val[:AR, 128:]], axis=1)
        return jnp.concatenate([top, val[AR:]], axis=0) if val.shape[0] > AR else top

    def post(*results):
        tokens[:] = [res[TM - AR:TM, c:c + 128] for res in results
                     for c in range(0, res.shape[1], 256)]

    def mod(k):
        return mod_v[0:1, k * D:(k + 1) * D]

    def ln1(i, r):
        xv = paced_rows(x_v[i, r:r + LR, :].astype(F32))
        h_s[i % 2, r // 2:(r + LR) // 2, :] = _pack(_ln_mod(xv, mod(1), mod(0)))

    def ln1_norm0(r):
        x1_s[0, r:r + LR, :] = _ln(x_v[0, r:r + LR, :].astype(F32))

    def ln1_apply0(j):
        cs = slice(j * MC, (j + 1) * MC)
        h_s[0, :, cs] = _pack(x1_s[0, :, cs] * mod_v[0:1, D + j * MC:D + (j + 1) * MC]
                              + mod_v[0:1, cs])

    def prep_qkv(j, k):
        for r in range(k * MC, (k + 1) * MC, 128):
            wqkv_v[r // 2:r // 2 + 64, j * D:(j + 1) * D] = _permute_cols(
                _pack(wraw_v[r:r + 128, j * D:(j + 1) * D]))

    def qkv_first(j, k):
        res = jnp.dot(_unpack(h_s[0, :, k * MC:(k + 1) * MC]),
                      _unpack(wqkv_v[k * MC // 2:(k + 1) * MC // 2, j * D:(j + 1) * D]),
                      preferred_element_type=F32)
        post(res)
        if k > 0:
            dst, r0 = ((q_s, 0), (k_s, HALO), (v_s, HALO))[j]
            res = res + jnp.concatenate([dst[0, t, r0:r0 + TM, :] for t in range(NLT)], axis=1)
        qkv_store(0, j, 0, res, final=k == D // MC - 1)

    def qkv_part(i, j, half):
        c0 = j * D + half * QC
        res = jnp.dot(_unpack(h_s[i % 2]), _unpack(wqkv_v[:, c0:c0 + QC]),
                      preferred_element_type=F32)
        qkv_store(i, j, half, res)
        post(res)

    def qkv_store(i, j, half, res, final=True):
        sl = i % 2
        for tt in range(res.shape[1] // 128):
            t = half * (QC // 128) + tt
            blk = res[:, tt * 128:(tt + 1) * 128]
            if j == 0:
                q_s[sl, t] = blk * SCALE if final else blk
                continue
            dst = k_s if j == 1 else v_s
            dst[sl, t, HALO:HALO + TM, :] = blk
            if not final:
                continue
            if i == 0:
                dst[sl, t, 0:HALO, :] = jnp.broadcast_to(blk[0:1], (HALO, 128))
            else:
                dst[sl, t, 0:HALO, :] = dst[1 - sl, t, TM:TM + HALO, :]

    live = {}

    def window(ref, sl, t, r, w):
        o = HALO + r - DIL * w
        return ref[sl, t, o:o + AR, :]

    def attn_qk(i, r):
        sl = i % 2
        lg = None
        for t in range(NLT):
            q = q_s[sl, t, r:r + AR, :]
            if t == 0:
                q = paced(q)
            else:
                q = after(lg[-1], q)
            prod = []
            for w in range(W):
                if w and w % G == 0:
                    q = after(prod[-1], q)
                prod.append(q * window(k_s, sl, t, r, w))
            lg = prod if lg is None else [a + b for a, b in zip(lg, prod)]
        live[i, r] = lg

    def attn_lanes(i, r):
        lane = lax.broadcasted_iota(jnp.int32, (AR, 128), 1)
        b0 = (lane & 1) == 0
        b1 = (lane & 2) == 0
        lg = [a + jnp.where(b0, pltpu.roll(a, 127, 1), pltpu.roll(a, 1, 1)) for a in live[i, r]]
        lg = [a + jnp.where(b1, pltpu.roll(a, 126, 1), pltpu.roll(a, 2, 1)) for a in lg]
        live[i, r] = lg

    def attn_softmax(i, r):
        lg = live[i, r]
        if i == 0 and r < DIL * (W - 1):
            row = lax.broadcasted_iota(jnp.int32, (AR, 128), 0) + r
            lg = [jnp.where(row >= DIL * w, a, -1000000000.0 * LOG2E) for w, a in enumerate(lg)]
        m = lg[0]
        for w in range(1, W):
            m = jnp.maximum(m, lg[w])
        e = [jnp.exp2(a - m) for a in lg]
        s = e[0]
        for w in range(1, W):
            s = s + e[w]
        inv = 1.0 / s
        live[i, r] = [a * inv for a in e]

    def attn_pv(i, r):
        sl = i % 2
        p = live.pop((i, r))
        outs = None
        for w in range(W):
            pw = after(outs[-1], p[w]) if w else p[w]
            prod = []
            for t in range(NLT):
                if t and t % GP == 0:
                    pw = after(prod[-1], pw)
                prod.append(pw * window(v_s, sl, t, r, w))
            outs = prod if outs is None else [a + b for a, b in zip(outs, prod)]
        o_s[r // 2:(r + AR) // 2, :] = _pack(jnp.concatenate(outs, axis=1))

    def attn_unpermute(i, r):
        rows = slice(r // 2, (r + AR) // 2)
        o_s[rows, :] = _permute_cols(o_s[rows, :])

    def wo_part(i, r0):
        y = jnp.dot(_unpack(o_s[r0 // 2:(r0 + WR) // 2, :]), wo_v[...],
                    preferred_element_type=F32)
        for r in range(r0, r0 + WR, LR):
            x1 = x_v[i, r:r + LR, :].astype(F32) + mod(2) * y[r - r0:r - r0 + LR]
            x1_s[i % 2, r:r + LR, :] = x1
            h2_s[r // 2:(r + LR) // 2, :] = _pack(_ln_mod(x1, mod(4), mod(3)))

    def gate_up(cix):
        cs = slice(cix * FC, (cix + 1) * FC)
        h2 = _unpack(h2_s[...])
        g = jnp.dot(h2, wg_v[:, cs], preferred_element_type=F32)
        u = jnp.dot(h2, wu_v[:, cs], preferred_element_type=F32)
        post(g, u)
        t = 0.5 * g
        act_s[:, cs] = _pack((t + t * jnp.tanh(t)) * u)

    def down(i, n):
        cs = slice(n * DC, (n + 1) * DC)
        y = jnp.dot(_unpack(act_s[...]), wd_v[:, cs], preferred_element_type=F32)
        post(y)
        gb = mod_v[0:1, 5 * D + n * DC:5 * D + (n + 1) * DC]
        out_v[i, :, cs] = (x1_s[i % 2, :, cs] + gb * y).astype(out_v.dtype)

    def par(mxu, vpu):
        done = 0
        for idx, (fn, *args) in enumerate(mxu):
            upto = len(vpu) * (idx + 1) // len(mxu)
            for vfn, *vargs in vpu[done:upto]:
                vfn(*vargs)
            done = upto
            fn(*args)

    halves = range(D // QC)

    def t_qkv(i, js=(0, 1, 2)):
        return [(qkv_part, i, j, hf) for j in js for hf in halves]

    def t_attn(i):
        stages = (attn_qk, attn_lanes, attn_softmax, attn_pv, attn_unpermute)
        nb = TM // AR
        return [(fn, i, (n - k * SKEW) * AR) for n in range(nb + (len(stages) - 1) * SKEW)
                for k, fn in reversed(list(enumerate(stages))) if 0 <= n - k * SKEW < nb]

    def t_ln(fn, i):
        return [(fn, i, r) for r in range(0, TM, LR)] if i < NT else []

    def t_wo(i):
        return [(wo_part, i, r) for r in range(0, TM, WR)]

    t_gu = [(gate_up, cix) for cix in range(NFC)]

    def t_down(i, ns):
        return [(down, i, n) for n in ns]

    def t_mod(ks):
        return [(mod_chunk_vpu, j) for k in ks for j in range(k * per, (k + 1) * per)]

    def wait(cps):
        for cp in cps:
            cp.wait()

    def chunk_cps(k):
        return [mod_cp(k), mod_cp(per + k), qkv_cp(k)]

    def modulate0(k):
        mod_chunk(k)
        mod_chunk(per + k)
        ln1_apply0(k)

    start(small_cps + [x_cp(0)] + chunk_cps(0))
    wait(small_cps)
    silu_c_columns()
    x_cp(0).wait()
    start([kv0_cp])
    par([(ln1_norm0, r) for r in range(0, TM, LR)], [])
    qkv_cp(0).wait()
    prep_qkv(0, 0)
    wait(chunk_cps(0)[:2])
    start(chunk_cps(1))
    modulate0(0)
    kv0_cp.wait()
    arrive = [chunk_cps(k) for k in range(per)]
    arrive[-1] += [x_cp(1)]
    later = [chunk_cps(k) for k in range(2, per)]
    later += [[x_cp(2)] + mod_cps(2) + [wo_cp], mod_cps(3) + mod_cps(4) + mod_cps(5)]
    steps = [(j, k) for k in range(per) for j in range(3)]
    ln_next = t_ln(ln1, 1)
    for n, (j, k) in enumerate(steps):
        if j == 2:
            if k + 1 < per:
                wait(arrive[k + 1])
            start(later[k])
            if k == 0:
                x_cp(1).start()
            if k + 1 < per:
                modulate0(k + 1)
        if n + 1 < len(steps):
            prep_qkv(*steps[n + 1])
        if n + 2 >= len(steps):
            half = len(ln_next) // 2
            par(ln_next[:half] if n + 2 == len(steps) else ln_next[half:], [])
        qkv_first(j, k)
    x_cp(2).wait()
    start([wg_cp])
    par(t_qkv(1), t_attn(0) + t_ln(ln1, 2))
    wait(mod_cps(2) + mod_cps(3) + mod_cps(4) + mod_cps(5) + [wo_cp])
    x_rest = [x_cp(i) for i in range(3, NT)]
    start([wu_cp])
    q2 = t_qkv(2)
    par(q2[:-1], t_mod((2, 3, 4)))
    start([wd_cp] + x_rest)
    par(t_wo(0), [])
    par(q2[-1:], [])
    wait([wg_cp, wu_cp])
    first, second = range(N_D1), range(N_D1, NDC)
    for i in range(1, NT):
        att = t_attn(i)
        par(t_gu, att[:N_GU] + (t_mod((5,)) if i == 1 else []))
        if i == 1:
            wait([wd_cp] + x_rest)
        par(t_down(i - 1, first), att[N_GU:] + t_ln(ln1, i + 2))
        par(t_wo(i), [])
        par(t_down(i - 1, second), [])
        if i + 2 < NT:
            par(t_qkv(i + 2), [])
        pass
    out_cps[0].start()
    par(t_gu, [])
    par(t_down(NT - 1, range(NDC - 1)), [])
    out_cps[1].start()
    down(NT - 1, NDC - 1)
    out_cps[2].start()
    wait(out_cps)


@jax.jit
def pallas_adaLN_cond__sliding_local_dilated__swiglu_ffn__prompt_kernel(
    A_x: jax.Array,
    A_wqkv: jax.Array,
    A_wo: jax.Array,
    B_x: jax.Array,
    B_w_gate: jax.Array,
    B_w_up: jax.Array,
    B_w_down: jax.Array,
    c: jax.Array,
    w_mod: jax.Array,
):
    del B_x
    x = A_x.reshape(NT, TM, D)
    hbm = pl.BlockSpec(memory_space=pl.ANY)
    out = pl.pallas_call(
        _kernel,
        in_specs=[hbm] * 9,
        out_specs=hbm,
        out_shape=jax.ShapeDtypeStruct((NT, TM, D), A_x.dtype),
        scratch_shapes=[
            pltpu.VMEM((AR, 128), jnp.int32),
            pltpu.VMEM((1, D), BF16),
            pltpu.VMEM((NT, TM, D), BF16),
            pltpu.VMEM((NT, TM, D), BF16),
            pltpu.VMEM((D, 6 * D), BF16),
            pltpu.VMEM((D, 3 * D), BF16),
            pltpu.VMEM((D // 2, 3 * D), U32),
            pltpu.VMEM((D, D), BF16),
            pltpu.VMEM((D, F), BF16),
            pltpu.VMEM((D, F), BF16),
            pltpu.VMEM((F, D), BF16),
            pltpu.VMEM((8, 6 * D), F32),
            pltpu.VMEM((D, 128), F32),
            pltpu.VMEM((2, TM // 2, D), U32),
            pltpu.VMEM((2, NLT, TM, 128), F32),
            pltpu.VMEM((2, NLT, HALO + TM, 128), F32),
            pltpu.VMEM((2, NLT, HALO + TM, 128), F32),
            pltpu.VMEM((TM // 2, D), U32),
            pltpu.VMEM((2, TM, D), F32),
            pltpu.VMEM((TM // 2, D), U32),
            pltpu.VMEM((TM // 2, F), U32),
            pltpu.SemaphoreType.DMA((6 * D // MC + 9,)),
            pltpu.SemaphoreType.DMA((D // MC + 1,)),
            pltpu.SemaphoreType.DMA((NT,)),
            pltpu.SemaphoreType.DMA((3,)),
        ],
        compiler_params=pltpu.CompilerParams(
            vmem_limit_bytes=110 * 1024 * 1024,
        ),
    )(np.zeros((AR, 128), np.int32), x, c, w_mod, A_wqkv, A_wo, B_w_gate, B_w_up, B_w_down)
    return out.reshape(A_x.shape)


def _rederive():
    global NT, NFC, NDC
    NT, NFC, NDC = S // TM, F // FC, D // DC
```

```python
import jax
import jax.numpy as jnp
import numpy as np
from jax import lax
from jax.experimental import pallas as pl
from jax.experimental.pallas import tpu as pltpu

S, D, F = 2048, 1024, 3584
H, DH, W, DIL = 32, 32, 8, 2
TM = 512
NT = S // TM
HALO = 16
FC = 256
NFC = F // FC
DC = 256
NDC = D // DC
AR = 16
LR = 16
MC = 256
NLT = D // 128
QC = 512
WR = 256
N_D1 = 3
G = 4
SKEW = 1
N_GU = 160
EPS = 1e-5
LOG2E = 1.4426950408889634
SCALE = DH ** -0.5 * LOG2E
F32, BF16, U32 = jnp.float32, jnp.bfloat16, jnp.uint32


def _swap_tiles_lanes(tiles):
    lane = lax.broadcasted_iota(jnp.int32, tiles[0].shape, 1)
    for b in range(3):
        sh = 4 << b
        low = (lane & sh) == 0
        new = list(tiles)
        for t in range(NLT):
            if not (t >> b) & 1:
                a, c = tiles[t], tiles[t | (1 << b)]
                new[t] = jnp.where(low, a, pltpu.roll(c, sh, 1))
                new[t | (1 << b)] = jnp.where(low, pltpu.roll(a, 128 - sh, 1), c)
        tiles = new
    return tiles


def _permute_cols(u):
    tiles = _swap_tiles_lanes([u[:, t * 128:(t + 1) * 128] for t in range(NLT)])
    return jnp.concatenate(tiles, axis=1)


def _pack(val):
    return pltpu.bitcast(val.astype(BF16), U32)


def _unpack(u):
    return pltpu.bitcast(u, BF16)


def _ln(x):
    m = jnp.mean(x, axis=-1, keepdims=True)
    xc = x - m
    v = jnp.mean(xc * xc, axis=-1, keepdims=True)
    return xc * lax.rsqrt(v + EPS)


def _ln_mod(x, scale1, shift):
    return _ln(x) * scale1 + shift


def _kernel(zero_hbm, x_hbm, c_hbm, wmod_hbm, wqkv_hbm, wo_hbm, wg_hbm, wu_hbm, wd_hbm, out_hbm,
            zero_v, c_v, x_v, out_v, wmod_v, wraw_v, wqkv_v, wo_v, wg_v, wu_v, wd_v, mod_v, scb_s, h_s, q_s, k_s, v_s, o_s,
            x1_s, h2_s, act_s, sems, qsems, xsems, osems):
    n_mod = 6 * D // MC

    def mod_cp(j):
        return pltpu.make_async_copy(wmod_hbm.at[:, pl.ds(j * MC, MC)],
                                     wmod_v.at[:, pl.ds(j * MC, MC)], sems.at[j])

    def qkv_cp(k):
        blk = (pl.ds(k * MC, MC), pl.ds(0, 3 * D if k else D))
        return pltpu.make_async_copy(wqkv_hbm.at[blk], wraw_v.at[blk], qsems.at[k])

    kv0 = (pl.ds(0, MC), pl.ds(D, 2 * D))
    kv0_cp = pltpu.make_async_copy(wqkv_hbm.at[kv0], wraw_v.at[kv0], qsems.at[D // MC])

    def x_cp(i):
        return pltpu.make_async_copy(x_hbm.at[i], x_v.at[i], xsems.at[i])

    last_cs = (pl.ds(0, D - DC), pl.ds(D - DC, DC))
    out_cps = [pltpu.make_async_copy(out_v.at[pl.ds(0, NT - 1)], out_hbm.at[pl.ds(0, NT - 1)],
                                     osems.at[0])]
    out_cps += [pltpu.make_async_copy(out_v.at[NT - 1, :, cs], out_hbm.at[NT - 1, :, cs],
                                      osems.at[1 + n]) for n, cs in enumerate(last_cs)]

    wo_cp = pltpu.make_async_copy(wo_hbm, wo_v, sems.at[n_mod + 3])
    wg_cp = pltpu.make_async_copy(wg_hbm, wg_v, sems.at[n_mod + 4])
    wu_cp = pltpu.make_async_copy(wu_hbm, wu_v, sems.at[n_mod + 5])
    wd_cp = pltpu.make_async_copy(wd_hbm, wd_v, sems.at[n_mod + 6])
    small_cps = [pltpu.make_async_copy(c_hbm, c_v, sems.at[n_mod + 7]),
                 pltpu.make_async_copy(zero_hbm, zero_v, sems.at[n_mod + 8])]
    per = D // MC

    def mod_cps(k):
        return [mod_cp(j) for j in range(k * per, (k + 1) * per)]

    def start(cps):
        for cp in cps:
            cp.start()

    def mod_chunk(j):
        cf = c_v[...].astype(F32)
        sc = jnp.broadcast_to(cf * jax.nn.sigmoid(cf), (16, D)).astype(BF16)
        r = jnp.dot(sc, wmod_v[:, j * MC:(j + 1) * MC], preferred_element_type=F32)
        if j // per in (1, 4):
            r = r + 1.0
        mod_v[:, j * MC:(j + 1) * MC] = r[0:8]

    def silu_c_columns():
        cf = c_v[...].astype(F32)
        sc = (cf * jax.nn.sigmoid(cf)).astype(BF16).astype(F32)
        for t in range(NLT):
            blk = jnp.broadcast_to(sc[:, t * 128:(t + 1) * 128], (128, 128))
            scb_s[t * 128:(t + 1) * 128, :] = blk.T

    def mod_chunk_vpu(j):
        cs = slice(j * MC, (j + 1) * MC)
        acc = paced(jnp.zeros((AR, 128), F32))
        acc = jnp.concatenate([acc] * (MC // 128), axis=1)
        for r in range(0, D, AR):
            sc = scb_s[r:r + AR, :]
            sc = jnp.concatenate([sc] * (MC // 128), axis=1)
            acc = acc + wmod_v[r:r + AR, cs].astype(F32) * sc
        res = jnp.sum(acc, axis=0, keepdims=True)
        if j // per in (1, 4):
            res = res + 1.0
        mod_v[:, cs] = jnp.broadcast_to(res, (8, MC))

    tokens = []

    def after(dep, val):
        return jnp.where(zero_v[...] != 0, dep, val)

    def paced(val):
        if not tokens:
            return val
        return after(tokens.pop(0), val)

    def paced_rows(val):
        top = jnp.concatenate([paced(val[:AR, :128]), val[:AR, 128:]], axis=1)
        return jnp.concatenate([top, val[AR:]], axis=0) if val.shape[0] > AR else top

    def post(*results):
        tokens[:] = [res[TM - AR:TM, c:c + 128] for res in results
                     for c in range(0, res.shape[1], 256)]

    def mod(k):
        return mod_v[0:1, k * D:(k + 1) * D]

    def ln1(i, r):
        xv = paced_rows(x_v[i, r:r + LR, :].astype(F32))
        h_s[i % 2, r // 2:(r + LR) // 2, :] = _pack(_ln_mod(xv, mod(1), mod(0)))

    def ln1_norm0(r):
        x1_s[0, r:r + LR, :] = _ln(x_v[0, r:r + LR, :].astype(F32))

    def ln1_apply0(j):
        cs = slice(j * MC, (j + 1) * MC)
        h_s[0, :, cs] = _pack(x1_s[0, :, cs] * mod_v[0:1, D + j * MC:D + (j + 1) * MC]
                              + mod_v[0:1, cs])

    def prep_qkv(j, k):
        for r in range(k * MC, (k + 1) * MC, 128):
            wqkv_v[r // 2:r // 2 + 64, j * D:(j + 1) * D] = _permute_cols(
                _pack(wraw_v[r:r + 128, j * D:(j + 1) * D]))

    def qkv_first(j, k):
        res = jnp.dot(_unpack(h_s[0, :, k * MC:(k + 1) * MC]),
                      _unpack(wqkv_v[k * MC // 2:(k + 1) * MC // 2, j * D:(j + 1) * D]),
                      preferred_element_type=F32)
        post(res)
        if k > 0:
            dst, r0 = ((q_s, 0), (k_s, HALO), (v_s, HALO))[j]
            res = res + jnp.concatenate([dst[0, t, r0:r0 + TM, :] for t in range(NLT)], axis=1)
        qkv_store(0, j, 0, res, final=k == D // MC - 1)

    def qkv_part(i, j, half):
        c0 = j * D + half * QC
        res = jnp.dot(_unpack(h_s[i % 2]), _unpack(wqkv_v[:, c0:c0 + QC]),
                      preferred_element_type=F32)
        qkv_store(i, j, half, res)
        post(res)

    def qkv_store(i, j, half, res, final=True):
        sl = i % 2
        for tt in range(res.shape[1] // 128):
            t = half * (QC // 128) + tt
            blk = res[:, tt * 128:(tt + 1) * 128]
            if j == 0:
                q_s[sl, t] = blk * SCALE if final else blk
                continue
            dst = k_s if j == 1 else v_s
            dst[sl, t, HALO:HALO + TM, :] = blk
            if not final:
                continue
            if i == 0:
                dst[sl, t, 0:HALO, :] = jnp.broadcast_to(blk[0:1], (HALO, 128))
            else:
                dst[sl, t, 0:HALO, :] = dst[1 - sl, t, TM:TM + HALO, :]

    live = {}

    def window(ref, sl, t, r, w):
        o = HALO + r - DIL * w
        return ref[sl, t, o:o + AR, :]

    def attn_qk(i, r):
        sl = i % 2
        lg = None
        for t in range(NLT):
            q = q_s[sl, t, r:r + AR, :]
            if t == 0:
                q = paced(q)
            else:
                q = after(lg[-1], q)
            prod = []
            for w in range(W):
                if w and w % G == 0:
                    q = after(prod[-1], q)
                prod.append(q * window(k_s, sl, t, r, w))
            lg = prod if lg is None else [a + b for a, b in zip(lg, prod)]
        live[i, r] = lg

    def attn_lanes(i, r):
        lane = lax.broadcasted_iota(jnp.int32, (AR, 128), 1)
        b0 = (lane & 1) == 0
        b1 = (lane & 2) == 0
        lg = [a + jnp.where(b0, pltpu.roll(a, 127, 1), pltpu.roll(a, 1, 1)) for a in live[i, r]]
        lg = [a + jnp.where(b1, pltpu.roll(a, 126, 1), pltpu.roll(a, 2, 1)) for a in lg]
        live[i, r] = lg

    def attn_softmax(i, r):
        lg = live[i, r]
        if i == 0 and r < DIL * (W - 1):
            row = lax.broadcasted_iota(jnp.int32, (AR, 128), 0) + r
            lg = [jnp.where(row >= DIL * w, a, -1000000000.0 * LOG2E) for w, a in enumerate(lg)]
        m = lg[0]
        for w in range(1, W):
            m = jnp.maximum(m, lg[w])
        e = [jnp.exp2(a - m) for a in lg]
        s = e[0]
        for w in range(1, W):
            s = s + e[w]
        inv = 1.0 / s
        live[i, r] = [a * inv for a in e]

    def attn_pv(i, r):
        sl = i % 2
        p = live.pop((i, r))
        outs = None
        for w in range(W):
            pw = after(outs[-1], p[w]) if w else p[w]
            prod = []
            for t in range(NLT):
                if t and t % G == 0:
                    pw = after(prod[-1], pw)
                prod.append(pw * window(v_s, sl, t, r, w))
            outs = prod if outs is None else [a + b for a, b in zip(outs, prod)]
        o_s[r // 2:(r + AR) // 2, :] = _pack(jnp.concatenate(outs, axis=1))

    def attn_unpermute(i, r):
        rows = slice(r // 2, (r + AR) // 2)
        o_s[rows, :] = _permute_cols(o_s[rows, :])

    def wo_part(i, r0):
        y = jnp.dot(_unpack(o_s[r0 // 2:(r0 + WR) // 2, :]), wo_v[...],
                    preferred_element_type=F32)
        done = []
        for r in range(r0, r0 + WR, LR):
            x1 = x_v[i, r:r + LR, :].astype(F32) + mod(2) * y[r - r0:r - r0 + LR]
            x1_s[i % 2, r:r + LR, :] = x1
            if done:
                x1 = jnp.concatenate([after(done[-1], x1[:, :128]), x1[:, 128:]], axis=1)
            h2 = _ln_mod(x1, mod(4), mod(3))
            done.append(h2[:, :128])
            h2_s[r // 2:(r + LR) // 2, :] = _pack(h2)

    def gate_up(cix):
        cs = slice(cix * FC, (cix + 1) * FC)
        h2 = _unpack(h2_s[...])
        g = jnp.dot(h2, wg_v[:, cs], preferred_element_type=F32)
        u = jnp.dot(h2, wu_v[:, cs], preferred_element_type=F32)
        post(g, u)
        t = 0.5 * g
        act_s[:, cs] = _pack((t + t * jnp.tanh(t)) * u)

    def down(i, n):
        cs = slice(n * DC, (n + 1) * DC)
        y = jnp.dot(_unpack(act_s[...]), wd_v[:, cs], preferred_element_type=F32)
        post(y)
        gb = mod_v[0:1, 5 * D + n * DC:5 * D + (n + 1) * DC]
        out_v[i, :, cs] = (x1_s[i % 2, :, cs] + gb * y).astype(out_v.dtype)

    def par(mxu, vpu):
        done = 0
        for idx, (fn, *args) in enumerate(mxu):
            upto = len(vpu) * (idx + 1) // len(mxu)
            for vfn, *vargs in vpu[done:upto]:
                vfn(*vargs)
            done = upto
            fn(*args)

    halves = range(D // QC)

    def t_qkv(i, js=(0, 1, 2)):
        return [(qkv_part, i, j, hf) for j in js for hf in halves]

    def t_attn(i):
        stages = (attn_qk, attn_lanes, attn_softmax, attn_pv, attn_unpermute)
        nb = TM // AR
        return [(fn, i, (n - k * SKEW) * AR) for n in range(nb + (len(stages) - 1) * SKEW)
                for k, fn in reversed(list(enumerate(stages))) if 0 <= n - k * SKEW < nb]

    def t_ln(fn, i):
        return [(fn, i, r) for r in range(0, TM, LR)] if i < NT else []

    def t_wo(i):
        return [(wo_part, i, r) for r in range(0, TM, WR)]

    t_gu = [(gate_up, cix) for cix in range(NFC)]

    def t_down(i, ns):
        return [(down, i, n) for n in ns]

    def t_mod(ks):
        return [(mod_chunk_vpu, j) for k in ks for j in range(k * per, (k + 1) * per)]

    def wait(cps):
        for cp in cps:
            cp.wait()

    def chunk_cps(k):
        return [mod_cp(k), mod_cp(per + k), qkv_cp(k)]

    def modulate0(k):
        mod_chunk(k)
        mod_chunk(per + k)
        ln1_apply0(k)

    start(small_cps + [x_cp(0)] + chunk_cps(0))
    wait(small_cps)
    silu_c_columns()
    x_cp(0).wait()
    start([kv0_cp])
    par([(ln1_norm0, r) for r in range(0, TM, LR)], [])
    qkv_cp(0).wait()
    prep_qkv(0, 0)
    wait(chunk_cps(0)[:2])
    start(chunk_cps(1))
    modulate0(0)
    kv0_cp.wait()
    arrive = [chunk_cps(k) for k in range(per)]
    arrive[-1] += [x_cp(1)]
    later = [chunk_cps(k) for k in range(2, per)]
    later += [[x_cp(2)] + mod_cps(2) + [wo_cp], mod_cps(3) + mod_cps(4) + mod_cps(5)]
    steps = [(j, k) for k in range(per) for j in range(3)]
    ln_next = t_ln(ln1, 1)
    for n, (j, k) in enumerate(steps):
        if j == 2:
            if k + 1 < per:
                wait(arrive[k + 1])
            start(later[k])
            if k == 0:
                x_cp(1).start()
            if k + 1 < per:
                modulate0(k + 1)
        if n + 1 < len(steps):
            prep_qkv(*steps[n + 1])
        if n + 2 >= len(steps):
            half = len(ln_next) // 2
            par(ln_next[:half] if n + 2 == len(steps) else ln_next[half:], [])
        qkv_first(j, k)
    x_cp(2).wait()
    start([wg_cp])
    par(t_qkv(1), t_attn(0) + t_ln(ln1, 2))
    wait(mod_cps(2) + mod_cps(3) + mod_cps(4) + mod_cps(5) + [wo_cp])
    x_rest = [x_cp(i) for i in range(3, NT)]
    start([wu_cp])
    q2 = t_qkv(2)
    par(q2[:-1], t_mod((2, 3, 4)))
    start([wd_cp] + x_rest)
    par(t_wo(0), [])
    par(q2[-1:], [])
    wait([wg_cp, wu_cp])
    first, second = range(N_D1), range(N_D1, NDC)
    for i in range(1, NT):
        att = t_attn(i)
        par(t_gu, att[:N_GU] + (t_mod((5,)) if i == 1 else []))
        if i == 1:
            wait([wd_cp] + x_rest)
        par(t_down(i - 1, first), att[N_GU:] + t_ln(ln1, i + 2))
        par(t_wo(i), [])
        par(t_down(i - 1, second), [])
        if i + 2 < NT:
            par(t_qkv(i + 2), [])
        pass
    out_cps[0].start()
    par(t_gu, [])
    par(t_down(NT - 1, range(NDC - 1)), [])
    out_cps[1].start()
    down(NT - 1, NDC - 1)
    out_cps[2].start()
    wait(out_cps)


@jax.jit
def pallas_adaLN_cond__sliding_local_dilated__swiglu_ffn__prompt_kernel(
    A_x: jax.Array,
    A_wqkv: jax.Array,
    A_wo: jax.Array,
    B_x: jax.Array,
    B_w_gate: jax.Array,
    B_w_up: jax.Array,
    B_w_down: jax.Array,
    c: jax.Array,
    w_mod: jax.Array,
):
    del B_x
    x = A_x.reshape(NT, TM, D)
    hbm = pl.BlockSpec(memory_space=pl.ANY)
    out = pl.pallas_call(
        _kernel,
        in_specs=[hbm] * 9,
        out_specs=hbm,
        out_shape=jax.ShapeDtypeStruct((NT, TM, D), A_x.dtype),
        scratch_shapes=[
            pltpu.VMEM((AR, 128), jnp.int32),
            pltpu.VMEM((1, D), BF16),
            pltpu.VMEM((NT, TM, D), BF16),
            pltpu.VMEM((NT, TM, D), BF16),
            pltpu.VMEM((D, 6 * D), BF16),
            pltpu.VMEM((D, 3 * D), BF16),
            pltpu.VMEM((D // 2, 3 * D), U32),
            pltpu.VMEM((D, D), BF16),
            pltpu.VMEM((D, F), BF16),
            pltpu.VMEM((D, F), BF16),
            pltpu.VMEM((F, D), BF16),
            pltpu.VMEM((8, 6 * D), F32),
            pltpu.VMEM((D, 128), F32),
            pltpu.VMEM((2, TM // 2, D), U32),
            pltpu.VMEM((2, NLT, TM, 128), F32),
            pltpu.VMEM((2, NLT, HALO + TM, 128), F32),
            pltpu.VMEM((2, NLT, HALO + TM, 128), F32),
            pltpu.VMEM((TM // 2, D), U32),
            pltpu.VMEM((2, TM, D), F32),
            pltpu.VMEM((TM // 2, D), U32),
            pltpu.VMEM((TM // 2, F), U32),
            pltpu.SemaphoreType.DMA((6 * D // MC + 9,)),
            pltpu.SemaphoreType.DMA((D // MC + 1,)),
            pltpu.SemaphoreType.DMA((NT,)),
            pltpu.SemaphoreType.DMA((3,)),
        ],
        compiler_params=pltpu.CompilerParams(
            vmem_limit_bytes=110 * 1024 * 1024,
        ),
    )(np.zeros((AR, 128), np.int32), x, c, w_mod, A_wqkv, A_wo, B_w_gate, B_w_up, B_w_down)
    return out.reshape(A_x.shape)


def _rederive():
    global NT, NFC, NDC
    NT, NFC, NDC = S // TM, F // FC, D // DC
```

```python
import jax
import jax.numpy as jnp
import numpy as np
from jax import lax
from jax.experimental import pallas as pl
from jax.experimental.pallas import tpu as pltpu

S, D, F = 2048, 1024, 3584
H, DH, W, DIL = 32, 32, 8, 2
TM = 512
NT = S // TM
HALO = 16
FC = 256
NFC = F // FC
DC = 256
NDC = D // DC
AR = 16
LR = 16
MC = 256
NLT = D // 128
QC = 512
WR = 256
N_D1 = 3
G = 4
EPS = 1e-5
LOG2E = 1.4426950408889634
SCALE = DH ** -0.5 * LOG2E
F32, BF16, U32 = jnp.float32, jnp.bfloat16, jnp.uint32


def _swap_tiles_lanes(tiles):
    lane = lax.broadcasted_iota(jnp.int32, tiles[0].shape, 1)
    for b in range(3):
        sh = 4 << b
        low = (lane & sh) == 0
        new = list(tiles)
        for t in range(NLT):
            if not (t >> b) & 1:
                a, c = tiles[t], tiles[t | (1 << b)]
                new[t] = jnp.where(low, a, pltpu.roll(c, sh, 1))
                new[t | (1 << b)] = jnp.where(low, pltpu.roll(a, 128 - sh, 1), c)
        tiles = new
    return tiles


def _permute_cols(u):
    tiles = _swap_tiles_lanes([u[:, t * 128:(t + 1) * 128] for t in range(NLT)])
    return jnp.concatenate(tiles, axis=1)


def _pack(val):
    return pltpu.bitcast(val.astype(BF16), U32)


def _unpack(u):
    return pltpu.bitcast(u, BF16)


def _ln(x):
    m = jnp.mean(x, axis=-1, keepdims=True)
    xc = x - m
    v = jnp.mean(xc * xc, axis=-1, keepdims=True)
    return xc * lax.rsqrt(v + EPS)


def _ln_mod(x, scale1, shift):
    return _ln(x) * scale1 + shift


def _kernel(zero_hbm, x_hbm, c_hbm, wmod_hbm, wqkv_hbm, wo_hbm, wg_hbm, wu_hbm, wd_hbm, out_hbm,
            zero_v, c_v, x_v, out_v, wmod_v, wraw_v, wqkv_v, wo_v, wg_v, wu_v, wd_v, mod_v, scb_s, h_s, q_s, k_s, v_s, o_s,
            x1_s, h2_s, act_s, sems, qsems, xsems, osems):
    n_mod = 6 * D // MC

    def block_cp(src, dst, blk, sem):
        return pltpu.make_async_copy(src.at[blk], dst.at[blk], sem)

    mod_cp = [block_cp(wmod_hbm, wmod_v, (slice(None), pl.ds(j * MC, MC)), sems.at[j])
              for j in range(n_mod)]
    qkv_cp = [block_cp(wqkv_hbm, wraw_v, (pl.ds(k * MC, MC), pl.ds(0, 3 * D if k else D)),
                       qsems.at[k]) for k in range(D // MC)]
    kv0_cp = block_cp(wqkv_hbm, wraw_v, (pl.ds(0, MC), pl.ds(D, 2 * D)), qsems.at[D // MC])
    x_cp = [block_cp(x_hbm, x_v, i, xsems.at[i]) for i in range(NT)]
    last_cs = (pl.ds(0, D - DC), pl.ds(D - DC, DC))
    out_cps = [pltpu.make_async_copy(out_v.at[pl.ds(0, NT - 1)], out_hbm.at[pl.ds(0, NT - 1)],
                                     osems.at[0])]
    out_cps += [pltpu.make_async_copy(out_v.at[NT - 1, :, cs], out_hbm.at[NT - 1, :, cs],
                                      osems.at[1 + n]) for n, cs in enumerate(last_cs)]

    wo_cp = pltpu.make_async_copy(wo_hbm, wo_v, sems.at[n_mod + 3])
    wg_cp = pltpu.make_async_copy(wg_hbm, wg_v, sems.at[n_mod + 4])
    wu_cp = pltpu.make_async_copy(wu_hbm, wu_v, sems.at[n_mod + 5])
    wd_cp = pltpu.make_async_copy(wd_hbm, wd_v, sems.at[n_mod + 6])
    small_cps = [pltpu.make_async_copy(c_hbm, c_v, sems.at[n_mod + 7]),
                 pltpu.make_async_copy(zero_hbm, zero_v, sems.at[n_mod + 8])]
    per = D // MC

    def mod_cps(k):
        return mod_cp[k * per:(k + 1) * per]

    def start(cps):
        for cp in cps:
            cp.start()

    def mod_chunk(j):
        cf = c_v[...].astype(F32)
        sc = jnp.broadcast_to(cf * jax.nn.sigmoid(cf), (16, D)).astype(BF16)
        r = jnp.dot(sc, wmod_v[:, j * MC:(j + 1) * MC], preferred_element_type=F32)
        if j // per in (1, 4):
            r = r + 1.0
        mod_v[:, j * MC:(j + 1) * MC] = r[0:8]

    def silu_c_columns():
        cf = c_v[...].astype(F32)
        sc = (cf * jax.nn.sigmoid(cf)).astype(BF16).astype(F32)
        for t in range(NLT):
            blk = jnp.broadcast_to(sc[:, t * 128:(t + 1) * 128], (128, 128))
            scb_s[t * 128:(t + 1) * 128, :] = blk.T

    def mod_chunk_vpu(j):
        cs = slice(j * MC, (j + 1) * MC)
        acc = paced(jnp.zeros((AR, 128), F32))
        acc = jnp.concatenate([acc] * (MC // 128), axis=1)
        for r in range(0, D, AR):
            sc = scb_s[r:r + AR, :]
            sc = jnp.concatenate([sc] * (MC // 128), axis=1)
            acc = acc + wmod_v[r:r + AR, cs].astype(F32) * sc
        res = jnp.sum(acc, axis=0, keepdims=True)
        if j // per in (1, 4):
            res = res + 1.0
        mod_v[:, cs] = jnp.broadcast_to(res, (8, MC))

    tokens = []

    def after(dep, val):
        return jnp.where(zero_v[...] != 0, dep, val)

    def paced(val):
        if not tokens:
            return val
        return after(tokens.pop(0), val)

    def paced_rows(val):
        top = jnp.concatenate([paced(val[:AR, :128]), val[:AR, 128:]], axis=1)
        return jnp.concatenate([top, val[AR:]], axis=0) if val.shape[0] > AR else top

    def post(*results):
        tokens[:] = [res[TM - AR:TM, c:c + 128] for res in results
                     for c in range(0, res.shape[1], 256)]

    def mod(k):
        return mod_v[0:1, k * D:(k + 1) * D]

    def ln1(i, r):
        xv = paced_rows(x_v[i, r:r + LR, :].astype(F32))
        h_s[i % 2, r // 2:(r + LR) // 2, :] = _pack(_ln_mod(xv, mod(1), mod(0)))

    def ln1_norm0(r):
        x1_s[0, r:r + LR, :] = _ln(x_v[0, r:r + LR, :].astype(F32))

    def ln1_apply0(j):
        cs = slice(j * MC, (j + 1) * MC)
        h_s[0, :, cs] = _pack(x1_s[0, :, cs] * mod_v[0:1, D + j * MC:D + (j + 1) * MC]
                              + mod_v[0:1, cs])

    def prep_qkv(j, k):
        for r in range(k * MC, (k + 1) * MC, 128):
            wqkv_v[r // 2:r // 2 + 64, j * D:(j + 1) * D] = _permute_cols(
                _pack(wraw_v[r:r + 128, j * D:(j + 1) * D]))

    def qkv_first(j, k):
        res = jnp.dot(_unpack(h_s[0, :, k * MC:(k + 1) * MC]),
                      _unpack(wqkv_v[k * MC // 2:(k + 1) * MC // 2, j * D:(j + 1) * D]),
                      preferred_element_type=F32)
        post(res)
        if k > 0:
            dst, r0 = ((q_s, 0), (k_s, HALO), (v_s, HALO))[j]
            res = res + jnp.concatenate([dst[0, t, r0:r0 + TM, :] for t in range(NLT)], axis=1)
        qkv_store(0, j, 0, res, final=k == D // MC - 1)

    def qkv_part(i, j, half):
        c0 = j * D + half * QC
        res = jnp.dot(_unpack(h_s[i % 2]), _unpack(wqkv_v[:, c0:c0 + QC]),
                      preferred_element_type=F32)
        qkv_store(i, j, half, res)
        post(res)

    def qkv_store(i, j, half, res, final=True):
        sl = i % 2
        for tt in range(res.shape[1] // 128):
            t = half * (QC // 128) + tt
            blk = res[:, tt * 128:(tt + 1) * 128]
            if j == 0:
                q_s[sl, t] = blk * SCALE if final else blk
                continue
            dst = k_s if j == 1 else v_s
            dst[sl, t, HALO:HALO + TM, :] = blk
            if not final:
                continue
            if i == 0:
                dst[sl, t, 0:HALO, :] = jnp.broadcast_to(blk[0:1], (HALO, 128))
            else:
                dst[sl, t, 0:HALO, :] = dst[1 - sl, t, TM:TM + HALO, :]

    live = {}

    def window(ref, sl, t, r, w):
        o = HALO + r - DIL * w
        return ref[sl, t, o:o + AR, :]

    def attn_qk(i, r):
        sl = i % 2
        lg = None
        for t in range(NLT):
            q = q_s[sl, t, r:r + AR, :]
            if t == 0:
                q = paced(q)
            else:
                q = after(lg[-1], q)
            prod = []
            for w in range(W):
                if w and w % G == 0:
                    q = after(prod[-1], q)
                prod.append(q * window(k_s, sl, t, r, w))
            lg = prod if lg is None else [a + b for a, b in zip(lg, prod)]
        live[i, r] = lg

    def attn_lanes(i, r):
        lane = lax.broadcasted_iota(jnp.int32, (AR, 128), 1)
        b0 = (lane & 1) == 0
        b1 = (lane & 2) == 0
        lg = [a + jnp.where(b0, pltpu.roll(a, 127, 1), pltpu.roll(a, 1, 1)) for a in live[i, r]]
        lg = [a + jnp.where(b1, pltpu.roll(a, 126, 1), pltpu.roll(a, 2, 1)) for a in lg]
        live[i, r] = lg

    def attn_softmax(i, r):
        lg = live[i, r]
        if i == 0 and r < DIL * (W - 1):
            row = lax.broadcasted_iota(jnp.int32, (AR, 128), 0) + r
            lg = [jnp.where(row >= DIL * w, a, -1000000000.0 * LOG2E) for w, a in enumerate(lg)]
        m = lg[0]
        for w in range(1, W):
            m = jnp.maximum(m, lg[w])
        e = [jnp.exp2(a - m) for a in lg]
        s = e[0]
        for w in range(1, W):
            s = s + e[w]
        inv = 1.0 / s
        live[i, r] = [a * inv for a in e]

    def attn_pv(i, r):
        sl = i % 2
        p = live.pop((i, r))
        outs = None
        for w in range(W):
            pw = after(outs[-1], p[w]) if w else p[w]
            prod = []
            for t in range(NLT):
                if t and t % G == 0:
                    pw = after(prod[-1], pw)
                prod.append(pw * window(v_s, sl, t, r, w))
            outs = prod if outs is None else [a + b for a, b in zip(outs, prod)]
        o_s[r // 2:(r + AR) // 2, :] = _pack(jnp.concatenate(outs, axis=1))

    def attn_unpermute(i, r):
        rows = slice(r // 2, (r + AR) // 2)
        o_s[rows, :] = _permute_cols(o_s[rows, :])

    def wo_part(i, r0):
        y = jnp.dot(_unpack(o_s[r0 // 2:(r0 + WR) // 2, :]), wo_v[...],
                    preferred_element_type=F32)
        done = []
        for r in range(r0, r0 + WR, LR):
            x1 = x_v[i, r:r + LR, :].astype(F32) + mod(2) * y[r - r0:r - r0 + LR]
            x1_s[i % 2, r:r + LR, :] = x1
            if done:
                x1 = jnp.concatenate([after(done[-1], x1[:, :128]), x1[:, 128:]], axis=1)
            h2 = _ln_mod(x1, mod(4), mod(3))
            done.append(h2[:, :128])
            h2_s[r // 2:(r + LR) // 2, :] = _pack(h2)

    def gate_up(cix):
        cs = slice(cix * FC, (cix + 1) * FC)
        h2 = _unpack(h2_s[...])
        g = jnp.dot(h2, wg_v[:, cs], preferred_element_type=F32)
        u = jnp.dot(h2, wu_v[:, cs], preferred_element_type=F32)
        post(g, u)
        t = 0.5 * g
        act_s[:, cs] = _pack((t + t * jnp.tanh(t)) * u)

    def down(i, n):
        cs = slice(n * DC, (n + 1) * DC)
        y = jnp.dot(_unpack(act_s[...]), wd_v[:, cs], preferred_element_type=F32)
        post(y)
        gb = mod_v[0:1, 5 * D + n * DC:5 * D + (n + 1) * DC]
        out_v[i, :, cs] = (x1_s[i % 2, :, cs] + gb * y).astype(out_v.dtype)

    def par(mxu, vpu):
        done = 0
        for idx, (fn, *args) in enumerate(mxu):
            upto = len(vpu) * (idx + 1) // len(mxu)
            for vfn, *vargs in vpu[done:upto]:
                vfn(*vargs)
            done = upto
            fn(*args)

    halves = range(D // QC)

    def t_qkv(i, js=(0, 1, 2)):
        return [(qkv_part, i, j, hf) for j in js for hf in halves]

    def t_attn(i):
        stages = (attn_qk, attn_lanes, attn_softmax, attn_pv, attn_unpermute)
        nb = TM // AR
        return [(fn, i, (n - k) * AR) for n in range(nb + len(stages) - 1)
                for k, fn in reversed(list(enumerate(stages))) if 0 <= n - k < nb]

    def t_ln(fn, i):
        return [(fn, i, r) for r in range(0, TM, LR)] if i < NT else []

    def t_wo(i):
        return [(wo_part, i, r) for r in range(0, TM, WR)]

    t_gu = [(gate_up, cix) for cix in range(NFC)]

    def t_down(i, ns):
        return [(down, i, n) for n in ns]

    def t_mod(ks):
        return [(mod_chunk_vpu, j) for k in ks for j in range(k * per, (k + 1) * per)]

    def wait(cps):
        for cp in cps:
            cp.wait()

    def chunk_cps(k):
        return [mod_cp[k], mod_cp[per + k], qkv_cp[k]]

    def modulate0(k):
        mod_chunk(k)
        mod_chunk(per + k)
        ln1_apply0(k)

    start(small_cps + [x_cp[0]] + chunk_cps(0))
    wait(small_cps)
    silu_c_columns()
    x_cp[0].wait()
    start([kv0_cp])
    par([(ln1_norm0, r) for r in range(0, TM, LR)], [])
    qkv_cp[0].wait()
    prep_qkv(0, 0)
    wait(chunk_cps(0)[:2])
    start(chunk_cps(1))
    modulate0(0)
    kv0_cp.wait()
    arrive = [chunk_cps(k) for k in range(per)]
    arrive[-1] += [x_cp[1]]
    later = [chunk_cps(k) for k in range(2, per)]
    later += [[x_cp[2]] + mod_cps(2) + [wo_cp], mod_cps(3) + mod_cps(4) + mod_cps(5)]
    steps = [(j, k) for k in range(per) for j in range(3)]
    ln_next = t_ln(ln1, 1)
    for n, (j, k) in enumerate(steps):
        if j == 2:
            if k + 1 < per:
                wait(arrive[k + 1])
            start(later[k])
            if k == 0:
                x_cp[1].start()
            if k + 1 < per:
                modulate0(k + 1)
        if n + 1 < len(steps):
            prep_qkv(*steps[n + 1])
        if n + 2 >= len(steps):
            half = len(ln_next) // 2
            par(ln_next[:half] if n + 2 == len(steps) else ln_next[half:], [])
        qkv_first(j, k)
    x_cp[2].wait()
    start([wg_cp])
    par(t_qkv(1), t_attn(0) + t_ln(ln1, 2))
    wait(mod_cps(2) + mod_cps(3) + mod_cps(4) + mod_cps(5) + [wo_cp])
    x_rest = [x_cp[i] for i in range(3, NT)]
    start([wu_cp])
    q2 = t_qkv(2)
    par(q2[:-1], t_mod((2, 3, 4)))
    start([wd_cp] + x_rest)
    par(t_wo(0), [])
    par(q2[-1:], [])
    wait([wg_cp, wu_cp])
    first, second = range(N_D1), range(N_D1, NDC)
    for i in range(1, NT):
        par(t_gu, t_attn(i) + (t_mod((5,)) if i == 1 else []))
        if i == 1:
            wait([wd_cp] + x_rest)
        par(t_down(i - 1, first), t_ln(ln1, i + 2))
        par(t_wo(i), [])
        par(t_down(i - 1, second), [])
        if i + 2 < NT:
            par(t_qkv(i + 2), [])
    out_cps[0].start()
    par(t_gu, [])
    par(t_down(NT - 1, range(NDC - 1)), [])
    out_cps[1].start()
    down(NT - 1, NDC - 1)
    out_cps[2].start()
    wait(out_cps)


@jax.jit
def pallas_adaLN_cond__sliding_local_dilated__swiglu_ffn__prompt_kernel(
    A_x: jax.Array,
    A_wqkv: jax.Array,
    A_wo: jax.Array,
    B_x: jax.Array,
    B_w_gate: jax.Array,
    B_w_up: jax.Array,
    B_w_down: jax.Array,
    c: jax.Array,
    w_mod: jax.Array,
):
    del B_x
    x = A_x.reshape(NT, TM, D)
    hbm = pl.BlockSpec(memory_space=pl.ANY)
    out = pl.pallas_call(
        _kernel,
        in_specs=[hbm] * 9,
        out_specs=hbm,
        out_shape=jax.ShapeDtypeStruct((NT, TM, D), A_x.dtype),
        scratch_shapes=[
            pltpu.VMEM((AR, 128), jnp.int32),
            pltpu.VMEM((1, D), BF16),
            pltpu.VMEM((NT, TM, D), BF16),
            pltpu.VMEM((NT, TM, D), BF16),
            pltpu.VMEM((D, 6 * D), BF16),
            pltpu.VMEM((D, 3 * D), BF16),
            pltpu.VMEM((D // 2, 3 * D), U32),
            pltpu.VMEM((D, D), BF16),
            pltpu.VMEM((D, F), BF16),
            pltpu.VMEM((D, F), BF16),
            pltpu.VMEM((F, D), BF16),
            pltpu.VMEM((8, 6 * D), F32),
            pltpu.VMEM((D, 128), F32),
            pltpu.VMEM((2, TM // 2, D), U32),
            pltpu.VMEM((2, NLT, TM, 128), F32),
            pltpu.VMEM((2, NLT, HALO + TM, 128), F32),
            pltpu.VMEM((2, NLT, HALO + TM, 128), F32),
            pltpu.VMEM((TM // 2, D), U32),
            pltpu.VMEM((2, TM, D), F32),
            pltpu.VMEM((TM // 2, D), U32),
            pltpu.VMEM((TM // 2, F), U32),
            pltpu.SemaphoreType.DMA((6 * D // MC + 9,)),
            pltpu.SemaphoreType.DMA((D // MC + 1,)),
            pltpu.SemaphoreType.DMA((NT,)),
            pltpu.SemaphoreType.DMA((3,)),
        ],
        compiler_params=pltpu.CompilerParams(
            vmem_limit_bytes=110 * 1024 * 1024,
        ),
    )(np.zeros((AR, 128), np.int32), x, c, w_mod, A_wqkv, A_wo, B_w_gate, B_w_up, B_w_down)
    return out.reshape(A_x.shape)


def _rederive():
    global NT, NFC, NDC
    NT, NFC, NDC = S // TM, F // FC, D // DC
```

```python
import jax
import jax.numpy as jnp
import numpy as np
from jax import lax
from jax.experimental import pallas as pl
from jax.experimental.pallas import tpu as pltpu

S, D, F = 2048, 1024, 3584
H, DH, W, DIL = 32, 32, 8, 2
TM = 512
NT = S // TM
HALO = 16
FC = 256
NFC = F // FC
DC = 256
NDC = D // DC
AR = 16
LR = 16
MC = 256
NLT = D // 128
QC = 512
WR = 256
N_D1 = 3
V = 3
MG = 2
NL = 4
G = 4
EPS = 1e-5
LOG2E = 1.4426950408889634
SCALE = DH ** -0.5 * LOG2E
F32, BF16, U32 = jnp.float32, jnp.bfloat16, jnp.uint32


def _swap_tiles_lanes(tiles):
    lane = lax.broadcasted_iota(jnp.int32, tiles[0].shape, 1)
    for b in range(3):
        sh = 4 << b
        low = (lane & sh) == 0
        new = list(tiles)
        for t in range(NLT):
            if not (t >> b) & 1:
                a, c = tiles[t], tiles[t | (1 << b)]
                new[t] = jnp.where(low, a, pltpu.roll(c, sh, 1))
                new[t | (1 << b)] = jnp.where(low, pltpu.roll(a, 128 - sh, 1), c)
        tiles = new
    return tiles


def _permute_cols(u):
    tiles = _swap_tiles_lanes([u[:, t * 128:(t + 1) * 128] for t in range(NLT)])
    return jnp.concatenate(tiles, axis=1)


def _pack(val):
    return pltpu.bitcast(val.astype(BF16), U32)


def _unpack(u):
    return pltpu.bitcast(u, BF16)


def _ln(x):
    m = jnp.mean(x, axis=-1, keepdims=True)
    xc = x - m
    v = jnp.mean(xc * xc, axis=-1, keepdims=True)
    return xc * lax.rsqrt(v + EPS)


def _ln_mod(x, scale1, shift):
    return _ln(x) * scale1 + shift


def _kernel(zero_hbm, x_hbm, c_hbm, wmod_hbm, wqkv_hbm, wo_hbm, wg_hbm, wu_hbm, wd_hbm, out_hbm,
            zero_v, c_v, x_v, out_v, wmod_v, wraw_v, wqkv_v, wo_v, wg_v, wu_v, wd_v, mod_v, scb_s, h_s, q_s, k_s, v_s, o_s,
            x1_s, h2_s, act_s, sems, qsems, xsems, osems):
    n_mod = 6 * D // MC

    def block_cp(src, dst, blk, sem):
        return pltpu.make_async_copy(src.at[blk], dst.at[blk], sem)

    mod_cp = [block_cp(wmod_hbm, wmod_v, (slice(None), pl.ds(j * MC, MC)), sems.at[j])
              for j in range(n_mod)]
    qkv_cp = [block_cp(wqkv_hbm, wraw_v, (pl.ds(k * MC, MC), pl.ds(0, 3 * D if k else D)),
                       qsems.at[k]) for k in range(D // MC)]
    kv0_cp = block_cp(wqkv_hbm, wraw_v, (pl.ds(0, MC), pl.ds(D, 2 * D)), qsems.at[D // MC])
    x_cp = [block_cp(x_hbm, x_v, i, xsems.at[i]) for i in range(NT)]
    last_cs = (pl.ds(0, D - DC), pl.ds(D - DC, DC))
    out_cps = [pltpu.make_async_copy(out_v.at[pl.ds(0, NT - 1)], out_hbm.at[pl.ds(0, NT - 1)],
                                     osems.at[0])]
    out_cps += [pltpu.make_async_copy(out_v.at[NT - 1, :, cs], out_hbm.at[NT - 1, :, cs],
                                      osems.at[1 + n]) for n, cs in enumerate(last_cs)]

    wo_cp = pltpu.make_async_copy(wo_hbm, wo_v, sems.at[n_mod + 3])
    wg_cp = pltpu.make_async_copy(wg_hbm, wg_v, sems.at[n_mod + 4])
    wu_cp = pltpu.make_async_copy(wu_hbm, wu_v, sems.at[n_mod + 5])
    wd_cp = pltpu.make_async_copy(wd_hbm, wd_v, sems.at[n_mod + 6])
    small_cps = [pltpu.make_async_copy(c_hbm, c_v, sems.at[n_mod + 7]),
                 pltpu.make_async_copy(zero_hbm, zero_v, sems.at[n_mod + 8])]
    per = D // MC

    def mod_cps(k):
        return mod_cp[k * per:(k + 1) * per]

    def start(cps):
        for cp in cps:
            cp.start()

    def mod_chunk(j):
        cf = c_v[...].astype(F32)
        sc = jnp.broadcast_to(cf * jax.nn.sigmoid(cf), (16, D)).astype(BF16)
        r = jnp.dot(sc, wmod_v[:, j * MC:(j + 1) * MC], preferred_element_type=F32)
        if j // per in (1, 4):
            r = r + 1.0
        mod_v[:, j * MC:(j + 1) * MC] = r[0:8]

    def silu_c_columns():
        cf = c_v[...].astype(F32)
        sc = (cf * jax.nn.sigmoid(cf)).astype(BF16).astype(F32)
        for t in range(NLT):
            blk = jnp.broadcast_to(sc[:, t * 128:(t + 1) * 128], (128, 128))
            scb_s[t * 128:(t + 1) * 128, :] = blk.T

    def mod_chunk_vpu(j):
        cs = slice(j * MC, (j + 1) * MC)
        acc = paced(jnp.zeros((AR, 128), F32))
        acc = jnp.concatenate([acc] * (MC // 128), axis=1)
        for r in range(0, D, AR):
            sc = after(acc[:, :128], scb_s[r:r + AR, :])
            sc = jnp.concatenate([sc] * (MC // 128), axis=1)
            acc = acc + wmod_v[r:r + AR, cs].astype(F32) * sc
        res = jnp.sum(acc, axis=0, keepdims=True)
        if j // per in (1, 4):
            res = res + 1.0
        mod_v[:, cs] = jnp.broadcast_to(res, (8, MC))

    tokens = []

    def after(dep, val):
        return jnp.where(zero_v[...] != 0, dep, val)

    def paced(val):
        if not tokens:
            return val
        return after(tokens.pop(0), val)

    def paced_rows(val):
        top = jnp.concatenate([paced(val[:AR, :128]), val[:AR, 128:]], axis=1)
        return jnp.concatenate([top, val[AR:]], axis=0) if val.shape[0] > AR else top

    def post(*results):
        tokens[:] = [res[TM - AR:TM, c:c + 128] for res in results
                     for c in range(0, res.shape[1], 256)]

    def mod(k):
        return mod_v[0:1, k * D:(k + 1) * D]

    def ln1(i, r):
        xv = paced_rows(x_v[i, r:r + LR, :].astype(F32))
        prev = live.pop(('ln', i, r - MG * LR), None)
        if prev is not None:
            xv = jnp.concatenate([after(prev, xv[:, :128]), xv[:, 128:]], axis=1)
        h = _ln_mod(xv, mod(1), mod(0))
        live['ln', i, r] = h[:, :128]
        h_s[i % 2, r // 2:(r + LR) // 2, :] = _pack(h)

    def ln1_norm0(r):
        x1_s[0, r:r + LR, :] = _ln(x_v[0, r:r + LR, :].astype(F32))

    def ln1_apply0(j):
        cs = slice(j * MC, (j + 1) * MC)
        h_s[0, :, cs] = _pack(x1_s[0, :, cs] * mod_v[0:1, D + j * MC:D + (j + 1) * MC]
                              + mod_v[0:1, cs])

    def prep_qkv(j, k):
        for r in range(k * MC, (k + 1) * MC, 128):
            wqkv_v[r // 2:r // 2 + 64, j * D:(j + 1) * D] = _permute_cols(
                _pack(wraw_v[r:r + 128, j * D:(j + 1) * D]))

    def qkv_first(j, k):
        res = jnp.dot(_unpack(h_s[0, :, k * MC:(k + 1) * MC]),
                      _unpack(wqkv_v[k * MC // 2:(k + 1) * MC // 2, j * D:(j + 1) * D]),
                      preferred_element_type=F32)
        post(res)
        if k > 0:
            dst, r0 = ((q_s, 0), (k_s, HALO), (v_s, HALO))[j]
            res = res + jnp.concatenate([dst[0, t, r0:r0 + TM, :] for t in range(NLT)], axis=1)
        qkv_store(0, j, 0, res, final=k == D // MC - 1)

    def qkv_part(i, j, half):
        c0 = j * D + half * QC
        res = jnp.dot(_unpack(h_s[i % 2]), _unpack(wqkv_v[:, c0:c0 + QC]),
                      preferred_element_type=F32)
        qkv_store(i, j, half, res)
        post(res)

    def qkv_store(i, j, half, res, final=True):
        sl = i % 2
        for tt in range(res.shape[1] // 128):
            t = half * (QC // 128) + tt
            blk = res[:, tt * 128:(tt + 1) * 128]
            if j == 0:
                q_s[sl, t] = blk * SCALE if final else blk
                continue
            dst = k_s if j == 1 else v_s
            dst[sl, t, HALO:HALO + TM, :] = blk
            if not final:
                continue
            if i == 0:
                dst[sl, t, 0:HALO, :] = jnp.broadcast_to(blk[0:1], (HALO, 128))
            else:
                dst[sl, t, 0:HALO, :] = dst[1 - sl, t, TM:TM + HALO, :]

    live = {}

    def window(ref, sl, t, r, w):
        o = HALO + r - DIL * w
        return ref[sl, t, o:o + AR, :]

    def attn_qk(i, r):
        sl = i % 2
        lg = None
        for t in range(NLT):
            q = q_s[sl, t, r:r + AR, :]
            if t == 0:
                q = paced(q)
            else:
                q = after(lg[-1], q)
            prod = []
            for w in range(W):
                if w and w % G == 0:
                    q = after(prod[-1], q)
                prod.append(q * window(k_s, sl, t, r, w))
            lg = prod if lg is None else [a + b for a, b in zip(lg, prod)]
        live[i, r] = lg

    def attn_lanes(i, r):
        lane = lax.broadcasted_iota(jnp.int32, (AR, 128), 1)
        b0 = (lane & 1) == 0
        b1 = (lane & 2) == 0
        lg = [a + jnp.where(b0, pltpu.roll(a, 127, 1), pltpu.roll(a, 1, 1)) for a in live[i, r]]
        lg = [a + jnp.where(b1, pltpu.roll(a, 126, 1), pltpu.roll(a, 2, 1)) for a in lg]
        live[i, r] = lg

    def attn_softmax(i, r):
        lg = live[i, r]
        if i == 0 and r < DIL * (W - 1):
            row = lax.broadcasted_iota(jnp.int32, (AR, 128), 0) + r
            lg = [jnp.where(row >= DIL * w, a, -1000000000.0 * LOG2E) for w, a in enumerate(lg)]
        m = lg[0]
        for w in range(1, W):
            m = jnp.maximum(m, lg[w])
        e = [jnp.exp2(a - m) for a in lg]
        s = e[0]
        for w in range(1, W):
            s = s + e[w]
        inv = 1.0 / s
        live[i, r] = [a * inv for a in e]

    def attn_pv(i, r):
        sl = i % 2
        p = live.pop((i, r))
        outs = None
        for w in range(W):
            pw = after(outs[-1], p[w]) if w else p[w]
            prod = []
            for t in range(NLT):
                if t and t % G == 0:
                    pw = after(prod[-1], pw)
                prod.append(pw * window(v_s, sl, t, r, w))
            outs = prod if outs is None else [a + b for a, b in zip(outs, prod)]
        o_s[r // 2:(r + AR) // 2, :] = _pack(jnp.concatenate(outs, axis=1))

    def attn_unpermute(i, r):
        rows = slice(r // 2, (r + AR) // 2)
        o_s[rows, :] = _permute_cols(o_s[rows, :])

    def wo_part(i, r0):
        y = jnp.dot(_unpack(o_s[r0 // 2:(r0 + WR) // 2, :]), wo_v[...],
                    preferred_element_type=F32)
        done = []
        for r in range(r0, r0 + WR, LR):
            x1 = x_v[i, r:r + LR, :].astype(F32) + mod(2) * y[r - r0:r - r0 + LR]
            x1_s[i % 2, r:r + LR, :] = x1
            if done:
                x1 = jnp.concatenate([after(done[-1], x1[:, :128]), x1[:, 128:]], axis=1)
            h2 = _ln_mod(x1, mod(4), mod(3))
            done.append(h2[:, :128])
            h2_s[r // 2:(r + LR) // 2, :] = _pack(h2)

    def gate_up(cix):
        cs = slice(cix * FC, (cix + 1) * FC)
        h2 = _unpack(h2_s[...])
        g = jnp.dot(h2, wg_v[:, cs], preferred_element_type=F32)
        u = jnp.dot(h2, wu_v[:, cs], preferred_element_type=F32)
        post(g, u)
        t = 0.5 * g
        act_s[:, cs] = _pack((t + t * jnp.tanh(t)) * u)

    def down(i, n):
        cs = slice(n * DC, (n + 1) * DC)
        y = jnp.dot(_unpack(act_s[...]), wd_v[:, cs], preferred_element_type=F32)
        post(y)
        gb = mod_v[0:1, 5 * D + n * DC:5 * D + (n + 1) * DC]
        out_v[i, :, cs] = (x1_s[i % 2, :, cs] + gb * y).astype(out_v.dtype)

    def par(mxu, vpu):
        done = 0
        for idx, (fn, *args) in enumerate(mxu):
            upto = len(vpu) * (idx + 1) // len(mxu)
            for vfn, *vargs in vpu[done:upto]:
                vfn(*vargs)
            done = upto
            fn(*args)

    def weave(a, b):
        keyed = [((n + 0.5) / len(ts), t) for ts in (a, b) for n, t in enumerate(ts)]
        return [t for _, t in sorted(keyed, key=lambda kt: kt[0])]

    halves = range(D // QC)

    def t_qkv(i, js=(0, 1, 2)):
        return [(qkv_part, i, j, hf) for j in js for hf in halves]

    def t_attn(i):
        stages = (attn_qk, attn_lanes, attn_softmax, attn_pv, attn_unpermute)
        nb = TM // AR
        return [(fn, i, (n - k) * AR) for n in range(nb + len(stages) - 1)
                for k, fn in reversed(list(enumerate(stages))) if 0 <= n - k < nb]

    def t_ln(fn, i):
        return [(fn, i, r) for r in range(0, TM, LR)] if i < NT else []

    def t_wo(i):
        return [(wo_part, i, r) for r in range(0, TM, WR)]

    t_gu = [(gate_up, cix) for cix in range(NFC)]

    def t_down(i, ns):
        return [(down, i, n) for n in ns]

    def t_mod(ks):
        return [(mod_chunk_vpu, j) for k in ks for j in range(k * per, (k + 1) * per)]

    def wait(cps):
        for cp in cps:
            cp.wait()

    def chunk_cps(k):
        return [mod_cp[k], mod_cp[per + k], qkv_cp[k]]

    def modulate0(k):
        tokens.clear()
        for j in (k, per + k):
            (mod_chunk_vpu if k else mod_chunk)(j)
        ln1_apply0(k)

    start(small_cps + [x_cp[0]] + chunk_cps(0))
    wait(small_cps)
    silu_c_columns()
    x_cp[0].wait()
    start([kv0_cp])
    par([(ln1_norm0, r) for r in range(0, TM, LR)], [])
    qkv_cp[0].wait()
    prep_qkv(0, 0)
    wait(chunk_cps(0)[:2])
    start(chunk_cps(1))
    modulate0(0)
    kv0_cp.wait()
    arrive = [chunk_cps(k) for k in range(per)]
    arrive[-1] += [x_cp[1]]
    later = [chunk_cps(k) for k in range(2, per)]
    later += [[x_cp[2]] + mod_cps(2) + [wo_cp], mod_cps(3) + mod_cps(4) + mod_cps(5)]
    steps = [(j, k) for k in range(per) for j in range(3)]
    ln_next = t_ln(ln1, 1)
    for n, (j, k) in enumerate(steps):
        if j == 2:
            if k + 1 < per:
                wait(arrive[k + 1])
            start(later[k])
            if k == 0:
                x_cp[1].start()
            if k + 1 < per:
                modulate0(k + 1)
        if n + 1 < len(steps):
            prep_qkv(*steps[n + 1])
        left = len(steps) - n
        if left <= NL:
            q = len(ln_next) // NL
            par(ln_next[(NL - left) * q:(NL - left + 1) * q], [])
        qkv_first(j, k)
    x_cp[2].wait()
    start([wg_cp])
    par(t_qkv(1), weave(t_attn(0), t_ln(ln1, 2)) if V & 1 else t_attn(0) + t_ln(ln1, 2))
    wait(mod_cps(2) + mod_cps(3) + mod_cps(4) + mod_cps(5) + [wo_cp])
    x_rest = [x_cp[i] for i in range(3, NT)]
    start([wu_cp])
    q2 = t_qkv(2)
    par(q2[:-1], t_mod((2, 3, 4)))
    start([wd_cp] + x_rest)
    par(t_wo(0), [])
    par(q2[-1:], [])
    wait([wg_cp, wu_cp])
    first, second = range(N_D1), range(N_D1, NDC)
    for i in range(1, NT):
        par(t_gu, (weave if V & 2 else lambda a, b: a + b)(t_attn(i), t_mod((5,)) if i == 1 else []))
        if i == 1:
            wait([wd_cp] + x_rest)
        par(t_down(i - 1, first), t_ln(ln1, i + 2))
        par(t_wo(i), [])
        par(t_down(i - 1, second), [])
        if i + 2 < NT:
            par(t_qkv(i + 2), [])
    out_cps[0].start()
    par(t_gu, [])
    par(t_down(NT - 1, range(NDC - 1)), [])
    out_cps[1].start()
    down(NT - 1, NDC - 1)
    out_cps[2].start()
    wait(out_cps)


@jax.jit
def pallas_adaLN_cond__sliding_local_dilated__swiglu_ffn__prompt_kernel(
    A_x: jax.Array,
    A_wqkv: jax.Array,
    A_wo: jax.Array,
    B_x: jax.Array,
    B_w_gate: jax.Array,
    B_w_up: jax.Array,
    B_w_down: jax.Array,
    c: jax.Array,
    w_mod: jax.Array,
):
    del B_x
    x = A_x.reshape(NT, TM, D)
    hbm = pl.BlockSpec(memory_space=pl.ANY)
    out = pl.pallas_call(
        _kernel,
        in_specs=[hbm] * 9,
        out_specs=hbm,
        out_shape=jax.ShapeDtypeStruct((NT, TM, D), A_x.dtype),
        scratch_shapes=[
            pltpu.VMEM((AR, 128), jnp.int32),
            pltpu.VMEM((1, D), BF16),
            pltpu.VMEM((NT, TM, D), BF16),
            pltpu.VMEM((NT, TM, D), BF16),
            pltpu.VMEM((D, 6 * D), BF16),
            pltpu.VMEM((D, 3 * D), BF16),
            pltpu.VMEM((D // 2, 3 * D), U32),
            pltpu.VMEM((D, D), BF16),
            pltpu.VMEM((D, F), BF16),
            pltpu.VMEM((D, F), BF16),
            pltpu.VMEM((F, D), BF16),
            pltpu.VMEM((8, 6 * D), F32),
            pltpu.VMEM((D, 128), F32),
            pltpu.VMEM((2, TM // 2, D), U32),
            pltpu.VMEM((2, NLT, TM, 128), F32),
            pltpu.VMEM((2, NLT, HALO + TM, 128), F32),
            pltpu.VMEM((2, NLT, HALO + TM, 128), F32),
            pltpu.VMEM((TM // 2, D), U32),
            pltpu.VMEM((2, TM, D), F32),
            pltpu.VMEM((TM // 2, D), U32),
            pltpu.VMEM((TM // 2, F), U32),
            pltpu.SemaphoreType.DMA((6 * D // MC + 9,)),
            pltpu.SemaphoreType.DMA((D // MC + 1,)),
            pltpu.SemaphoreType.DMA((NT,)),
            pltpu.SemaphoreType.DMA((3,)),
        ],
        compiler_params=pltpu.CompilerParams(
            vmem_limit_bytes=110 * 1024 * 1024,
        ),
    )(np.zeros((AR, 128), np.int32), x, c, w_mod, A_wqkv, A_wo, B_w_gate, B_w_up, B_w_down)
    return out.reshape(A_x.shape)


def _rederive():
    global NT, NFC, NDC
    NT, NFC, NDC = S // TM, F // FC, D // DC
```

```python
import jax
import jax.numpy as jnp
import numpy as np
from jax import lax
from jax.experimental import pallas as pl
from jax.experimental.pallas import tpu as pltpu

S, D, F = 2048, 1024, 3584
H, DH, W, DIL = 32, 32, 8, 2
TM = 512
NT = S // TM
HALO = 16
FC = 256
NFC = F // FC
DC = 256
NDC = D // DC
AR = 16
LR = 16
MC = 256
NLT = D // 128
QC = 512
WR = 256
N_D1 = 2
V = 0
MG = 2
NL = 4
G = 4
EPS = 1e-5
LOG2E = 1.4426950408889634
SCALE = DH ** -0.5 * LOG2E
F32, BF16, U32 = jnp.float32, jnp.bfloat16, jnp.uint32


def _swap_tiles_lanes(tiles):
    lane = lax.broadcasted_iota(jnp.int32, tiles[0].shape, 1)
    for b in range(3):
        sh = 4 << b
        low = (lane & sh) == 0
        new = list(tiles)
        for t in range(NLT):
            if not (t >> b) & 1:
                a, c = tiles[t], tiles[t | (1 << b)]
                new[t] = jnp.where(low, a, pltpu.roll(c, sh, 1))
                new[t | (1 << b)] = jnp.where(low, pltpu.roll(a, 128 - sh, 1), c)
        tiles = new
    return tiles


def _permute_cols(u):
    tiles = _swap_tiles_lanes([u[:, t * 128:(t + 1) * 128] for t in range(NLT)])
    return jnp.concatenate(tiles, axis=1)


def _pack(val):
    return pltpu.bitcast(val.astype(BF16), U32)


def _unpack(u):
    return pltpu.bitcast(u, BF16)


def _ln(x):
    m = jnp.mean(x, axis=-1, keepdims=True)
    xc = x - m
    v = jnp.mean(xc * xc, axis=-1, keepdims=True)
    return xc * lax.rsqrt(v + EPS)


def _ln_mod(x, scale1, shift):
    return _ln(x) * scale1 + shift


def _kernel(zero_hbm, x_hbm, c_hbm, wmod_hbm, wqkv_hbm, wo_hbm, wg_hbm, wu_hbm, wd_hbm, out_hbm,
            zero_v, c_v, x_v, out_v, wmod_v, wraw_v, wqkv_v, wo_v, wg_v, wu_v, wd_v, mod_v, scb_s, h_s, q_s, k_s, v_s, o_s,
            x1_s, h2_s, act_s, sems, qsems, xsems, osems):
    n_mod = 6 * D // MC

    def block_cp(src, dst, blk, sem):
        return pltpu.make_async_copy(src.at[blk], dst.at[blk], sem)

    mod_cp = [block_cp(wmod_hbm, wmod_v, (slice(None), pl.ds(j * MC, MC)), sems.at[j])
              for j in range(n_mod)]
    qkv_cp = [block_cp(wqkv_hbm, wraw_v, (pl.ds(k * MC, MC), pl.ds(0, 3 * D if k else D)),
                       qsems.at[k]) for k in range(D // MC)]
    kv0_cp = block_cp(wqkv_hbm, wraw_v, (pl.ds(0, MC), pl.ds(D, 2 * D)), qsems.at[D // MC])
    x_cp = [block_cp(x_hbm, x_v, i, xsems.at[i]) for i in range(NT)]
    last_cs = (pl.ds(0, D - DC), pl.ds(D - DC, DC))
    out_cps = [pltpu.make_async_copy(out_v.at[pl.ds(0, NT - 1)], out_hbm.at[pl.ds(0, NT - 1)],
                                     osems.at[0])]
    out_cps += [pltpu.make_async_copy(out_v.at[NT - 1, :, cs], out_hbm.at[NT - 1, :, cs],
                                      osems.at[1 + n]) for n, cs in enumerate(last_cs)]

    wo_cp = pltpu.make_async_copy(wo_hbm, wo_v, sems.at[n_mod + 3])
    wg_cp = pltpu.make_async_copy(wg_hbm, wg_v, sems.at[n_mod + 4])
    wu_cp = pltpu.make_async_copy(wu_hbm, wu_v, sems.at[n_mod + 5])
    wd_cp = pltpu.make_async_copy(wd_hbm, wd_v, sems.at[n_mod + 6])
    small_cps = [pltpu.make_async_copy(c_hbm, c_v, sems.at[n_mod + 7]),
                 pltpu.make_async_copy(zero_hbm, zero_v, sems.at[n_mod + 8])]
    per = D // MC

    def mod_cps(k):
        return mod_cp[k * per:(k + 1) * per]

    def start(cps):
        for cp in cps:
            cp.start()

    def mod_chunk(j):
        cf = c_v[...].astype(F32)
        sc = jnp.broadcast_to(cf * jax.nn.sigmoid(cf), (16, D)).astype(BF16)
        r = jnp.dot(sc, wmod_v[:, j * MC:(j + 1) * MC], preferred_element_type=F32)
        if j // per in (1, 4):
            r = r + 1.0
        mod_v[:, j * MC:(j + 1) * MC] = r[0:8]

    def silu_c_columns():
        cf = c_v[...].astype(F32)
        sc = (cf * jax.nn.sigmoid(cf)).astype(BF16).astype(F32)
        for t in range(NLT):
            blk = jnp.broadcast_to(sc[:, t * 128:(t + 1) * 128], (128, 128))
            scb_s[t * 128:(t + 1) * 128, :] = blk.T

    def mod_chunk_vpu(j):
        cs = slice(j * MC, (j + 1) * MC)
        acc = paced(jnp.zeros((AR, 128), F32))
        acc = jnp.concatenate([acc] * (MC // 128), axis=1)
        for r in range(0, D, AR):
            sc = after(acc[:, :128], scb_s[r:r + AR, :])
            sc = jnp.concatenate([sc] * (MC // 128), axis=1)
            acc = acc + wmod_v[r:r + AR, cs].astype(F32) * sc
        res = jnp.sum(acc, axis=0, keepdims=True)
        if j // per in (1, 4):
            res = res + 1.0
        mod_v[:, cs] = jnp.broadcast_to(res, (8, MC))

    tokens = []

    def after(dep, val):
        return jnp.where(zero_v[...] != 0, dep, val)

    def paced(val):
        if not tokens:
            return val
        return after(tokens.pop(0), val)

    def paced_rows(val):
        top = jnp.concatenate([paced(val[:AR, :128]), val[:AR, 128:]], axis=1)
        return jnp.concatenate([top, val[AR:]], axis=0) if val.shape[0] > AR else top

    def post(*results):
        tokens[:] = [res[TM - AR:TM, c:c + 128] for c0 in (0, 128)
                     for res in results for c in range(c0, res.shape[1], 256)]

    def mod(k):
        return mod_v[0:1, k * D:(k + 1) * D]

    def ln1(i, r):
        xv = paced_rows(x_v[i, r:r + LR, :].astype(F32))
        prev = live.pop(('ln', i, r - MG * LR), None)
        if prev is not None:
            xv = jnp.concatenate([after(prev, xv[:, :128]), xv[:, 128:]], axis=1)
        h = _ln_mod(xv, mod(1), mod(0))
        live['ln', i, r] = h[:, :128]
        h_s[i % 2, r // 2:(r + LR) // 2, :] = _pack(h)

    def ln1_norm0(r):
        x1_s[0, r:r + LR, :] = _ln(x_v[0, r:r + LR, :].astype(F32))

    def ln1_apply0(j):
        cs = slice(j * MC, (j + 1) * MC)
        h_s[0, :, cs] = _pack(x1_s[0, :, cs] * mod_v[0:1, D + j * MC:D + (j + 1) * MC]
                              + mod_v[0:1, cs])

    def prep_qkv(j, k):
        for r in range(k * MC, (k + 1) * MC, 128):
            wqkv_v[r // 2:r // 2 + 64, j * D:(j + 1) * D] = _permute_cols(
                _pack(wraw_v[r:r + 128, j * D:(j + 1) * D]))

    def qkv_first(j, k):
        res = jnp.dot(_unpack(h_s[0, :, k * MC:(k + 1) * MC]),
                      _unpack(wqkv_v[k * MC // 2:(k + 1) * MC // 2, j * D:(j + 1) * D]),
                      preferred_element_type=F32)
        post(res)
        if k > 0:
            dst, r0 = ((q_s, 0), (k_s, HALO), (v_s, HALO))[j]
            res = res + jnp.concatenate([dst[0, t, r0:r0 + TM, :] for t in range(NLT)], axis=1)
        qkv_store(0, j, 0, res, final=k == D // MC - 1)

    def qkv_part(i, j, half):
        c0 = j * D + half * QC
        res = jnp.dot(_unpack(h_s[i % 2]), _unpack(wqkv_v[:, c0:c0 + QC]),
                      preferred_element_type=F32)
        qkv_store(i, j, half, res)
        post(res)

    def qkv_store(i, j, half, res, final=True):
        sl = i % 2
        for tt in range(res.shape[1] // 128):
            t = half * (QC // 128) + tt
            blk = res[:, tt * 128:(tt + 1) * 128]
            if j == 0:
                q_s[sl, t] = blk * SCALE if final else blk
                continue
            dst = k_s if j == 1 else v_s
            dst[sl, t, HALO:HALO + TM, :] = blk
            if not final:
                continue
            if i == 0:
                dst[sl, t, 0:HALO, :] = jnp.broadcast_to(blk[0:1], (HALO, 128))
            else:
                dst[sl, t, 0:HALO, :] = dst[1 - sl, t, TM:TM + HALO, :]

    live = {}

    def window(ref, sl, t, r, w):
        o = HALO + r - DIL * w
        return ref[sl, t, o:o + AR, :]

    def attn_qk(i, r):
        sl = i % 2
        lg = None
        for t in range(NLT):
            q = q_s[sl, t, r:r + AR, :]
            if t == 0:
                q = paced(q)
            else:
                q = after(lg[-1], q)
            prod = []
            for w in range(W):
                if w and w % G == 0:
                    q = after(prod[-1], q)
                prod.append(q * window(k_s, sl, t, r, w))
            lg = prod if lg is None else [a + b for a, b in zip(lg, prod)]
        live[i, r] = lg

    def attn_lanes(i, r):
        lane = lax.broadcasted_iota(jnp.int32, (AR, 128), 1)
        b0 = (lane & 1) == 0
        b1 = (lane & 2) == 0
        lg = [a + jnp.where(b0, pltpu.roll(a, 127, 1), pltpu.roll(a, 1, 1)) for a in live[i, r]]
        lg = [a + jnp.where(b1, pltpu.roll(a, 126, 1), pltpu.roll(a, 2, 1)) for a in lg]
        live[i, r] = lg

    def attn_softmax(i, r):
        lg = live[i, r]
        if i == 0 and r < DIL * (W - 1):
            row = lax.broadcasted_iota(jnp.int32, (AR, 128), 0) + r
            lg = [jnp.where(row >= DIL * w, a, -1000000000.0 * LOG2E) for w, a in enumerate(lg)]
        m = lg[0]
        for w in range(1, W):
            m = jnp.maximum(m, lg[w])
        e = []
        for w, a in enumerate(lg):
            if w and w % 2 == 0:
                m = after(e[-1], m)
            e.append(jnp.exp2(a - m))
        s = e[0]
        for w in range(1, W):
            s = s + e[w]
        inv = 1.0 / s
        live[i, r] = [a * inv for a in e]

    def attn_pv(i, r):
        sl = i % 2
        p = live.pop((i, r))
        outs = None
        for w in range(W):
            pw = after(outs[-1], p[w]) if w else p[w]
            prod = []
            for t in range(NLT):
                if t and t % G == 0:
                    pw = after(prod[-1], pw)
                prod.append(pw * window(v_s, sl, t, r, w))
            outs = prod if outs is None else [a + b for a, b in zip(outs, prod)]
        o_s[r // 2:(r + AR) // 2, :] = _pack(jnp.concatenate(outs, axis=1))

    def attn_unpermute(i, r):
        rows = slice(r // 2, (r + AR) // 2)
        o_s[rows, :] = _permute_cols(o_s[rows, :])

    def wo_part(i, r0):
        y = jnp.dot(_unpack(o_s[r0 // 2:(r0 + WR) // 2, :]), wo_v[...],
                    preferred_element_type=F32)
        done = []
        for r in range(r0, r0 + WR, LR):
            x1 = x_v[i, r:r + LR, :].astype(F32) + mod(2) * y[r - r0:r - r0 + LR]
            x1_s[i % 2, r:r + LR, :] = x1
            if done:
                x1 = jnp.concatenate([after(done[-1], x1[:, :128]), x1[:, 128:]], axis=1)
            h2 = _ln_mod(x1, mod(4), mod(3))
            done.append(h2[:, :128])
            h2_s[r // 2:(r + LR) // 2, :] = _pack(h2)

    def gate_up(cix):
        cs = slice(cix * FC, (cix + 1) * FC)
        h2 = _unpack(h2_s[...])
        g = jnp.dot(h2, wg_v[:, cs], preferred_element_type=F32)
        u = jnp.dot(h2, wu_v[:, cs], preferred_element_type=F32)
        post(g, u)
        t = 0.5 * g
        act_s[:, cs] = _pack((t + t * jnp.tanh(t)) * u)

    def down(i, n):
        cs = slice(n * DC, (n + 1) * DC)
        y = jnp.dot(_unpack(act_s[...]), wd_v[:, cs], preferred_element_type=F32)
        post(y)
        gb = mod_v[0:1, 5 * D + n * DC:5 * D + (n + 1) * DC]
        out_v[i, :, cs] = (x1_s[i % 2, :, cs] + gb * y).astype(out_v.dtype)

    def par(mxu, vpu):
        done = 0
        for idx, (fn, *args) in enumerate(mxu):
            upto = len(vpu) * (idx + 1) // len(mxu)
            for vfn, *vargs in vpu[done:upto]:
                vfn(*vargs)
            done = upto
            fn(*args)

    def weave(a, b):
        keyed = [((n + 0.5) / len(ts), t) for ts in (a, b) for n, t in enumerate(ts)]
        return [t for _, t in sorted(keyed, key=lambda kt: kt[0])]

    halves = range(D // QC)

    def t_qkv(i, js=(0, 1, 2)):
        return [(qkv_part, i, j, hf) for j in js for hf in halves]

    def t_attn(i):
        stages = (attn_qk, attn_lanes, attn_softmax, attn_pv, attn_unpermute)
        nb = TM // AR
        return [(fn, i, (n - k) * AR) for n in range(nb + len(stages) - 1)
                for k, fn in reversed(list(enumerate(stages))) if 0 <= n - k < nb]

    def t_ln(fn, i):
        return [(fn, i, r) for r in range(0, TM, LR)] if i < NT else []

    def t_wo(i):
        return [(wo_part, i, r) for r in range(0, TM, WR)]

    t_gu = [(gate_up, cix) for cix in range(NFC)]

    def t_down(i, ns):
        return [(down, i, n) for n in ns]

    def t_mod(ks):
        return [(mod_chunk_vpu, j) for k in ks for j in range(k * per, (k + 1) * per)]

    def wait(cps):
        for cp in cps:
            cp.wait()

    def chunk_cps(k):
        return [mod_cp[k], mod_cp[per + k], qkv_cp[k]]

    def modulate0(k):
        tokens.clear()
        for j in (k, per + k):
            (mod_chunk_vpu if k else mod_chunk)(j)
        ln1_apply0(k)

    start(small_cps + [x_cp[0]] + chunk_cps(0))
    wait(small_cps)
    silu_c_columns()
    x_cp[0].wait()
    start([kv0_cp])
    par([(ln1_norm0, r) for r in range(0, TM, LR)], [])
    qkv_cp[0].wait()
    prep_qkv(0, 0)
    wait(chunk_cps(0)[:2])
    start(chunk_cps(1))
    modulate0(0)
    kv0_cp.wait()
    arrive = [chunk_cps(k) for k in range(per)]
    arrive[-1] += [x_cp[1]]
    later = [chunk_cps(k) for k in range(2, per)]
    later += [[x_cp[2]] + mod_cps(2) + [wo_cp], mod_cps(3) + mod_cps(4) + mod_cps(5)]
    steps = [(j, k) for k in range(per) for j in range(3)]
    ln_next = t_ln(ln1, 1)
    for n, (j, k) in enumerate(steps):
        if j == 2:
            if k + 1 < per:
                wait(arrive[k + 1])
            start(later[k])
            if k == 0:
                x_cp[1].start()
            if k + 1 < per:
                modulate0(k + 1)
        if n + 1 < len(steps):
            prep_qkv(*steps[n + 1])
        left = len(steps) - n
        if left <= NL:
            q = len(ln_next) // NL
            par(ln_next[(NL - left) * q:(NL - left + 1) * q], [])
        qkv_first(j, k)
    x_cp[2].wait()
    start([wg_cp])
    par(t_qkv(1), weave(t_attn(0), t_ln(ln1, 2)))
    wait(mod_cps(2) + mod_cps(3) + mod_cps(4) + mod_cps(5) + [wo_cp])
    x_rest = [x_cp[i] for i in range(3, NT)]
    start([wu_cp])
    q2 = t_qkv(2)
    par(q2[:-1], t_mod((2, 3, 4)))
    start([wd_cp] + x_rest)
    par(t_wo(0), [])
    par(q2[-1:], [])
    wait([wg_cp, wu_cp])
    first, second = range(N_D1), range(N_D1, NDC)
    for i in range(1, NT):
        par(t_gu, weave(t_attn(i), t_mod((5,)) if i == 1 else []))
        if i == 1:
            wait([wd_cp] + x_rest)
        par(t_down(i - 1, first), t_ln(ln1, i + 2))
        par(t_wo(i), [])
        par(t_down(i - 1, second), [])
        if i + 2 < NT:
            par(t_qkv(i + 2), [])
    out_cps[0].start()
    par(t_gu, [])
    par(t_down(NT - 1, range(NDC - 1)), [])
    out_cps[1].start()
    down(NT - 1, NDC - 1)
    out_cps[2].start()
    wait(out_cps)


@jax.jit
def pallas_adaLN_cond__sliding_local_dilated__swiglu_ffn__prompt_kernel(
    A_x: jax.Array,
    A_wqkv: jax.Array,
    A_wo: jax.Array,
    B_x: jax.Array,
    B_w_gate: jax.Array,
    B_w_up: jax.Array,
    B_w_down: jax.Array,
    c: jax.Array,
    w_mod: jax.Array,
):
    del B_x
    x = A_x.reshape(NT, TM, D)
    hbm = pl.BlockSpec(memory_space=pl.ANY)
    out = pl.pallas_call(
        _kernel,
        in_specs=[hbm] * 9,
        out_specs=hbm,
        out_shape=jax.ShapeDtypeStruct((NT, TM, D), A_x.dtype),
        scratch_shapes=[
            pltpu.VMEM((AR, 128), jnp.int32),
            pltpu.VMEM((1, D), BF16),
            pltpu.VMEM((NT, TM, D), BF16),
            pltpu.VMEM((NT, TM, D), BF16),
            pltpu.VMEM((D, 6 * D), BF16),
            pltpu.VMEM((D, 3 * D), BF16),
            pltpu.VMEM((D // 2, 3 * D), U32),
            pltpu.VMEM((D, D), BF16),
            pltpu.VMEM((D, F), BF16),
            pltpu.VMEM((D, F), BF16),
            pltpu.VMEM((F, D), BF16),
            pltpu.VMEM((8, 6 * D), F32),
            pltpu.VMEM((D, 128), F32),
            pltpu.VMEM((2, TM // 2, D), U32),
            pltpu.VMEM((2, NLT, TM, 128), F32),
            pltpu.VMEM((2, NLT, HALO + TM, 128), F32),
            pltpu.VMEM((2, NLT, HALO + TM, 128), F32),
            pltpu.VMEM((TM // 2, D), U32),
            pltpu.VMEM((2, TM, D), F32),
            pltpu.VMEM((TM // 2, D), U32),
            pltpu.VMEM((TM // 2, F), U32),
            pltpu.SemaphoreType.DMA((6 * D // MC + 9,)),
            pltpu.SemaphoreType.DMA((D // MC + 1,)),
            pltpu.SemaphoreType.DMA((NT,)),
            pltpu.SemaphoreType.DMA((3,)),
        ],
        compiler_params=pltpu.CompilerParams(
            vmem_limit_bytes=110 * 1024 * 1024,
        ),
    )(np.zeros((AR, 128), np.int32), x, c, w_mod, A_wqkv, A_wo, B_w_gate, B_w_up, B_w_down)
    return out.reshape(A_x.shape)


def _rederive():
    global NT, NFC, NDC
    NT, NFC, NDC = S // TM, F // FC, D // DC
```

```python
import jax
import jax.numpy as jnp
import numpy as np
from jax import lax
from jax.experimental import pallas as pl
from jax.experimental.pallas import tpu as pltpu

S, D, F = 2048, 1024, 3584
H, DH, W, DIL = 32, 32, 8, 2
TM = 512
NT = S // TM
HALO = 16
FC = 256
NFC = F // FC
DC = 128
NDC = D // DC
AR = 16
LR = 16
MC = 256
NLT = D // 128
QC = 512
WR = 256
N_D1 = 4
NA = 140
MG = 2
NL = 2
G = (8, 3)
EPS = 1e-5
LOG2E = 1.4426950408889634
SCALE = DH ** -0.5 * LOG2E
F32, BF16, U32 = jnp.float32, jnp.bfloat16, jnp.uint32


def _swap_tiles_lanes(tiles):
    lane = lax.broadcasted_iota(jnp.int32, tiles[0].shape, 1)
    for b in range(3):
        sh = 4 << b
        low = (lane & sh) == 0
        new = list(tiles)
        for t in range(NLT):
            if not (t >> b) & 1:
                a, c = tiles[t], tiles[t | (1 << b)]
                new[t] = jnp.where(low, a, pltpu.roll(c, sh, 1))
                new[t | (1 << b)] = jnp.where(low, pltpu.roll(a, 128 - sh, 1), c)
        tiles = new
    return tiles


def _permute_cols(u):
    tiles = _swap_tiles_lanes([u[:, t * 128:(t + 1) * 128] for t in range(NLT)])
    return jnp.concatenate(tiles, axis=1)


def _pack(val):
    return pltpu.bitcast(val.astype(BF16), U32)


def _unpack(u):
    return pltpu.bitcast(u, BF16)


def _ln(x):
    m = jnp.mean(x, axis=-1, keepdims=True)
    xc = x - m
    v = jnp.mean(xc * xc, axis=-1, keepdims=True)
    return xc * lax.rsqrt(v + EPS)


def _ln_mod(x, scale1, shift):
    return _ln(x) * scale1 + shift


def _kernel(zero_hbm, x_hbm, c_hbm, wmod_hbm, wqkv_hbm, wo_hbm, wg_hbm, wu_hbm, wd_hbm, out_hbm,
            zero_v, c_v, x_v, out_v, wmod_v, wraw_v, wqkv_v, wo_v, wg_v, wu_v, wd_v, mod_v, scb_s, h_s, q_s, k_s, v_s, o_s,
            x1_s, h2_s, act_s, sems, qsems, xsems, osems):
    n_mod = 6 * D // MC

    def block_cp(src, dst, blk, sem):
        return pltpu.make_async_copy(src.at[blk], dst.at[blk], sem)

    mod_cp = [block_cp(wmod_hbm, wmod_v, (slice(None), pl.ds(j * MC, MC)), sems.at[j])
              for j in range(n_mod)]
    qkv_cp = [block_cp(wqkv_hbm, wraw_v, (pl.ds(k * MC, MC), pl.ds(0, 3 * D if k else D)),
                       qsems.at[k]) for k in range(D // MC)]
    kv0_cp = block_cp(wqkv_hbm, wraw_v, (pl.ds(0, MC), pl.ds(D, 2 * D)), qsems.at[D // MC])
    x_cp = [block_cp(x_hbm, x_v, i, xsems.at[i]) for i in range(NT)]
    last_cs = (pl.ds(0, D - DC), pl.ds(D - DC, DC))
    out_cps = [pltpu.make_async_copy(out_v.at[pl.ds(0, NT - 1)], out_hbm.at[pl.ds(0, NT - 1)],
                                     osems.at[0])]
    out_cps += [pltpu.make_async_copy(out_v.at[NT - 1, :, cs], out_hbm.at[NT - 1, :, cs],
                                      osems.at[1 + n]) for n, cs in enumerate(last_cs)]

    wo_cp = pltpu.make_async_copy(wo_hbm, wo_v, sems.at[n_mod + 3])
    wg_cp = pltpu.make_async_copy(wg_hbm, wg_v, sems.at[n_mod + 4])
    wu_cp = pltpu.make_async_copy(wu_hbm, wu_v, sems.at[n_mod + 5])
    wd_cp = pltpu.make_async_copy(wd_hbm, wd_v, sems.at[n_mod + 6])
    small_cps = [pltpu.make_async_copy(c_hbm, c_v, sems.at[n_mod + 7]),
                 pltpu.make_async_copy(zero_hbm, zero_v, sems.at[n_mod + 8])]
    per = D // MC

    def mod_cps(k):
        return mod_cp[k * per:(k + 1) * per]

    def start(cps):
        for cp in cps:
            cp.start()

    def mod_chunk(j):
        cf = c_v[...].astype(F32)
        sc = jnp.broadcast_to(cf * jax.nn.sigmoid(cf), (16, D)).astype(BF16)
        r = jnp.dot(sc, wmod_v[:, j * MC:(j + 1) * MC], preferred_element_type=F32)
        if j // per in (1, 4):
            r = r + 1.0
        mod_v[:, j * MC:(j + 1) * MC] = r[0:8]

    def silu_c_columns():
        cf = c_v[...].astype(F32)
        sc = (cf * jax.nn.sigmoid(cf)).astype(BF16).astype(F32)
        for t in range(NLT):
            blk = jnp.broadcast_to(sc[:, t * 128:(t + 1) * 128], (128, 128))
            scb_s[t * 128:(t + 1) * 128, :] = blk.T

    def mod_chunk_vpu(j):
        cs = slice(j * MC, (j + 1) * MC)
        acc = paced(jnp.zeros((AR, 128), F32))
        acc = jnp.concatenate([acc] * (MC // 128), axis=1)
        for r in range(0, D, AR):
            sc = after(acc[:, :128], scb_s[r:r + AR, :])
            sc = jnp.concatenate([sc] * (MC // 128), axis=1)
            acc = acc + wmod_v[r:r + AR, cs].astype(F32) * sc
        res = jnp.sum(acc, axis=0, keepdims=True)
        if j // per in (1, 4):
            res = res + 1.0
        mod_v[:, cs] = jnp.broadcast_to(res, (8, MC))

    tokens = []

    def after(dep, val):
        return jnp.where(zero_v[...] != 0, dep, val)

    def paced(val):
        if not tokens:
            return val
        return after(tokens.pop(0), val)

    def paced_rows(val):
        top = jnp.concatenate([paced(val[:AR, :128]), val[:AR, 128:]], axis=1)
        return jnp.concatenate([top, val[AR:]], axis=0) if val.shape[0] > AR else top

    def post(*results):
        tokens[:] = [res[TM - AR:TM, c:c + 128] for c0 in (0, 128)
                     for res in results for c in range(c0, res.shape[1], 256)]

    def mod(k):
        return mod_v[0:1, k * D:(k + 1) * D]

    def ln1(i, r):
        xv = paced_rows(x_v[i, r:r + LR, :].astype(F32))
        prev = live.pop(('ln', i, r - MG * LR), None)
        if prev is not None:
            xv = jnp.concatenate([after(prev, xv[:, :128]), xv[:, 128:]], axis=1)
        h = _ln_mod(xv, mod(1), mod(0))
        live['ln', i, r] = h[:, :128]
        h_s[i % 2, r // 2:(r + LR) // 2, :] = _pack(h)

    def ln1_norm0(r):
        x1_s[0, r:r + LR, :] = _ln(x_v[0, r:r + LR, :].astype(F32))

    def ln1_apply0(j):
        cs = slice(j * MC, (j + 1) * MC)
        h_s[0, :, cs] = _pack(x1_s[0, :, cs] * mod_v[0:1, D + j * MC:D + (j + 1) * MC]
                              + mod_v[0:1, cs])

    def prep_qkv(j, k):
        for r in range(k * MC, (k + 1) * MC, 128):
            wqkv_v[r // 2:r // 2 + 64, j * D:(j + 1) * D] = _permute_cols(
                _pack(wraw_v[r:r + 128, j * D:(j + 1) * D]))

    def qkv_first(j, k):
        res = jnp.dot(_unpack(h_s[0, :, k * MC:(k + 1) * MC]),
                      _unpack(wqkv_v[k * MC // 2:(k + 1) * MC // 2, j * D:(j + 1) * D]),
                      preferred_element_type=F32)
        post(res)
        if k > 0:
            dst, r0 = ((q_s, 0), (k_s, HALO), (v_s, HALO))[j]
            res = res + jnp.concatenate([dst[0, t, r0:r0 + TM, :] for t in range(NLT)], axis=1)
        qkv_store(0, j, 0, res, final=k == D // MC - 1)

    def qkv_part(i, j, half):
        c0 = j * D + half * QC
        res = jnp.dot(_unpack(h_s[i % 2]), _unpack(wqkv_v[:, c0:c0 + QC]),
                      preferred_element_type=F32)
        qkv_store(i, j, half, res)
        post(res)

    def qkv_store(i, j, half, res, final=True):
        sl = i % 2
        for tt in range(res.shape[1] // 128):
            t = half * (QC // 128) + tt
            blk = res[:, tt * 128:(tt + 1) * 128]
            if j == 0:
                q_s[sl, t] = blk * SCALE if final else blk
                continue
            dst = k_s if j == 1 else v_s
            dst[sl, t, HALO:HALO + TM, :] = blk
            if not final:
                continue
            if i == 0:
                dst[sl, t, 0:HALO, :] = jnp.broadcast_to(blk[0:1], (HALO, 128))
            else:
                dst[sl, t, 0:HALO, :] = dst[1 - sl, t, TM:TM + HALO, :]

    live = {}

    def window(ref, sl, t, r, w):
        o = HALO + r - DIL * w
        return ref[sl, t, o:o + AR, :]

    def attn_qk(i, r):
        sl = i % 2
        lg = None
        for t in range(NLT):
            q = q_s[sl, t, r:r + AR, :]
            if t == 0:
                q = paced(q)
            else:
                q = after(lg[-1], q)
            prod = []
            for w in range(W):
                if w and w % G[i > 0] == 0:
                    q = after(prod[-1], q)
                prod.append(q * window(k_s, sl, t, r, w))
            lg = prod if lg is None else [a + b for a, b in zip(lg, prod)]
        live[i, r] = lg

    def attn_lanes(i, r):
        lane = lax.broadcasted_iota(jnp.int32, (AR, 128), 1)
        b0 = (lane & 1) == 0
        b1 = (lane & 2) == 0
        lg = [a + jnp.where(b0, pltpu.roll(a, 127, 1), pltpu.roll(a, 1, 1)) for a in live[i, r]]
        lg = [a + jnp.where(b1, pltpu.roll(a, 126, 1), pltpu.roll(a, 2, 1)) for a in lg]
        live[i, r] = lg

    def attn_softmax(i, r):
        lg = live[i, r]
        if i == 0 and r < DIL * (W - 1):
            row = lax.broadcasted_iota(jnp.int32, (AR, 128), 0) + r
            lg = [jnp.where(row >= DIL * w, a, -1000000000.0 * LOG2E) for w, a in enumerate(lg)]
        m = lg[0]
        for w in range(1, W):
            m = jnp.maximum(m, lg[w])
        e = []
        for w, a in enumerate(lg):
            if w and w % 2 == 0:
                m = after(e[-1], m)
            e.append(jnp.exp2(a - m))
        s = e[0]
        for w in range(1, W):
            s = s + e[w]
        inv = 1.0 / s
        live[i, r] = [a * inv for a in e]

    def attn_pv(i, r):
        sl = i % 2
        p = live.pop((i, r))
        outs = None
        for w in range(W):
            pw = after(outs[-1], p[w]) if w else p[w]
            prod = []
            for t in range(NLT):
                if t and t % G[i > 0] == 0:
                    pw = after(prod[-1], pw)
                prod.append(pw * window(v_s, sl, t, r, w))
            outs = prod if outs is None else [a + b for a, b in zip(outs, prod)]
        o_s[r // 2:(r + AR) // 2, :] = _pack(jnp.concatenate(outs, axis=1))

    def attn_unpermute(i, r):
        rows = slice(r // 2, (r + AR) // 2)
        o_s[rows, :] = _permute_cols(o_s[rows, :])

    def wo_part(i, r0):
        y = jnp.dot(_unpack(o_s[r0 // 2:(r0 + WR) // 2, :]), wo_v[...],
                    preferred_element_type=F32)
        done = []
        for r in range(r0, r0 + WR, LR):
            x1 = x_v[i, r:r + LR, :].astype(F32) + mod(2) * y[r - r0:r - r0 + LR]
            x1_s[i % 2, r:r + LR, :] = x1
            if done:
                x1 = jnp.concatenate([after(done[-1], x1[:, :128]), x1[:, 128:]], axis=1)
            h2 = _ln_mod(x1, mod(4), mod(3))
            done.append(h2[:, :128])
            h2_s[r // 2:(r + LR) // 2, :] = _pack(h2)

    def gate_up(cix):
        cs = slice(cix * FC, (cix + 1) * FC)
        h2 = _unpack(h2_s[...])
        g = jnp.dot(h2, wg_v[:, cs], preferred_element_type=F32)
        u = jnp.dot(h2, wu_v[:, cs], preferred_element_type=F32)
        post(g, u)
        t = 0.5 * g
        act_s[:, cs] = _pack((t + t * jnp.tanh(t)) * u)

    def down(i, n):
        cs = slice(n * DC, (n + 1) * DC)
        y = jnp.dot(_unpack(act_s[...]), wd_v[:, cs], preferred_element_type=F32)
        post(y)
        gb = mod_v[0:1, 5 * D + n * DC:5 * D + (n + 1) * DC]
        out_v[i, :, cs] = (x1_s[i % 2, :, cs] + gb * y).astype(out_v.dtype)

    def par(mxu, vpu):
        done = 0
        for idx, (fn, *args) in enumerate(mxu):
            upto = len(vpu) * (idx + 1) // len(mxu)
            for vfn, *vargs in vpu[done:upto]:
                vfn(*vargs)
            done = upto
            fn(*args)

    def weave(a, b):
        keyed = [((n + 0.5) / len(ts), t) for ts in (a, b) for n, t in enumerate(ts)]
        return [t for _, t in sorted(keyed, key=lambda kt: kt[0])]

    halves = range(D // QC)

    def t_qkv(i, js=(0, 1, 2)):
        return [(qkv_part, i, j, hf) for j in js for hf in halves]

    def t_attn(i):
        stages = (attn_qk, attn_lanes, attn_softmax, attn_pv, attn_unpermute)
        nb = TM // AR
        return [(fn, i, (n - k) * AR) for n in range(nb + len(stages) - 1)
                for k, fn in reversed(list(enumerate(stages))) if 0 <= n - k < nb]

    def t_ln(fn, i):
        return [(fn, i, r) for r in range(0, TM, LR)] if i < NT else []

    def t_wo(i):
        return [(wo_part, i, r) for r in range(0, TM, WR)]

    t_gu = [(gate_up, cix) for cix in range(NFC)]

    def t_down(i, ns):
        return [(down, i, n) for n in ns]

    def t_mod(ks):
        return [(mod_chunk_vpu, j) for k in ks for j in range(k * per, (k + 1) * per)]

    def wait(cps):
        for cp in cps:
            cp.wait()

    def chunk_cps(k):
        return [mod_cp[k], mod_cp[per + k], qkv_cp[k]]

    def modulate0(k):
        tokens.clear()
        for j in (k, per + k):
            (mod_chunk_vpu if k else mod_chunk)(j)
        ln1_apply0(k)

    start(small_cps + [x_cp[0]] + chunk_cps(0))
    wait(small_cps)
    silu_c_columns()
    x_cp[0].wait()
    start([kv0_cp])
    par([(ln1_norm0, r) for r in range(0, TM, LR)], [])
    qkv_cp[0].wait()
    prep_qkv(0, 0)
    wait(chunk_cps(0)[:2])
    start(chunk_cps(1))
    modulate0(0)
    kv0_cp.wait()
    arrive = [chunk_cps(k) for k in range(per)]
    arrive[-1] += [x_cp[1]]
    later = [chunk_cps(k) for k in range(2, per)]
    later += [[x_cp[2]] + mod_cps(2) + [wo_cp], mod_cps(3) + mod_cps(4) + mod_cps(5)]
    steps = [(j, k) for k in range(per) for j in range(3)]
    ln_next = t_ln(ln1, 1)
    for n, (j, k) in enumerate(steps):
        if j == 2:
            if k + 1 < per:
                wait(arrive[k + 1])
            start(later[k])
            if k == 0:
                x_cp[1].start()
            if k + 1 < per:
                modulate0(k + 1)
        if n + 1 < len(steps):
            prep_qkv(*steps[n + 1])
        left = len(steps) - n
        if left <= NL:
            q = len(ln_next) // NL
            par(ln_next[(NL - left) * q:(NL - left + 1) * q], [])
        qkv_first(j, k)
    x_cp[2].wait()
    start([wg_cp])
    par(t_qkv(1), weave(t_attn(0), t_ln(ln1, 2)))
    wait(mod_cps(2) + mod_cps(3) + mod_cps(4) + mod_cps(5) + [wo_cp])
    x_rest = [x_cp[i] for i in range(3, NT)]
    start([wu_cp])
    q2 = t_qkv(2)
    par(q2[:-1], t_mod((2, 3, 4)))
    par(t_wo(0), [])
    par(q2[-1:], [])
    wait([wg_cp, wu_cp])
    start([wd_cp] + x_rest)
    first, second = range(N_D1), range(N_D1, NDC)
    for i in range(1, NT):
        att = t_attn(i)
        par(t_gu, weave(att[:NA], t_mod((5,)) if i == 1 else []))
        if i == 1:
            wait([wd_cp] + x_rest)
        par(t_down(i - 1, first), weave(att[NA:], t_ln(ln1, i + 2)))
        par(t_wo(i), [])
        par(t_down(i - 1, second), [])
        if i + 2 < NT:
            par(t_qkv(i + 2), [])
    out_cps[0].start()
    par(t_gu, [])
    par(t_down(NT - 1, range(NDC - 1)), [])
    out_cps[1].start()
    down(NT - 1, NDC - 1)
    out_cps[2].start()
    wait(out_cps)


@jax.jit
def pallas_adaLN_cond__sliding_local_dilated__swiglu_ffn__prompt_kernel(
    A_x: jax.Array,
    A_wqkv: jax.Array,
    A_wo: jax.Array,
    B_x: jax.Array,
    B_w_gate: jax.Array,
    B_w_up: jax.Array,
    B_w_down: jax.Array,
    c: jax.Array,
    w_mod: jax.Array,
):
    del B_x
    x = A_x.reshape(NT, TM, D)
    hbm = pl.BlockSpec(memory_space=pl.ANY)
    out = pl.pallas_call(
        _kernel,
        in_specs=[hbm] * 9,
        out_specs=hbm,
        out_shape=jax.ShapeDtypeStruct((NT, TM, D), A_x.dtype),
        scratch_shapes=[
            pltpu.VMEM((AR, 128), jnp.int32),
            pltpu.VMEM((1, D), BF16),
            pltpu.VMEM((NT, TM, D), BF16),
            pltpu.VMEM((NT, TM, D), BF16),
            pltpu.VMEM((D, 6 * D), BF16),
            pltpu.VMEM((D, 3 * D), BF16),
            pltpu.VMEM((D // 2, 3 * D), U32),
            pltpu.VMEM((D, D), BF16),
            pltpu.VMEM((D, F), BF16),
            pltpu.VMEM((D, F), BF16),
            pltpu.VMEM((F, D), BF16),
            pltpu.VMEM((8, 6 * D), F32),
            pltpu.VMEM((D, 128), F32),
            pltpu.VMEM((2, TM // 2, D), U32),
            pltpu.VMEM((2, NLT, TM, 128), F32),
            pltpu.VMEM((2, NLT, HALO + TM, 128), F32),
            pltpu.VMEM((2, NLT, HALO + TM, 128), F32),
            pltpu.VMEM((TM // 2, D), U32),
            pltpu.VMEM((2, TM, D), F32),
            pltpu.VMEM((TM // 2, D), U32),
            pltpu.VMEM((TM // 2, F), U32),
            pltpu.SemaphoreType.DMA((6 * D // MC + 9,)),
            pltpu.SemaphoreType.DMA((D // MC + 1,)),
            pltpu.SemaphoreType.DMA((NT,)),
            pltpu.SemaphoreType.DMA((3,)),
        ],
        compiler_params=pltpu.CompilerParams(
            vmem_limit_bytes=110 * 1024 * 1024,
        ),
    )(np.zeros((AR, 128), np.int32), x, c, w_mod, A_wqkv, A_wo, B_w_gate, B_w_up, B_w_down)
    return out.reshape(A_x.shape)
```
